```python
import jax
import jax.numpy as jnp

def _softmax(x, axis=-1):
    return jax.nn.softmax(x, axis=axis)

def _gelu(x):
    return jax.nn.gelu(x, approximate=True)

def _silu(x):
    return jax.nn.silu(x)

def _sigmoid(x):
    return jax.nn.sigmoid(x)

def _layernorm(x, axis=-1, eps=1e-05):
    m = jnp.mean(x, axis=axis, keepdims=True)
    v = jnp.var(x, axis=axis, keepdims=True)
    return (x - m) / jnp.sqrt(v + eps)

def _scatter_add(tgt, idx, src, axis=0):
    return tgt.at[idx].add(src)

def _segment_sum(src, seg, n):
    return jax.ops.segment_sum(src, seg, n)

class _Rng:

    def __init__(self, key):
        self._k = key

    def _next(self):
        self._k, sub = jax.random.split(self._k)
        return sub

    def normal(self, shape):
        return jax.random.normal(self._next(), shape, dtype=jnp.bfloat16)

    def randint(self, lo, hi, shape):
        return jax.random.randint(self._next(), shape, lo, hi, dtype=jnp.int32)

    def uniform(self, shape, lo=0.0, hi=1.0):
        return jax.random.uniform(self._next(), shape, jnp.bfloat16, lo, hi)

    def permutation(self, n):
        return jax.random.permutation(self._next(), n)
kernel_name = 'parallel_sum__memory_aug_infini_attn__moe_arch_mod__prompt'

def setup_inputs():
    _rng = _Rng(jax.random.key(int.from_bytes(__import__("os").urandom(4), "little")))
    _w = lambda a: (lambda t: t.astype(jnp.bfloat16) if jnp.issubdtype(t.dtype, jnp.floating) else t)(jnp.asarray(a))

    def _A_setup():
        B, S, D, H = (1, 2048, 576, 32)
        N = 4
        L = max(1, S // N)
        sc = D ** (-0.5)
        return {'x': _w((lambda *s: _rng.normal(s) * 0.05)(B, N * L, D)), 'wq': _w((lambda *s: _rng.normal(s) * 0.05)(D, D) * sc), 'wk': _w((lambda *s: _rng.normal(s) * 0.05)(D, D) * sc), 'wv': _w((lambda *s: _rng.normal(s) * 0.05)(D, D) * sc), 'wo': _w((lambda *s: _rng.normal(s) * 0.05)(D, D) * sc), 'beta': _w((lambda *s: _rng.normal(s) * 0.05)(H))}
    _A_in = _A_setup()

    def _B_setup():
        B, S, D, F, C = (1, 2048, 576, 4608, 2)
        return {'x': _w((lambda *s: _rng.normal(s) * 0.05)(B, S, D)), 'w_r': _w((lambda *s: _rng.normal(s) * 0.05)(D)), 'w_gate': _w((lambda *s: _rng.normal(s) * 0.05)(D, F)), 'w_up': _w((lambda *s: _rng.normal(s) * 0.05)(D, F)), 'w_down': _w((lambda *s: _rng.normal(s) * 0.05)(F, D))}
    _B_in = _B_setup()
    return {'A_x': _A_in['x'], 'A_wq': _A_in['wq'], 'A_wk': _A_in['wk'], 'A_wv': _A_in['wv'], 'A_wo': _A_in['wo'], 'A_beta': _A_in['beta'], 'B_x': _B_in['x'], 'B_w_r': _B_in['w_r'], 'B_w_gate': _B_in['w_gate'], 'B_w_up': _B_in['w_up'], 'B_w_down': _B_in['w_down']}

def reference(A_x, A_wq, A_wk, A_wv, A_wo, A_beta, B_x, B_w_r, B_w_gate, B_w_up, B_w_down):

    def _A_ref(x, wq, wk, wv, wo, beta):
        B, S, D = x.shape
        H = 32
        Dh = D // H
        N = 4
        L = S // N
        q = (lambda x, *d: x.transpose(*d))((x @ wq).reshape(B, S, H, Dh), 0, 2, 1, 3).reshape(B, H, N, L, Dh)
        k = (lambda x, *d: x.transpose(*d))((x @ wk).reshape(B, S, H, Dh), 0, 2, 1, 3).reshape(B, H, N, L, Dh)
        v = (lambda x, *d: x.transpose(*d))((x @ wv).reshape(B, S, H, Dh), 0, 2, 1, 3).reshape(B, H, N, L, Dh)
        phi = lambda t: jnp.where(t > 0, t + 1.0, jnp.exp(t))
        scale = Dh ** (-0.5)
        ar = jnp.arange(L)
        mask = (lambda x, dt: x.astype(dt))(ar[:, None] < ar[None, :], x.dtype) * -1000000000.0
        g = _sigmoid(beta).reshape(1, H, 1, 1)
        M = jnp.einsum('bhd,bhe->bhde', q[:, :, 0, 0, :] * 0.0, q[:, :, 0, 0, :] * 0.0)
        z = q[:, :, 0, 0, :] * 0.0
        outs = []
        for s in range(N):
            qs, ks, vs = (q[:, :, s].copy(), k[:, :, s].copy(), v[:, :, s].copy())
            logits = jnp.einsum('bhqd,bhkd->bhqk', qs, ks) * scale + mask
            p = _softmax(logits, axis=-1)
            a_dot = jnp.einsum('bhqk,bhkd->bhqd', p, vs)
            pq = phi(qs)
            num = jnp.einsum('bhld,bhde->bhle', pq, M)
            den = jnp.einsum('bhld,bhd->bhl', pq, z)[..., None] + 1e-06
            a_mem = num / den
            o = g * a_mem + (1.0 - g) * a_dot
            outs.append(o)
            pk = phi(ks)
            M = M + jnp.einsum('bhld,bhle->bhde', pk, vs)
            z = z + jnp.einsum('bhld->bhd', pk)
        o = (lambda x, *d: x.transpose(*d))(jnp.stack(outs, 2).reshape(B, H, S, Dh), 0, 2, 1, 3).reshape(B, S, D)
        return o @ wo

    def _B_ref(x, w_r, w_gate, w_up, w_down):
        B, S, D = x.shape
        C = 2
        r = x @ w_r
        idx = jnp.argsort(-r, axis=-1)[:, :C]
        idx_e = jnp.repeat(idx.reshape(B, C, 1), D, axis=2)
        x_sel = jnp.take_along_axis(x, idx_e, axis=1)
        g = _silu(x_sel @ w_gate)
        u = x_sel @ w_up
        y = g * u @ w_down
        r_sel = _sigmoid(jnp.take_along_axis(r, idx, axis=1))
        y = y * r_sel.reshape(B, C, 1)
        b_off = (jnp.arange(B) * S).reshape(B, 1)
        flat_idx = (idx + b_off).reshape(B * C)
        zero = (x * 0.0).reshape(B * S, D)
        upd = _scatter_add(zero, flat_idx, y.reshape(B * C, D), axis=0)
        return x + upd.reshape(B, S, D)
    x = A_x
    xn = _layernorm(x, axis=-1)
    return x + _A_ref(xn, A_wq, A_wk, A_wv, A_wo, A_beta) + _B_ref(xn, B_w_r, B_w_gate, B_w_up, B_w_down)
```

```python
import functools

import jax
import jax.numpy as jnp
import numpy as np
from jax import lax
import jax.experimental.pallas as pl
import jax.experimental.pallas.tpu as pltpu

D = 576
DP = 640
S = 2048
H = 32
DH = 18
NSEG = 4
L = 512
F = 4608
NG = 8
GH = 4
GR = 72
GP = 80
T = 128
NT = L // T

F32 = jnp.float32
BF16 = jnp.bfloat16
U32 = jnp.uint32
LOG2E = 1.4426950408889634
QSCALE = float(DH ** -0.5 * LOG2E)
EPS_BF16 = float(np.asarray(1e-5, dtype=jnp.bfloat16).astype(np.float32))


def _rnd(x):
    return x.astype(BF16).astype(F32)


def _pack(x):
    return pltpu.bitcast(x.astype(BF16), U32)


def _unpack(x):
    return pltpu.bitcast(x, BF16)


def _dot(a, b):
    return lax.dot_general(a, b, (((1,), (0,)), ((), ())), preferred_element_type=F32)


def _dot_nt(a, b):
    return lax.dot_general(a, b, (((1,), (1,)), ((), ())), preferred_element_type=F32)


def _phi(t):
    return jnp.where(t > 0, t + 1.0, jnp.exp(t))


def _iota(shape, axis):
    return lax.broadcasted_iota(jnp.int32, shape, axis)


def _head_of(i):
    return (i * 57) >> 10


def _kernel(x_hbm, wq_hbm, wk_hbm, wv_hbm, wo_hbm, beta_ref, wr_ref, wg_hbm, wu_hbm, wd_hbm,
            out_hbm,
            xbuf, wbuf, wg_s, wu_s, wd_s, xn_s, base_s, wt_s, wot_s, gate_s, m_s, ot_s, out_s,
            r_s, y_s, q_s, k_s, v_s, pq_s, pk_s, sems):

    def x_copy(s):
        return pltpu.make_async_copy(x_hbm.at[:, :, pl.ds(s * L, L)], xbuf.at[s], sems.at[s])

    def w_copy(i):
        return pltpu.make_async_copy((wq_hbm, wk_hbm, wv_hbm, wo_hbm)[i], wbuf.at[i], sems.at[4 + i])

    def f_copy(i):
        return pltpu.make_async_copy((wg_hbm, wu_hbm, wd_hbm)[i], (wg_s, wu_s, wd_s)[i], sems.at[8 + i])

    def o_copy(s):
        return pltpu.make_async_copy(out_s.at[s], out_hbm.at[:, :, pl.ds(s * L, L)], sems.at[11 + s])

    x_copy(0).start()
    for i in range(3):
        w_copy(i).start()
    for s in range(1, NSEG):
        x_copy(s).start()
    w_copy(3).start()

    g_row = jax.nn.sigmoid(beta_ref[...].astype(F32)).reshape(1, H)
    for g in range(NG):
        head = _head_of(_iota((GR, H), 0)) + g * GH
        col = jnp.sum(jnp.where(head == _iota((GR, H), 1), g_row, 0.0), axis=1, keepdims=True)
        gate_s[g] = jnp.broadcast_to(col, (GR, T))
    m_s[...] = jnp.zeros(m_s.shape, F32)

    wr_row = wr_ref[...].astype(F32).reshape(1, D)
    wr_lhs = jnp.concatenate([jnp.broadcast_to(wr_row, (8, D)), jnp.zeros((8, DP - D), F32)], axis=1)

    def layer_norm(s):
        for t in range(NT):
            lanes = pl.ds(t * T, T)
            xf = xbuf[s, :, :, lanes].astype(F32).reshape(D, T)
            mean = jnp.sum(xf, axis=0, keepdims=True) / D
            cen = xf - mean
            var = jnp.sum(cen * cen, axis=0, keepdims=True) / D
            sd = _rnd(jnp.sqrt(_rnd(_rnd(var) + EPS_BF16)))
            xn = _rnd(_rnd(xf - _rnd(mean)) * (1.0 / sd))
            base_s[s, :, :, lanes] = (xf + xn).reshape(NG, GR, T)
            xn_s[s, :, lanes] = _pack(jnp.concatenate([xn, jnp.zeros((DP - D, T), F32)], axis=0))
        r_s[:, pl.ds(s * L, L)] = _dot(wr_lhs, _unpack(xn_s[s]))

    x_copy(0).wait()
    layer_norm(0)

    for i in range(3):
        w_copy(i).wait()
        w = wbuf[i].astype(F32)
        w = jnp.concatenate([w, jnp.zeros((DP - D, D), F32)], axis=0)
        w = jnp.concatenate([w, jnp.zeros((DP, DP - D), F32)], axis=1)
        wt = w.T
        for g in range(NG):
            wt_s[g, pl.ds(i * GR, GR), :] = wt[g * GR:(g + 1) * GR]

    for s in range(1, NSEG):
        x_copy(s).wait()
    w_copy(3).wait()
    for i in range(3):
        f_copy(i).start()
    for s in range(1, NSEG):
        layer_norm(s)

    w = wbuf[3].astype(F32)
    w = jnp.concatenate([w, jnp.zeros((D, DP - D), F32)], axis=1)
    parts = []
    for g in range(NG):
        parts += [w[g * GR:(g + 1) * GR], jnp.zeros((GP - GR, DP), F32)]
    wt = jnp.concatenate(parts, axis=0).T
    for g in range(NG):
        wot_s[g] = wt[g * GR:(g + 1) * GR]

    r = _rnd(r_s[...])
    tok = _iota((8, S), 1)
    r0 = jnp.max(r, axis=1, keepdims=True)
    i0 = jnp.min(jnp.where(r == r0, tok, S - 1), axis=1, keepdims=True)
    rest = jnp.where(tok == i0, -jnp.inf, r)
    r1 = jnp.max(rest, axis=1, keepdims=True)
    i1 = jnp.min(jnp.where((rest == r1) & (tok != i0), tok, S - 1), axis=1, keepdims=True)
    idx = (jnp.clip(jnp.max(i0), 0, S - 1), jnp.clip(jnp.max(i1), 0, S - 1))
    r_sel = jax.nn.sigmoid(jnp.where(_iota((8, 1), 0) == 0, r0, r1))

    def qkv(s, g):
        qkvt = _dot(wt_s[g], _unpack(xn_s[s]))
        qt, kt, vt = qkvt[0:GR], qkvt[GR:2 * GR], qkvt[2 * GR:3 * GR]
        zpad = jnp.zeros((GP - GR, L), F32)
        q_s[...] = _pack(jnp.concatenate([qt * QSCALE, zpad], axis=0))
        pq_s[...] = _pack(jnp.concatenate([_phi(qt), zpad], axis=0))
        kn = jnp.concatenate([kt, jnp.zeros((T - GR, L), F32)], axis=0).T
        k_s[...] = _pack(kn)
        pk_s[...] = _pack(_phi(kn))
        v_s[...] = _rnd(vt)

    def attention(g, slot):
        vt = v_s[...]
        sub = _iota((8, L), 0)
        vwin = [
            jnp.concatenate([vt[0:16], jnp.where(sub == 7, 1.0, vt[16:24])], axis=0),
            jnp.concatenate([vt[16:32], jnp.where(sub == 7, 1.0, vt[32:40])], axis=0),
            jnp.concatenate([vt[32:48], jnp.where(sub == 7, 1.0, vt[48:56])], axis=0),
            jnp.concatenate([jnp.where(sub == 0, 1.0, vt[48:56]), vt[56:72]], axis=0),
        ]
        ones_row = [23, 23, 23, 0]

        row = _iota((GP, T), 0)
        col = _iota((GP, T), 1)
        row_head = jnp.where(row < GR, _head_of(row), row - GR)
        m_old = m_s[g]
        m_lhs = jnp.where((row_head == _head_of(col)) & (col < GR), m_old, 0.0).astype(BF16)
        pq = jnp.concatenate([pq_s[...], jnp.zeros(((T - GP) // 2, L), U32)], axis=0)
        nd = _dot(m_lhs, _unpack(pq))
        inv_den = 1.0 / (nd[GR:GP] + 1e-6)
        v1 = jnp.concatenate([vt, jnp.ones((GP - GR, L), F32)], axis=0).astype(BF16)
        m_s[g] = m_old + _dot(v1, _unpack(pk_s[...]))

        gate = gate_s[g]
        s8 = _iota((8, T), 0)
        causal = jnp.where(_iota((T, T), 0) > _iota((T, T), 1), -1e30, 0.0)
        causal = jnp.concatenate([causal] * GH, axis=1)
        for i in range(NT):
            lanes = pl.ds(i * T, T)
            nk = (i + 1) * T
            qp = q_s[:, lanes]
            prow = _iota((GP // 2, T), 0)
            rhs = []
            for j in range(GH):
                qm = jnp.where((prow >= 9 * j) & (prow < 9 * (j + 1)), qp, jnp.uint32(0))
                rhs.append(jnp.concatenate([qm, jnp.zeros(((T - GP) // 2, T), U32)], axis=0))
            rhs = _unpack(jnp.concatenate(rhs, axis=1))
            st = _dot(_unpack(k_s[pl.ds(0, nk // 2), :]), rhs)
            if i == 0:
                st = st + causal
            else:
                st = jnp.concatenate([st[:nk - T], st[nk - T:] + causal], axis=0)
            mx = jnp.max(st, axis=0, keepdims=True)
            p = jnp.exp2(st - mx).astype(BF16)
            o = []
            for j in range(GH):
                oj = _dot(vwin[j][:, :nk], p[:, j * T:(j + 1) * T])
                o.append(oj * (1.0 / oj[ones_row[j]:ones_row[j] + 1]))
            a_dot = jnp.concatenate([
                o[0][0:16], jnp.where(s8 < 2, o[0][16:24], o[1][0:8]),
                o[1][8:16], jnp.where(s8 < 4, o[1][16:24], o[2][0:8]),
                o[2][8:16], jnp.where(s8 < 6, o[2][16:24], o[3][0:8]),
                o[3][8:24]], axis=0)
            iv = [jnp.broadcast_to(inv_den[j:j + 1, i * T:(i + 1) * T], (8, T)) for j in range(GH)]
            ivr = jnp.concatenate([
                iv[0], iv[0], jnp.where(s8 < 2, iv[0], iv[1]),
                iv[1], jnp.where(s8 < 4, iv[1], iv[2]),
                iv[2], jnp.where(s8 < 6, iv[2], iv[3]),
                iv[3], iv[3]], axis=0)
            a_mem = nd[0:GR, i * T:(i + 1) * T] * ivr
            og = gate * a_mem + (1.0 - gate) * a_dot
            og = jnp.concatenate([og, jnp.zeros((GP - GR, T), F32)], axis=0)
            ot_s[slot, pl.ds(pl.multiple_of(g * (GP // 2), 8), GP // 2), lanes] = _pack(og)

    def out_proj(s, g):
        a = _dot(wot_s[g], _unpack(ot_s[s % 2]))
        out_s[s, g] = (base_s[s, g] + a).astype(BF16)

    def ffn():
        xs = jnp.zeros((8, DP), F32)
        for c in range(2):
            tile = xn_s[idx[c] // L, :, pl.ds(pl.multiple_of((idx[c] % L) // T * T, T), T)]
            hot = ((_iota((8, T), 1) == idx[c] % T) & (_iota((8, T), 0) == c)).astype(F32)
            xs = xs + _dot_nt(hot, _unpack(tile))
        xs = xs[:, :D]
        for i in range(3):
            f_copy(i).wait()
        gt = _dot(xs, wg_s[...])
        up = _dot(xs, wu_s[...])
        h = _rnd(gt * jax.nn.sigmoid(gt) * up)
        y = _dot_nt(h, wd_s[...]) * r_sel
        y = jnp.concatenate([y, jnp.zeros((8, DP - D), F32)], axis=1)
        yt = jnp.concatenate([y, jnp.zeros((T - 8, DP), F32)], axis=0).T[:D]
        for c in range(2):
            y_s[c] = jnp.broadcast_to(yt[:, c:c + 1], (D, T)).reshape(NG, GR, T)

    def finalize(s):
        for c in range(2):
            @pl.when(idx[c] // L == s)
            def _():
                lanes = pl.ds(pl.multiple_of((idx[c] % L) // T * T, T), T)
                cur = out_s[s, :, :, lanes].astype(F32)
                hit = _iota((NG, GR, T), 2) == idx[c] % T
                out_s[s, :, :, lanes] = jnp.where(hit, cur + y_s[c], cur).astype(BF16)
        o_copy(s).start()

    def segment(s, c):
        def group(g, c):
            qkv(s, g)
            attention(g, s % 2)
            return c
        lax.fori_loop(0, NG, group, 0)

        def oproj(g, c):
            out_proj(s, g)
            return c
        lax.fori_loop(0, NG, oproj, 0)

        @pl.when(s == 1)
        def _():
            ffn()
            finalize(0)

        @pl.when(s >= 1)
        def _():
            finalize(s)
        return c

    lax.fori_loop(0, NSEG, segment, 0)
    for s in range(NSEG):
        o_copy(s).wait()


@jax.jit
def pallas_parallel_sum__memory_aug_infini_attn__moe_arch_mod__prompt_kernel(
    A_x, A_wq, A_wk, A_wv, A_wo, A_beta, B_x, B_w_r, B_w_gate, B_w_up, B_w_down,
):
    del B_x
    xt = jnp.transpose(A_x[0]).reshape(NG, GR, S)
    wdt = jnp.transpose(B_w_down)
    hbm = pl.BlockSpec(memory_space=pltpu.HBM)
    vmem = pl.BlockSpec(memory_space=pltpu.VMEM)
    out = pl.pallas_call(
        _kernel,
        out_shape=jax.ShapeDtypeStruct((NG, GR, S), BF16),
        in_specs=[hbm, hbm, hbm, hbm, hbm, vmem, vmem, hbm, hbm, hbm],
        out_specs=hbm,
        scratch_shapes=[
            pltpu.VMEM((NSEG, NG, GR, L), BF16),
            pltpu.VMEM((4, D, D), BF16),
            pltpu.VMEM((D, F), BF16),
            pltpu.VMEM((D, F), BF16),
            pltpu.VMEM((D, F), BF16),
            pltpu.VMEM((NSEG, DP // 2, L), U32),
            pltpu.VMEM((NSEG, NG, GR, L), F32),
            pltpu.VMEM((NG, 3 * GR, DP), F32),
            pltpu.VMEM((NG, GR, DP), F32),
            pltpu.VMEM((NG, GR, T), F32),
            pltpu.VMEM((NG, GP, T), F32),
            pltpu.VMEM((2, DP // 2, L), U32),
            pltpu.VMEM((NSEG, NG, GR, L), BF16),
            pltpu.VMEM((8, S), F32),
            pltpu.VMEM((2, NG, GR, T), F32),
            pltpu.VMEM((GP // 2, L), U32),
            pltpu.VMEM((L // 2, T), U32),
            pltpu.VMEM((GR, L), F32),
            pltpu.VMEM((GP // 2, L), U32),
            pltpu.VMEM((L // 2, T), U32),
            pltpu.SemaphoreType.DMA((15,)),
        ],
        compiler_params=pltpu.CompilerParams(vmem_limit_bytes=100 * 1024 * 1024),
        name="infini_mod",
    )(xt, A_wq, A_wk, A_wv, A_wo, A_beta, B_w_r, B_w_gate, B_w_up, wdt)
    return jnp.transpose(out.reshape(D, S))[None]
```

```python
import jax
import jax.numpy as jnp
import numpy as np
from jax import lax
import jax.experimental.pallas as pl
import jax.experimental.pallas.tpu as pltpu

D = 576
DP = 640
S = 2048
H = 32
DH = 18
NSEG = 4
L = 512
F = 4608
NG = 8
GH = 4
GR = 72
GP = 80
T = 128
HT = T // 2
NT = L // T

F32 = jnp.float32
BF16 = jnp.bfloat16
LOG2E = 1.4426950408889634
QSCALE = float(DH ** -0.5 * LOG2E)
EPS_BF16 = float(np.asarray(1e-5, dtype=jnp.bfloat16).astype(np.float32))
NEG = -1e30

ORDER = "pmxfo"
KP = 128


def _rnd(x):
    return x.astype(BF16).astype(F32)


def _dot(a, b):
    return lax.dot_general(a, b, (((1,), (0,)), ((), ())), preferred_element_type=F32)


def _dot_nt(a, b):
    return lax.dot_general(a, b, (((1,), (1,)), ((), ())), preferred_element_type=F32)


def _phi(t):
    return jnp.where(t > 0, t + 1.0, jnp.exp(t))


def _iota(shape, axis):
    return lax.broadcasted_iota(jnp.int32, shape, axis)


def _head_of(i):
    return (i * 57) >> 10


def _ds(i, n, align):
    return pl.ds(i if isinstance(i, int) else pl.multiple_of(i, align), n)


def _lane_tile(t):
    return _ds(t * T, T, T)


def _rows_max(x):
    return jnp.max(x.reshape(x.shape[0] // 8, 8, T), axis=0)


def _exp2_shifted(x, m):
    return jnp.exp2(x.reshape(x.shape[0] // 8, 8, T) - m[None]).reshape(x.shape)


def _kernel(x_hbm, wq_hbm, wk_hbm, wv_hbm, wo_hbm, beta_ref, wr_ref, wg_hbm, wu_hbm, wd_hbm,
            out_hbm,
            xbuf, wa_s, wb_s, wo_s, wg_s, wu_s, wd_s, xn_s, base_s, wt_s, wot_s, wr_s, gate_s, m_s,
            ot_s, out_s, r_s, y_s, q_s, k_s, buf_a, buf_b, st_s, sb_s, mx_s, sems):
    w_hbm = (wq_hbm, wk_hbm, wv_hbm)
    WA = 2 * T

    def x0_copy(t):
        return pltpu.make_async_copy(x_hbm.at[:, :, pl.ds(t * T, T)], xbuf.at[0, :, :, pl.ds(t * T, T)], sems.at[t])

    def x_copy(s):
        return pltpu.make_async_copy(x_hbm.at[:, :, pl.ds(s * L, L)], xbuf.at[s], sems.at[3 + s])

    def wa_copy(i):
        return pltpu.make_async_copy(w_hbm[i].at[:, pl.ds(0, WA)], wa_s.at[i], sems.at[7 + i])

    def wb_copy(i):
        return pltpu.make_async_copy(w_hbm[i].at[:, pl.ds(WA, D - WA)], wb_s.at[i], sems.at[10 + i])

    def wo_copy():
        return pltpu.make_async_copy(wo_hbm, wo_s, sems.at[13])

    def f_copy(i):
        return pltpu.make_async_copy((wg_hbm, wu_hbm, wd_hbm)[i], (wg_s, wu_s, wd_s)[i], sems.at[14 + i])

    def o_copy(s):
        return pltpu.make_async_copy(out_s[s], out_hbm.at[:, :, pl.ds(s * L, L)], sems.at[17 + s])

    def o_last_copy(t):
        return pltpu.make_async_copy(out_s[NSEG - 1].at[:, :, pl.ds(t * T, T)],
                                     out_hbm.at[:, :, pl.ds((NSEG - 1) * L + t * T, T)], sems.at[20 + t])

    for t in range(NT):
        x0_copy(t).start()
    for i in range(3):
        wa_copy(i).start()

    g_row = jax.nn.sigmoid(beta_ref[...].astype(F32)).reshape(1, H)
    for g in range(NG):
        head = _head_of(_iota((GR, H), 0)) + g * GH
        col = jnp.sum(jnp.where(head == _iota((GR, H), 1), g_row, 0.0), axis=1, keepdims=True)
        gate_s[g] = jnp.broadcast_to(col, (GR, T))

    wr_row = wr_ref[...].astype(F32).reshape(1, D)
    wr_s[...] = jnp.concatenate([jnp.broadcast_to(wr_row, (8, D)), jnp.zeros((8, DP - D), F32)], axis=1)

    def layer_norm(s, t):
        lanes = _lane_tile(t)
        xf = xbuf[s, :, :, lanes].astype(F32).reshape(D, T)
        mean = jnp.sum(xf, axis=0, keepdims=True) / D
        cen = xf - mean
        var = jnp.sum(cen * cen, axis=0, keepdims=True) / D
        sd = _rnd(jnp.sqrt(_rnd(_rnd(var) + EPS_BF16)))
        xn = _rnd(_rnd(xf - _rnd(mean)) * (1.0 / sd))
        base_s[s][:, :, lanes] = (xf + xn).reshape(NG, GR, T)
        xn = jnp.concatenate([xn, jnp.zeros((DP - D, T), F32)], axis=0).astype(BF16)
        xn_s[s, :, lanes] = xn
        r_s[s, :, lanes] = _dot(wr_s[...], xn)

    def transpose_w(i, c, w):
        w = jnp.concatenate([w.astype(F32), jnp.zeros((DP - D, T), F32)], axis=0)
        wt_s[i, _lane_tile(c), :] = w.T

    def transpose_wo():
        w = wo_s[...].astype(F32)
        w = jnp.concatenate([w, jnp.zeros((D, DP - D), F32)], axis=1)
        parts = []
        for g in range(NG):
            parts += [w[g * GR:(g + 1) * GR], jnp.zeros((GP - GR, DP), F32)]
        wot_s[...] = jnp.concatenate(parts, axis=0).T[:D]

    s8 = _iota((8, T), 0)

    def project(s, g, buf):
        v_s, pq_s, pk_s = buf
        rows = _ds(g * GR, GR, 8)
        qkvt = _dot(jnp.concatenate([wt_s[i, rows, :] for i in range(3)], axis=0), xn_s[s])
        qt, kt, vt = qkvt[0:GR], qkvt[GR:2 * GR], qkvt[2 * GR:3 * GR]
        q_s[...] = qt * QSCALE
        kn = jnp.concatenate([kt, jnp.zeros((T - GR, L), F32)], axis=0).T
        k_s[...] = kn.astype(k_s.dtype)
        pq_s[...] = _phi(qt)
        pk_s[...] = _phi(kn).astype(pk_s.dtype)
        v_s[...] = vt

    def query_tiles(i):
        qp = q_s[:, pl.ds(i * T, T)]
        qr = pltpu.roll(qp, HT, 1)
        row = _iota((GR, T), 0)
        return [jnp.where((row >= DH * j) & (row < DH * (j + 1)), qp if j % 2 else qr, 0.0) for j in range(GH)]

    def as_weights(tiles):
        pad = jnp.zeros((KP - GR, T), F32)
        return jnp.concatenate([jnp.concatenate([q, pad], axis=0).astype(BF16) for q in tiles], axis=1)

    def attend(i, v_s, consume, produce):
        lane = _iota((HT, T), 1)
        tri = _iota((HT, T), 0) > (lane & (HT - 1))
        masks = [jnp.where(tri & (lane >= HT), NEG, 0.0), jnp.where(tri & (lane < HT), NEG, 0.0)]
        rhs = as_weights(query_tiles(i)) if produce else None
        m_old = [mx_s[i * GH + j] for j in range(GH)] if consume else None
        o = [None] * GH
        mx = [None] * GH

        def weighted_sum(kb, ps):
            keys = pl.ds(kb * T, T)
            for j in range(GH):
                if j < GH - 1:
                    vw = jnp.concatenate([v_s[pl.ds(16 * j, 16), keys],
                                          jnp.where(s8 == 7, 1.0, v_s[pl.ds(16 * j + 16, 8), keys])], axis=0)
                else:
                    vw = jnp.concatenate([jnp.where(s8 == 0, 1.0, v_s[pl.ds(48, 8), keys]),
                                          v_s[pl.ds(56, 16), keys]], axis=0)
                oj = _dot(vw, ps[j])
                o[j] = oj if o[j] is None else o[j] + oj

        def full_probs(kb):
            keys = pl.ds(kb * T, T)
            return [_exp2_shifted(st_s[i][j][keys, :], m_old[j]).astype(BF16) for j in range(GH)]

        def diag_probs():
            ps = []
            for j in range(GH):
                if j % 2 == 0:
                    mb = jnp.where(_iota((8, T), 1) < HT, m_old[j], m_old[j + 1])
                    pb = _exp2_shifted(sb_s[i][j // 2][...], mb)
                head = _exp2_shifted(st_s[i][j][pl.ds(i * T, HT), :], m_old[j])
                tail = jnp.where(lane >= HT if j % 2 else lane < HT, pb, 0.0)
                ps.append(jnp.concatenate([head, tail], axis=0).astype(BF16))
            return ps

        def logits(k0, n):
            st = _dot(k_s[pl.ds(k0, n), :][:, :KP], rhs)
            for j in range(GH):
                sj = st[:, j * T:(j + 1) * T]
                if k0 + n > i * T:
                    tail = sj[n - HT:] + masks[j % 2]
                    sj = tail if n == HT else jnp.concatenate([sj[:n - HT], tail], axis=0)
                st_s[i][j][pl.ds(k0, n), :] = sj
                m = _rows_max(sj)
                mx[j] = m if mx[j] is None else jnp.maximum(mx[j], m)

        pd = diag_probs() if consume else None
        for kb in range(max(i, 1)):
            ps = full_probs(kb) if consume and kb < i else None
            if produce:
                logits(kb * T, T if kb < i - 1 else i * T + HT - kb * T)
            if ps is not None:
                weighted_sum(kb, ps)
        if not consume:
            return None, mx
        weighted_sum(i, pd)
        for j in range(GH):
            one = 23 if j < GH - 1 else 0
            o[j] = o[j] * (1.0 / o[j][one:one + 1])
            if j % 2 == 0:
                o[j] = pltpu.roll(o[j], HT, 1)
        return jnp.concatenate([
            o[0][0:16], jnp.where(s8 < 2, o[0][16:24], o[1][0:8]),
            o[1][8:16], jnp.where(s8 < 4, o[1][16:24], o[2][0:8]),
            o[2][8:16], jnp.where(s8 < 6, o[2][16:24], o[3][0:8]),
            o[3][8:24]], axis=0), mx

    def corner_logits(i, mx):
        lane = _iota((HT, T), 1)
        mask = jnp.where(_iota((HT, T), 0) > (lane & (HT - 1)), NEG, 0.0)
        low = _iota((GR, T), 1) < HT
        q = query_tiles(i)
        rhs = as_weights([jnp.where(low, q[j], q[j + 1]) for j in range(0, GH, 2)])
        st = _dot(k_s[pl.ds(i * T + HT, HT), :][:, :KP], rhs)
        for j in range(0, GH, 2):
            sb = st[:, j // 2 * T:(j // 2 + 1) * T] + mask
            sb_s[i][j // 2][...] = sb
            mb = _rows_max(sb)
            for e in range(2):
                m = jnp.maximum(mx[j + e], jnp.where((_iota((8, T), 1) >= HT) == bool(e), mb, -jnp.inf))
                mx_s[i * GH + j + e] = jnp.broadcast_to(jnp.max(m, axis=0, keepdims=True), (8, T))

    def out_proj(s, g):
        a = _dot(wot_s[_ds(g * GR, GR, 8), :], ot_s[s].reshape(DP, L)[...])
        out_s[s][g] = (base_s[s][g] + a).astype(BF16)

    def step(s, g, buf, nbuf, extra=None, last=False):
        first = s == 0
        v_s, pq_s, pk_s = buf

        def mem_read():
            if first:
                return None
            row = _iota((GP, T), 0)
            col = _iota((GP, T), 1)
            row_head = jnp.where(row < GR, _head_of(row), row - GR)
            m_lhs = jnp.where((row_head == _head_of(col)) & (col < GR), m_s[g], 0.0)
            pq = jnp.concatenate([pq_s[...], jnp.zeros((T - GR, L), F32)], axis=0).astype(BF16)
            return _dot(m_lhs, pq)

        def mem_write():
            if s == NSEG - 1:
                return
            v1 = jnp.concatenate([v_s[...], jnp.ones((GP - GR, L), F32)], axis=0)
            upd = _dot(v1, pk_s[...])
            m_s[g] = upd if first else m_s[g] + upd

        def emit(i, a_dot, nd):
            gate = gate_s[g]
            og = (1.0 - gate) * a_dot
            if not first:
                inv_den = 1.0 / (nd[GR:GP, i * T:(i + 1) * T] + 1e-6)
                iv = [jnp.broadcast_to(inv_den[j:j + 1], (8, T)) for j in range(GH)]
                ivr = jnp.concatenate([
                    iv[0], iv[0], jnp.where(s8 < 2, iv[0], iv[1]),
                    iv[1], jnp.where(s8 < 4, iv[1], iv[2]),
                    iv[2], jnp.where(s8 < 6, iv[2], iv[3]),
                    iv[3], iv[3]], axis=0)
                og = gate * (nd[0:GR, i * T:(i + 1) * T] * ivr) + og
            og = jnp.concatenate([og, jnp.zeros((GP - GR, T), F32)], axis=0)
            ot_s[s][g, :, pl.ds(i * T, T)] = og.astype(BF16)

        nxt = s * NG + g + 1
        nd = None
        for ch in ORDER:
            if ch == "p" and not last:
                project(nxt // NG, nxt % NG, nbuf)
            if ch == "o" and not first:
                out_proj(s - 1, g)
            if ch == "m":
                nd = mem_read()
                mem_write()
            if ch == "f":
                for pair in ((3, 2), (1, 0)):
                    mxs = []
                    for i in pair:
                        a_dot, mx = attend(i, v_s, True, not last)
                        emit(i, a_dot, nd)
                        mxs.append(mx)
                    if not last:
                        for i, mx in zip(pair, mxs):
                            corner_logits(i, mx)
            if ch == "x" and extra is not None:
                extra()

    def route():
        r = _rnd(jnp.concatenate([r_s[s] for s in range(NSEG)], axis=1))
        tok = _iota((8, S), 1)
        r0 = jnp.max(r, axis=1, keepdims=True)
        i0 = jnp.min(jnp.where(r == r0, tok, S - 1), axis=1, keepdims=True)
        rest = jnp.where(tok == i0, -jnp.inf, r)
        r1 = jnp.max(rest, axis=1, keepdims=True)
        i1 = jnp.min(jnp.where((rest == r1) & (tok != i0), tok, S - 1), axis=1, keepdims=True)
        idx = (jnp.clip(jnp.max(i0), 0, S - 1), jnp.clip(jnp.max(i1), 0, S - 1))
        return idx, jax.nn.sigmoid(jnp.where(_iota((8, 1), 0) == 0, r0, r1))

    def ffn(idx, r_sel):
        xs = jnp.zeros((8, DP), F32)
        for c in range(2):
            tile = xn_s[idx[c] // L, :, _lane_tile((idx[c] % L) // T)]
            hot = ((_iota((8, T), 1) == idx[c] % T) & (_iota((8, T), 0) == c)).astype(F32)
            xs = xs + _dot_nt(hot, tile)
        xs = xs[:, :D]
        gt = _dot(xs, wg_s[...])
        up = _dot(xs, wu_s[...])
        h = gt * jax.nn.sigmoid(gt) * up
        y = _dot_nt(h, wd_s[...]) * r_sel
        y = jnp.concatenate([y, jnp.zeros((8, DP - D), F32)], axis=1)
        yt = jnp.concatenate([y, jnp.zeros((T - 8, DP), F32)], axis=0).T[:D]
        for c in range(2):
            y_s[c] = jnp.broadcast_to(yt[:, c:c + 1], (D, T)).reshape(NG, GR, T)

    def add_routed(s, idx):
        for c in range(2):
            @pl.when(idx[c] // L == s)
            def _():
                lanes = _lane_tile((idx[c] % L) // T)
                cur = out_s[s][:, :, lanes].astype(F32)
                hit = _iota((NG, GR, T), 2) == idx[c] % T
                out_s[s][:, :, lanes] = jnp.where(hit, cur + y_s[c], cur).astype(BF16)

    with jax.named_scope("pro"):
        for t in range(NT):
            x0_copy(t).wait()
            layer_norm(0, t)
        for i in range(3):
            wa_copy(i).wait()
            if i == 1:
                for e in range(3):
                    wb_copy(e).start()
                x_copy(1).start()
            for c in range(2):
                transpose_w(i, c, wa_s[i, :, pl.ds(c * T, T)])
    with jax.named_scope("pro2"):
        project(0, 0, buf_a)
        for i in range(NT):
            corner_logits(i, attend(i, None, False, True)[1])
        for i in range(3):
            wb_copy(i).wait()
        x_copy(1).wait()

    for s in range(NSEG):
        def body(p, c, s=s):
            if s == 0:
                @pl.when(p == 0)
                def _():
                    wo_copy().start()
                    x_copy(2).start()
                    x_copy(3).start()
                    for i in range(3):
                        f_copy(i).start()

            def more_weights():
                c = jnp.minimum(p, 2)
                for i in range(3):
                    transpose_w(i, c + 2, wb_s[i, :, _lane_tile(c)])

            step(s, 2 * p, buf_a, buf_b, (lambda: layer_norm(s + 1, p)) if s < NSEG - 1 else None)
            step(s, 2 * p + 1, buf_b, buf_a, more_weights if s == 0 else None)
            return c
        with jax.named_scope(f"seg{s}"):
            if s < NSEG - 1:
                lax.fori_loop(0, NG // 2, body, 0)
            else:
                lax.fori_loop(0, NG // 2 - 1, body, 0)
                o_copy(0).wait()
                o_copy(1).wait()
                step(s, NG - 2, buf_a, buf_b)
                step(s, NG - 1, buf_b, buf_a, last=True)
        if s == 0:
            with jax.named_scope("wo"):
                wo_copy().wait()
                x_copy(2).wait()
                x_copy(3).wait()
                transpose_wo()
        if s == 2:
            with jax.named_scope("ffn"):
                for i in range(3):
                    f_copy(i).wait()
                idx, r_sel = route()
                ffn(idx, r_sel)
            for e in range(2):
                add_routed(e, idx)
                o_copy(e).start()

    add_routed(NSEG - 2, idx)
    o_copy(NSEG - 2).start()
    with jax.named_scope("oproj"):
        s = NSEG - 1
        for t in range(NT):
            lanes = pl.ds(t * T, T)
            a = _dot(wot_s[...], ot_s[s].reshape(DP, L)[:, lanes]).reshape(NG, GR, T)
            tok = _iota((NG, GR, T), 2) + (s * L + t * T)
            upd = jnp.where(tok == idx[0], y_s[0], jnp.where(tok == idx[1], y_s[1], 0.0))
            out_s[s][:, :, lanes] = (base_s[s][:, :, lanes] + a + upd).astype(BF16)
            o_last_copy(t).start()
    with jax.named_scope("fin"):
        o_copy(NSEG - 2).wait()
        for t in range(NT):
            o_last_copy(t).wait()


@jax.jit
def pallas_parallel_sum__memory_aug_infini_attn__moe_arch_mod__prompt_kernel(
    A_x, A_wq, A_wk, A_wv, A_wo, A_beta, B_x, B_w_r, B_w_gate, B_w_up, B_w_down,
):
    del B_x
    xt = jnp.transpose(A_x[0]).reshape(NG, GR, S)
    wdt = jnp.transpose(B_w_down)
    hbm = pl.BlockSpec(memory_space=pltpu.HBM)
    vmem = pl.BlockSpec(memory_space=pltpu.VMEM)
    carry = (pltpu.VMEM((GR, L), F32), pltpu.VMEM((GR, L), F32), pltpu.VMEM((L, T), BF16))
    out = pl.pallas_call(
        _kernel,
        out_shape=jax.ShapeDtypeStruct((NG, GR, S), BF16),
        in_specs=[hbm, hbm, hbm, hbm, hbm, vmem, vmem, hbm, hbm, hbm],
        out_specs=hbm,
        scratch_shapes=[
            pltpu.VMEM((NSEG, NG, GR, L), BF16),
            pltpu.VMEM((3, D, 2 * T), BF16),
            pltpu.VMEM((3, D, D - 2 * T), BF16),
            pltpu.VMEM((D, D), BF16),
            pltpu.VMEM((D, F), BF16),
            pltpu.VMEM((D, F), BF16),
            pltpu.VMEM((D, F), BF16),
            pltpu.VMEM((NSEG, DP, L), BF16),
            [pltpu.VMEM((NG, GR, L), F32)] * NSEG,
            pltpu.VMEM((3, DP, DP), F32),
            pltpu.VMEM((D, DP), F32),
            pltpu.VMEM((8, DP), F32),
            pltpu.VMEM((NG, GR, T), F32),
            pltpu.VMEM((NG, GP, T), F32),
            [pltpu.VMEM((NG, GP, L), BF16)] * NSEG,
            [pltpu.VMEM((NG, GR, L), BF16)] * NSEG,
            pltpu.VMEM((NSEG, 8, L), F32),
            pltpu.VMEM((2, NG, GR, T), F32),
            pltpu.VMEM((GR, L), F32),
            pltpu.VMEM((L, T), BF16),
            carry, carry,
            [[pltpu.VMEM((i * T + HT, T), F32)] * GH for i in range(NT)],
            [[pltpu.VMEM((HT, T), F32)] * (GH // 2)] * NT,
            pltpu.VMEM((NT * GH, 8, T), F32),
            pltpu.SemaphoreType.DMA((24,)),
        ],
        compiler_params=pltpu.CompilerParams(vmem_limit_bytes=100 * 1024 * 1024),
        name="infini_mod",
    )(xt, A_wq, A_wk, A_wv, A_wo, A_beta, B_w_r, B_w_gate, B_w_up, wdt)
    return jnp.transpose(out.reshape(D, S))[None]
```

```python
import jax
import jax.numpy as jnp
import numpy as np
from jax import lax
import jax.experimental.pallas as pl
import jax.experimental.pallas.tpu as pltpu

D = 576
DP = 640
S = 2048
H = 32
DH = 18
NSEG = 4
L = 512
F = 4608
NG = 8
GH = 4
GR = 72
GP = 80
T = 128
HT = T // 2
NT = L // T

F32 = jnp.float32
BF16 = jnp.bfloat16
LOG2E = 1.4426950408889634
QSCALE = float(DH ** -0.5 * LOG2E)
EPS_BF16 = float(np.asarray(1e-5, dtype=jnp.bfloat16).astype(np.float32))
NEG = -1e30

ORDER = "mnapxowb"
WT = BF16
MT = BF16
KP = 128
CH = 8
PACE1 = False


def _rnd(x):
    return x.astype(BF16).astype(F32)


def _dot(a, b):
    return lax.dot_general(a, b, (((1,), (0,)), ((), ())), preferred_element_type=F32)


def _dot_nt(a, b):
    return lax.dot_general(a, b, (((1,), (1,)), ((), ())), preferred_element_type=F32)


def _phi(t):
    return jnp.where(t > 0, t + 1.0, jnp.exp(t))


def _iota(shape, axis):
    return lax.broadcasted_iota(jnp.int32, shape, axis)


def _head_of(i):
    return (i * 57) >> 10


def _ds(i, n, align):
    return pl.ds(i if isinstance(i, int) else pl.multiple_of(i, align), n)


def _lane_tile(t):
    return _ds(t * T, T, T)


def _rows_max(x):
    return jnp.max(x.reshape(x.shape[0] // 8, 8, T), axis=0)


def _exp2_shifted(x, m):
    return jnp.exp2(x.reshape(x.shape[0] // 8, 8, T) - m[None]).reshape(x.shape)


def _pad_groups(x, axis):
    zeros = jnp.zeros_like(lax.slice_in_dim(x, 0, GP - GR, axis=axis))
    parts = []
    for g in range(NG):
        parts += [lax.slice_in_dim(x, g * GR, (g + 1) * GR, axis=axis), zeros]
    return jnp.concatenate(parts, axis=axis)


def _kernel(x_hbm, wq_hbm, wk_hbm, wv_hbm, wo_hbm, beta_hbm, wr_hbm, wg_hbm, wu_hbm, wd_hbm,
            out_hbm,
            xbuf, w_s, beta_ref, wr_ref, wg_s, wu_s, wd_s, xn_s, base_s, wt_s, wr_s, gate_s, m_s,
            ot_s, out_s, r_s, y_s, bufs, v_keep, st_s, sb_s, mx_s, xsel_s, h_s, yacc_s, stat_s, zero_s, x_sems, w_sems, sems):
    w_hbm = (wq_hbm, wk_hbm, wv_hbm)

    def x_copy(t0, n):
        return pltpu.make_async_copy(x_hbm.at[:, :, pl.ds(t0 * T, n * T)],
                                     xbuf.at[t0 // NT, :, :, pl.ds(t0 % NT * T, n * T)], x_sems.at[t0])

    def w_copy(i, c):
        cols = pl.ds(0, 2 * T) if c == 0 else pl.ds((c + 1) * T, min(T, D - (c + 1) * T))
        return pltpu.make_async_copy(w_hbm[i].at[:, cols], w_s.at[i, :, cols], w_sems.at[4 * i + c])

    def wo_copy():
        return pltpu.make_async_copy(wo_hbm, w_s.at[3], sems.at[0])

    def f_copy(i):
        return pltpu.make_async_copy((wg_hbm, wu_hbm, wd_hbm)[i], (wg_s, wu_s, wd_s)[i], sems.at[1 + i])

    def o_copy(s):
        return pltpu.make_async_copy(out_s[s], out_hbm.at[:, :, pl.ds(s * L, L)], sems.at[4 + s])

    def o_last_copy(t):
        return pltpu.make_async_copy(out_s[NSEG - 1].at[:, :, pl.ds(t * T, T)],
                                     out_hbm.at[:, :, pl.ds((NSEG - 1) * L + t * T, T)], sems.at[7 + t])

    wr_copy = pltpu.make_async_copy(wr_hbm, wr_ref, sems.at[11])
    beta_copy = pltpu.make_async_copy(beta_hbm, beta_ref, sems.at[12])

    def make_gate():
        g_row = jax.nn.sigmoid(beta_ref[...].astype(F32)).reshape(1, H)
        for g in range(NG):
            head = _head_of(_iota((GR, H), 0)) + g * GH
            col = jnp.sum(jnp.where(head == _iota((GR, H), 1), g_row, 0.0), axis=1, keepdims=True)
            gate_s[g] = jnp.broadcast_to(col, (GR, T))

    def make_router():
        row = jnp.broadcast_to(wr_ref[...].astype(F32).reshape(1, D), (8, D))
        wr_s[...] = _pad_groups(row, 1)

    def layer_norm(n, score=True, paced=True):
        s, lanes = n // NT, _lane_tile(n % NT)
        def x(g):
            return xbuf[s, g, :, lanes].astype(F32).reshape(GR // 8, 8, T)

        def mean_of(f):
            acc = f(x(0))
            for g in range(1, NG):
                acc = acc + f(x(g))
            acc = acc[0:3] + acc[3:6] + acc[6:9]
            tot = jnp.sum(acc[0] + acc[1] + acc[2], axis=0, keepdims=True)
            return jnp.broadcast_to(tot / D, (8, T))

        if paced:
            xf = xbuf[s, :, :, lanes].astype(F32).reshape(D, T)
            mean = jnp.sum(xf, axis=0, keepdims=True) / D
            cen = xf - mean
            var = jnp.sum(cen * cen, axis=0, keepdims=True) / D
            mb = jnp.broadcast_to(_rnd(mean), (8, T))
            inv = jnp.broadcast_to(1.0 / _rnd(jnp.sqrt(_rnd(_rnd(var) + EPS_BF16))), (8, T))
            never = _iota((8, T), 0) < zero_s[0]
            ys = []
            for c in range(0, D, 8):
                ys.append(_rnd(_rnd(xf[c:c + 8] - mb) * inv))
                mb = jnp.where(never, ys[-1], mb)
            xn = jnp.concatenate(ys, axis=0)
            base_s[s, :, :, lanes] = (xf + xn).reshape(NG, GR, T)
            xn_s[s, :, lanes] = _pad_groups(xn, 0).astype(BF16)
        else:
            stat_s[0] = mean = mean_of(lambda v: v)
            stat_s[1] = var = mean_of(lambda v: (v - mean[None]) * (v - mean[None]))
            mb = _rnd(mean)
            inv = 1.0 / _rnd(jnp.sqrt(_rnd(_rnd(var) + EPS_BF16)))
            for g in range(NG):
                xg = x(g)
                xn = _rnd(_rnd(xg - mb[None]) * inv[None]).reshape(GR, T)
                base_s[s, g, :, lanes] = xg.reshape(GR, T) + xn
                xn = jnp.concatenate([xn, jnp.zeros((GP - GR, T), F32)], axis=0)
                xn_s[s, pl.ds(g * GP, GP), lanes] = xn.astype(BF16)
        if score:
            r_s[s, :, lanes] = _dot(wr_s[...], xn_s[s, :, lanes])

    def transpose_w(i, c):
        parts = []
        for g in range(NG):
            parts += [w_s[i, pl.ds(g * GR, GR), _lane_tile(c)], jnp.zeros((GP - GR, T), BF16)]
        wt_s[i, _lane_tile(c), :] = jnp.concatenate(parts, axis=0).T

    s8 = _iota((8, T), 0)

    def wide_dot(i, p, rhs, fill):
        rows = _ds(p * 2 * GR, 2 * GR, 16)
        if not fill:
            return _dot(wt_s[i, rows, :], rhs(slice(None), slice(None)))
        rest = _dot(wt_s[i, rows, pl.ds(4 * T, T)], rhs(pl.ds(4 * T, T), slice(None)))
        fill.pop(0)()
        parts = []
        for t in range(NT):
            parts.append(_dot(wt_s[i, rows, pl.ds(0, 4 * T)], rhs(pl.ds(0, 4 * T), pl.ds(t * T, T))))
            if fill:
                fill.pop(0)()
        return jnp.concatenate(parts, axis=1) + rest

    def project(s, p, fill=None):
        if fill:
            qkvt = jnp.concatenate([wide_dot(i, p, lambda r, c: xn_s[s, r, c], fill) for i in range(3)], axis=0)
        else:
            rows = _ds(p * 2 * GR, 2 * GR, 16)
            qkvt = _dot(jnp.concatenate([wt_s[i, rows, :] for i in range(3)], axis=0), xn_s[s])
        keep_projection(qkvt)

    def keep_projection(qkvt):
        for e, (q_s, k_s, v_s, pq_s, pk_s) in enumerate(bufs):
            qt, kt, vt = (qkvt[(2 * i + e) * GR:(2 * i + e + 1) * GR] for i in range(3))
            q_s[...] = qt * QSCALE
            kn = jnp.concatenate([kt, jnp.zeros((T - GR, L), F32)], axis=0).T
            k_s[...] = kn.astype(k_s.dtype)
            pq_s[...] = _phi(qt)
            pk_s[...] = _phi(kn).astype(pk_s.dtype)
            v_s[...] = vt

    def query_tiles(i, q_s):
        qp = q_s[:, pl.ds(i * T, T)]
        qr = pltpu.roll(qp, HT, 1)
        row = _iota((GR, T), 0)
        return [jnp.where((row >= DH * j) & (row < DH * (j + 1)), qp if j % 2 else qr, 0.0) for j in range(GH)]

    def as_weights(tiles):
        pad = jnp.zeros((KP - GR, T), F32)
        return jnp.concatenate([jnp.concatenate([q, pad], axis=0).astype(BF16) for q in tiles], axis=1)

    def attend(i, v_s, qk):
        consume, produce = v_s is not None, qk is not None
        lane = _iota((HT, T), 1)
        tri = _iota((HT, T), 0) > (lane & (HT - 1))
        masks = [jnp.where(tri & (lane >= HT), NEG, 0.0), jnp.where(tri & (lane < HT), NEG, 0.0)]
        rhs = as_weights(query_tiles(i, qk[0])) if produce else None
        m_old = [mx_s[i * GH + j] for j in range(GH)] if consume else None
        o = [None] * GH
        mx = [None] * GH

        def weighted_sum(kb, ps):
            keys = pl.ds(kb * T, T)
            for j in range(GH):
                if j < GH - 1:
                    vw = jnp.concatenate([v_s[pl.ds(16 * j, 16), keys],
                                          jnp.where(s8 == 7, 1.0, v_s[pl.ds(16 * j + 16, 8), keys])], axis=0)
                else:
                    vw = jnp.concatenate([jnp.where(s8 == 0, 1.0, v_s[pl.ds(48, 8), keys]),
                                          v_s[pl.ds(56, 16), keys]], axis=0)
                oj = _dot(vw, ps[j])
                o[j] = oj if o[j] is None else o[j] + oj

        def full_probs(kb):
            keys = pl.ds(kb * T, T)
            return [_exp2_shifted(st_s[i][j][keys, :], m_old[j]).astype(BF16) for j in range(GH)]

        def diag_probs():
            ps = []
            for j in range(GH):
                if j % 2 == 0:
                    mb = jnp.where(_iota((8, T), 1) < HT, m_old[j], m_old[j + 1])
                    pb = _exp2_shifted(sb_s[i][j // 2][...], mb)
                head = _exp2_shifted(st_s[i][j][pl.ds(i * T, HT), :], m_old[j])
                tail = jnp.where(lane >= HT if j % 2 else lane < HT, pb, 0.0)
                ps.append(jnp.concatenate([head, tail], axis=0).astype(BF16))
            return ps

        def logits(k0, n):
            st = _dot(qk[1][pl.ds(k0, n), :][:, :KP], rhs)
            for j in range(GH):
                sj = st[:, j * T:(j + 1) * T]
                if k0 + n > i * T:
                    tail = sj[n - HT:] + masks[j % 2]
                    sj = tail if n == HT else jnp.concatenate([sj[:n - HT], tail], axis=0)
                st_s[i][j][pl.ds(k0, n), :] = sj
                m = _rows_max(sj)
                mx[j] = m if mx[j] is None else jnp.maximum(mx[j], m)

        pd = diag_probs() if consume else None
        for kb in range(max(i, 1)):
            ps = full_probs(kb) if consume and kb < i else None
            if produce:
                logits(kb * T, T if kb < i - 1 else i * T + HT - kb * T)
            if ps is not None:
                weighted_sum(kb, ps)
        if not consume:
            return None, mx
        weighted_sum(i, pd)
        for j in range(GH):
            one = 23 if j < GH - 1 else 0
            o[j] = o[j] * (1.0 / o[j][one:one + 1])
            if j % 2 == 0:
                o[j] = pltpu.roll(o[j], HT, 1)
        return jnp.concatenate([
            o[0][0:16], jnp.where(s8 < 2, o[0][16:24], o[1][0:8]),
            o[1][8:16], jnp.where(s8 < 4, o[1][16:24], o[2][0:8]),
            o[2][8:16], jnp.where(s8 < 6, o[2][16:24], o[3][0:8]),
            o[3][8:24]], axis=0), mx

    def corner_logits(i, mx, qk):
        lane = _iota((HT, T), 1)
        mask = jnp.where(_iota((HT, T), 0) > (lane & (HT - 1)), NEG, 0.0)
        low = _iota((GR, T), 1) < HT
        q = query_tiles(i, qk[0])
        rhs = as_weights([jnp.where(low, q[j], q[j + 1]) for j in range(0, GH, 2)])
        st = _dot(qk[1][pl.ds(i * T + HT, HT), :][:, :KP], rhs)
        for j in range(0, GH, 2):
            sb = st[:, j // 2 * T:(j // 2 + 1) * T] + mask
            sb_s[i][j // 2][...] = sb
            mb = _rows_max(sb)
            for e in range(2):
                m = jnp.maximum(mx[j + e], jnp.where((_iota((8, T), 1) >= HT) == bool(e), mb, -jnp.inf))
                mx_s[i * GH + j + e] = jnp.broadcast_to(jnp.max(m, axis=0, keepdims=True), (8, T))

    def out_proj(s, p, fill=None):
        a = wide_dot(3, p, lambda r, c: ot_s[s].reshape(DP, L)[r, c], fill)
        for e in range(2):
            out_s[s][2 * p + e] = (base_s[s, 2 * p + e] + a[e * GR:(e + 1) * GR]).astype(BF16)

    def memory(s, g, buf):
        _, _, v_s, pq_s, pk_s = buf
        nd = None
        if s > 0:
            row = _iota((GP, T), 0)
            col = _iota((GP, T), 1)
            row_head = jnp.where(row < GR, _head_of(row), row - GR)
            m_lhs = jnp.where((row_head == _head_of(col)) & (col < GR), m_s[g], 0.0)
            pq = jnp.concatenate([pq_s[...], jnp.zeros((T - GR, L), F32)], axis=0).astype(BF16)
            nd = _dot(m_lhs.astype(MT), pq)
        if s < NSEG - 1:
            v1 = jnp.concatenate([v_s[...], jnp.ones((GP - GR, L), F32)], axis=0)
            upd = _dot(v1.astype(MT), pk_s[...])
            m_s[g] = m_s[g] + upd if s > 0 else upd
        return nd

    def attention(s, g, nd, v_s, qk):
        gate = gate_s[g]
        for pair in ((3, 2), (1, 0)):
            mxs = []
            for i in pair:
                a_dot, mx = attend(i, v_s, qk)
                mxs.append(mx)
                og = (1.0 - gate) * a_dot
                if nd is not None:
                    inv_den = 1.0 / (nd[GR:GP, i * T:(i + 1) * T] + 1e-6)
                    iv = [jnp.broadcast_to(inv_den[j:j + 1], (8, T)) for j in range(GH)]
                    ivr = jnp.concatenate([
                        iv[0], iv[0], jnp.where(s8 < 2, iv[0], iv[1]),
                        iv[1], jnp.where(s8 < 4, iv[1], iv[2]),
                        iv[2], jnp.where(s8 < 6, iv[2], iv[3]),
                        iv[3], iv[3]], axis=0)
                    og = gate * (nd[0:GR, i * T:(i + 1) * T] * ivr) + og
                og = jnp.concatenate([og, jnp.zeros((GP - GR, T), F32)], axis=0)
                ot_s[s][g, :, pl.ds(i * T, T)] = og.astype(BF16)
            if qk is not None:
                for i, mx in zip(pair, mxs):
                    corner_logits(i, mx, qk)

    def pair_step(s, p, last=False):
        nxt = s * (NG // 2) + p + 1
        nd = [None, None]
        fill = gate_up(p) if s == NSEG - 2 else down(p) if s == NSEG - 1 and not last else None
        for ch in ORDER:
            if ch == "x":
                if s < 2:
                    layer_norm(2 * NT + s * NT + p)
            if ch == "w":
                if s == 0:
                    for e in range(3):
                        transpose_w(jnp.where(p < 2, e, 3),
                                    jnp.where(p < 2, p + 3, jnp.minimum(3 * (p - 2) + e, 4)))
            if ch == "m":
                nd[0] = memory(s, 2 * p, bufs[0])
            if ch == "n":
                nd[1] = memory(s, 2 * p + 1, bufs[1])
                v_keep[...] = bufs[1][2][...]
            if ch == "a":
                attention(s, 2 * p, nd[0], bufs[0][2], bufs[1])
            if ch == "p" and not last:
                project(nxt // (NG // 2), nxt % (NG // 2), fill)
            if ch == "o" and s > 0:
                out_proj(s - 1, p, fill)
            if ch == "b":
                attention(s, 2 * p + 1, nd[1], v_keep, None if last else bufs[0])

    def route():
        r = _rnd(jnp.concatenate([r_s[s] for s in range(NSEG)], axis=1))
        tok = _iota((8, S), 1)
        r0 = jnp.max(r, axis=1, keepdims=True)
        i0 = jnp.min(jnp.where(r == r0, tok, S - 1), axis=1, keepdims=True)
        rest = jnp.where(tok == i0, -jnp.inf, r)
        r1 = jnp.max(rest, axis=1, keepdims=True)
        i1 = jnp.min(jnp.where((rest == r1) & (tok != i0), tok, S - 1), axis=1, keepdims=True)
        idx = (jnp.clip(jnp.max(i0), 0, S - 1), jnp.clip(jnp.max(i1), 0, S - 1))
        return idx, jax.nn.sigmoid(jnp.where(_iota((8, 1), 0) == 0, r0, r1))

    def gather(idx):
        xs = jnp.zeros((8, DP), F32)
        for c in range(2):
            tile = xn_s[idx[c] // L, :, _lane_tile((idx[c] % L) // T)]
            hot = ((_iota((8, T), 1) == idx[c] % T) & (_iota((8, T), 0) == c)).astype(F32)
            xs = xs + _dot_nt(hot, tile)
        xsel_s[...] = jnp.concatenate([xs[:, g * GP:g * GP + GR] for g in range(NG)], axis=1)
        yacc_s[...] = jnp.zeros((8, DP), F32)

    FA = F // T // (NG // 2)
    FB = F // T // (NG // 2 - 1)

    def gate_up(p):
        pre = {}

        def remainder(m):
            w = (wg_s, wu_s)[m]
            pre[m] = _dot(xsel_s[:, pl.ds(4 * T, D - 4 * T)], w[pl.ds(4 * T, D - 4 * T), _ds(p * FA * T, FA * T, T)])

        def main(t, m):
            w = (wg_s, wu_s)[m]
            acc = _dot(xsel_s[:, pl.ds(0, 4 * T)], w[pl.ds(0, 4 * T), _lane_tile(p * FA + t)])
            pre[m, t] = acc + pre[m][:, t * T:(t + 1) * T]
            if m == 1:
                h_s[:, _lane_tile(p * FA + t)] = pre[0, t] * jax.nn.sigmoid(pre[0, t]) * pre[1, t]

        jobs = [lambda m=m: remainder(m) for m in range(2)]
        return jobs + [lambda t=t, m=m: main(t, m) for t in range(FA) for m in range(2)]

    def down(p):
        def piece(c, d):
            n = min(T, D - d * T)
            cols = _ds((p * FB + 4 * c) * T, 4 * T, T)
            yacc_s[:, pl.ds(d * T, n)] += _dot_nt(h_s[:, cols], wd_s[pl.ds(d * T, n), cols])
        return [lambda c=c, d=d: piece(c, d) for c in range(FB // 4) for d in range(DP // T)]

    def spread_routed(r_sel):
        y = yacc_s[...] * r_sel
        yt = jnp.concatenate([y, jnp.zeros((T - 8, DP), F32)], axis=0).T[:D]
        for c in range(2):
            y_s[c] = jnp.broadcast_to(yt[:, c:c + 1], (D, T)).reshape(NG, GR, T)

    def add_routed(s, idx):
        for c in range(2):
            @pl.when(idx[c] // L == s)
            def _():
                lanes = _lane_tile((idx[c] % L) // T)
                cur = out_s[s][:, :, lanes].astype(F32)
                hit = _iota((NG, GR, T), 2) == idx[c] % T
                out_s[s][:, :, lanes] = jnp.where(hit, cur + y_s[c], cur).astype(BF16)

    with jax.named_scope("pro"):
        zero_s[0] = 0
        for t in range(NT):
            x_copy(t, 1).start()
        for t in range(NT):
            x_copy(t, 1).wait()
            if t < 3:
                w_copy((1, 0, 2)[t], 0).start()
            if t == 2:
                wr_copy.start()
                beta_copy.start()
            if t == NT - 1:
                x_copy(NT, NT).start()
            layer_norm(t, score=False, paced=False)
    with jax.named_scope("pro2"):
        def first_dot(i):
            return _dot(wt_s[i, pl.ds(0, 2 * GR), :], xn_s[0])
        w_copy(1, 0).wait()
        w_copy(0, 0).wait()
        for i in range(3):
            w_copy(i, 1).start()
        for c in range(2):
            transpose_w(1, c)
        kt = first_dot(1)
        for c in range(2):
            transpose_w(0, c)
        w_copy(2, 0).wait()
        wr_copy.wait()
        beta_copy.wait()
        x_copy(2 * NT, 1).start()
        for i in range(3):
            w_copy(i, 2).start()
        qt = first_dot(0)
        for c in range(2):
            transpose_w(2, c)
        make_gate()
        make_router()
        keep_projection(jnp.concatenate([qt, kt, first_dot(2)], axis=0))
    with jax.named_scope("pro3"):
        x_copy(NT, NT).wait()
        for i in range(3):
            w_copy(i, 1).wait()
        for i in range(3):
            w_copy(i, 3).start()
        x_copy(2 * NT + 1, NT - 1).start()
        r_s[0] = _dot(wr_s[...], xn_s[0])
        for i in range(3):
            transpose_w(i, 2)
        for i in range(NT):
            corner_logits(i, attend(i, None, bufs[0])[1], bufs[0])
        for t in range(NT):
            layer_norm(NT + t, score=False, paced=PACE1)
        r_s[1] = _dot(wr_s[...], xn_s[1])
        x_copy(2 * NT, 1).wait()
        for i in range(3):
            w_copy(i, 2).wait()

    for s in range(NSEG):
        def body(p, c, s=s):
            if s == 0:
                @pl.when(p == 0)
                def _():
                    wo_copy().start()
                    x_copy(3 * NT, NT).start()

                @pl.when(p == 1)
                def _():
                    for i in range(3):
                        w_copy(i, 3).wait()
                    x_copy(2 * NT + 1, NT - 1).wait()
                    wo_copy().wait()
                    x_copy(3 * NT, NT).wait()
                    for i in range(3):
                        f_copy(i).start()
            pair_step(s, p)
            return c
        with jax.named_scope(f"seg{s}"):
            if s < NSEG - 1:
                lax.fori_loop(0, NG // 2, body, 0)
            else:
                lax.fori_loop(0, NG // 2 - 1, body, 0)
                spread_routed(r_sel)
                for e in range(2):
                    add_routed(e, idx)
                    o_copy(e).start()
                pair_step(s, NG // 2 - 1, last=True)
        if s == 1:
            with jax.named_scope("ffn"):
                for i in range(3):
                    f_copy(i).wait()
                idx, r_sel = route()
                gather(idx)

    add_routed(NSEG - 2, idx)
    o_copy(NSEG - 2).start()
    with jax.named_scope("oproj"):
        s = NSEG - 1
        for t in range(NT):
            lanes = pl.ds(t * T, T)
            a = _dot(wt_s[3, pl.ds(0, D), :], ot_s[s].reshape(DP, L)[:, lanes]).reshape(NG, GR, T)
            tok = _iota((NG, GR, T), 2) + (s * L + t * T)
            upd = jnp.where(tok == idx[0], y_s[0], jnp.where(tok == idx[1], y_s[1], 0.0))
            out_s[s][:, :, lanes] = (base_s[s, :, :, lanes] + a + upd).astype(BF16)
            o_last_copy(t).start()
    with jax.named_scope("fin"):
        for s in range(NSEG - 1):
            o_copy(s).wait()
        for t in range(NT):
            o_last_copy(t).wait()


@jax.jit
def pallas_parallel_sum__memory_aug_infini_attn__moe_arch_mod__prompt_kernel(
    A_x, A_wq, A_wk, A_wv, A_wo, A_beta, B_x, B_w_r, B_w_gate, B_w_up, B_w_down,
):
    del B_x
    xt = jnp.transpose(A_x[0]).reshape(NG, GR, S)
    wdt = jnp.transpose(B_w_down)
    hbm = pl.BlockSpec(memory_space=pltpu.HBM)
    carry = (pltpu.VMEM((GR, L), F32), pltpu.VMEM((L, T), BF16), pltpu.VMEM((GR, L), F32),
             pltpu.VMEM((GR, L), F32), pltpu.VMEM((L, T), BF16))
    out = pl.pallas_call(
        _kernel,
        out_shape=jax.ShapeDtypeStruct((NG, GR, S), BF16),
        in_specs=[hbm] * 10,
        out_specs=hbm,
        scratch_shapes=[
            pltpu.VMEM((NSEG, NG, GR, L), BF16),
            pltpu.VMEM((4, D, D), BF16),
            pltpu.VMEM((H,), BF16),
            pltpu.VMEM((D,), BF16),
            pltpu.VMEM((D, F), BF16),
            pltpu.VMEM((D, F), BF16),
            pltpu.VMEM((D, F), BF16),
            pltpu.VMEM((NSEG, DP, L), BF16),
            pltpu.VMEM((NSEG, NG, GR, L), F32),
            pltpu.VMEM((4, DP, DP), WT),
            pltpu.VMEM((8, DP), F32),
            pltpu.VMEM((NG, GR, T), F32),
            pltpu.VMEM((NG, GP, T), F32),
            [pltpu.VMEM((NG, GP, L), BF16)] * NSEG,
            [pltpu.VMEM((NG, GR, L), BF16)] * NSEG,
            pltpu.VMEM((NSEG, 8, L), F32),
            pltpu.VMEM((2, NG, GR, T), F32),
            (carry, carry),
            pltpu.VMEM((GR, L), F32),
            [[pltpu.VMEM((i * T + HT, T), F32)] * GH for i in range(NT)],
            [[pltpu.VMEM((HT, T), F32)] * (GH // 2)] * NT,
            pltpu.VMEM((NT * GH, 8, T), F32),
            pltpu.VMEM((8, D), F32),
            pltpu.VMEM((8, F), F32),
            pltpu.VMEM((8, DP), F32),
            pltpu.VMEM((2, 8, T), F32),
            pltpu.SMEM((1,), jnp.int32),
            pltpu.SemaphoreType.DMA((NSEG * NT,)),
            pltpu.SemaphoreType.DMA((12,)),
            pltpu.SemaphoreType.DMA((13,)),
        ],
        compiler_params=pltpu.CompilerParams(vmem_limit_bytes=100 * 1024 * 1024),
        name="infini_mod",
    )(xt, A_wq, A_wk, A_wv, A_wo, A_beta, B_w_r, B_w_gate, B_w_up, wdt)
    return jnp.transpose(out.reshape(D, S))[None]
```

```python
import jax
import jax.numpy as jnp
import numpy as np
from jax import lax
import jax.experimental.pallas as pl
import jax.experimental.pallas.tpu as pltpu

D = 576
DP = 640
S = 2048
H = 32
DH = 18
NSEG = 4
L = 512
F = 4608
NG = 8
GH = 4
GR = 72
GP = 80
T = 128
HT = T // 2
NT = L // T

F32 = jnp.float32
BF16 = jnp.bfloat16
LOG2E = 1.4426950408889634
QSCALE = float(DH ** -0.5 * LOG2E)
EPS_BF16 = float(np.asarray(1e-5, dtype=jnp.bfloat16).astype(np.float32))
NEG = -1e30
F32_TINY = float(np.finfo(np.float32).tiny)
BF16_MAX = float(jnp.finfo(jnp.bfloat16).max)

ORDER = "mnapxowb"
WT = BF16
MT = BF16
KP = 128
CH = 8
PACE1 = False
PACE2 = False
NA = 4
SPLITP = False


def _rnd(x):
    return x.astype(BF16).astype(F32)


def _dot(a, b):
    return lax.dot_general(a, b, (((1,), (0,)), ((), ())), preferred_element_type=F32)


def _dot_nt(a, b):
    return lax.dot_general(a, b, (((1,), (1,)), ((), ())), preferred_element_type=F32)


def _phi(t):
    return jnp.where(t > 0, t + 1.0, jnp.exp(t))


def _iota(shape, axis):
    return lax.broadcasted_iota(jnp.int32, shape, axis)


def _head_of(i):
    return (i * 57) >> 10


def _ds(i, n, align):
    return pl.ds(i if isinstance(i, int) else pl.multiple_of(i, align), n)


def _lane_tile(t):
    return _ds(t * T, T, T)


def _rows_max(x):
    return jnp.max(x.reshape(x.shape[0] // 8, 8, T), axis=0)


def _exp2_shifted(x, m):
    return jnp.exp2(x.reshape(x.shape[0] // 8, 8, T) - m[None]).reshape(x.shape)


def _pad_groups(x, axis):
    zeros = jnp.zeros_like(lax.slice_in_dim(x, 0, GP - GR, axis=axis))
    parts = []
    for g in range(NG):
        parts += [lax.slice_in_dim(x, g * GR, (g + 1) * GR, axis=axis), zeros]
    return jnp.concatenate(parts, axis=axis)


def _kernel(x_hbm, wq_hbm, wk_hbm, wv_hbm, wo_hbm, beta_hbm, wr_hbm, wg_hbm, wu_hbm, wd_hbm,
            out_hbm,
            xbuf, w_s, beta_ref, wr_ref, wg_s, wu_s, wd_s, xn_s, base_s, wt_s, wr_s, gate_s, m_s,
            ot_s, out_s, r_s, y_s, bufs, v_keep, st_s, sb_s, mx_s, xsel_s, h_s, yacc_s, stat_s, zero_s, x_sems, w_sems, sems):
    w_hbm = (wq_hbm, wk_hbm, wv_hbm)

    def x_copy(t0, n):
        return pltpu.make_async_copy(x_hbm.at[:, :, pl.ds(t0 * T, n * T)],
                                     xbuf.at[t0 // NT, :, :, pl.ds(t0 % NT * T, n * T)], x_sems.at[t0])

    def w_copy(i, c):
        cols = pl.ds(0, 2 * T) if c == 0 else pl.ds((c + 1) * T, min(T, D - (c + 1) * T))
        return pltpu.make_async_copy(w_hbm[i].at[:, cols], w_s.at[i, :, cols], w_sems.at[4 * i + c])

    def wo_copy():
        return pltpu.make_async_copy(wo_hbm, w_s.at[3], sems.at[0])

    def f_copy(i):
        return pltpu.make_async_copy((wg_hbm, wu_hbm, wd_hbm)[i], (wg_s, wu_s, wd_s)[i], sems.at[1 + i])

    def o_copy(s):
        return pltpu.make_async_copy(out_s.at[s], out_hbm.at[:, :, pl.ds(s * L, L)], sems.at[4 + s])

    def tile_copy(n, sem):
        return pltpu.make_async_copy(out_s.at[n // NT, :, :, _lane_tile(n % NT)],
                                     out_hbm.at[:, :, _lane_tile(n)], sems.at[sem])

    wr_copy = pltpu.make_async_copy(wr_hbm, wr_ref, sems.at[11])
    beta_copy = pltpu.make_async_copy(beta_hbm, beta_ref, sems.at[12])

    def make_gate():
        g_row = jax.nn.sigmoid(beta_ref[...].astype(F32)).reshape(1, H)
        for g in range(NG):
            head = _head_of(_iota((GR, H), 0)) + g * GH
            col = jnp.sum(jnp.where(head == _iota((GR, H), 1), g_row, 0.0), axis=1, keepdims=True)
            gate_s[g] = jnp.broadcast_to(col, (GR, T))

    def make_router():
        row = jnp.broadcast_to(wr_ref[...].astype(F32).reshape(1, D), (8, D))
        wr_s[...] = _pad_groups(row, 1)

    def layer_norm(n, score=True, paced=True):
        s, lanes = n // NT, _lane_tile(n % NT)
        def x(g):
            return xbuf[s, g, :, lanes].astype(F32).reshape(GR // 8, 8, T)

        def mean_of(f):
            acc = f(x(0))
            for g in range(1, NG):
                acc = acc + f(x(g))
            acc = acc[0:3] + acc[3:6] + acc[6:9]
            tot = jnp.sum(acc[0] + acc[1] + acc[2], axis=0, keepdims=True)
            return jnp.broadcast_to(tot / D, (8, T))

        if paced:
            xf = xbuf[s, :, :, lanes].astype(F32).reshape(D, T)
            mean = jnp.sum(xf, axis=0, keepdims=True) / D
            cen = xf - mean
            var = jnp.sum(cen * cen, axis=0, keepdims=True) / D
            mb = jnp.broadcast_to(_rnd(mean), (8, T))
            inv = jnp.broadcast_to(1.0 / _rnd(jnp.sqrt(_rnd(_rnd(var) + EPS_BF16))), (8, T))
            never = _iota((8, T), 0) < zero_s[0]
            ys = []
            for c in range(0, D, 8):
                ys.append(_rnd(_rnd(xf[c:c + 8] - mb) * inv))
                mb = jnp.where(never, ys[-1], mb)
            xn = jnp.concatenate(ys, axis=0)
            base_s[s, :, :, lanes] = (xf + xn).reshape(NG, GR, T)
            xn_s[s, :, lanes] = _pad_groups(xn, 0).astype(BF16)
        else:
            stat_s[0] = mean = mean_of(lambda v: v)
            stat_s[1] = var = mean_of(lambda v: (v - mean[None]) * (v - mean[None]))
            mb = _rnd(mean)
            inv = 1.0 / _rnd(jnp.sqrt(_rnd(_rnd(var) + EPS_BF16)))
            for g in range(NG):
                xg = x(g)
                xn = _rnd(_rnd(xg - mb[None]) * inv[None]).reshape(GR, T)
                base_s[s, g, :, lanes] = xg.reshape(GR, T) + xn
                xn = jnp.concatenate([xn, jnp.zeros((GP - GR, T), F32)], axis=0)
                xn_s[s, pl.ds(g * GP, GP), lanes] = xn.astype(BF16)
        if score:
            r_s[s, :, lanes] = _dot(wr_s[...], xn_s[s, :, lanes])

    def transpose_w(i, c):
        parts = []
        for g in range(NG):
            parts += [w_s[i, pl.ds(g * GR, GR), _lane_tile(c)], jnp.zeros((GP - GR, T), BF16)]
        wt_s[i, _lane_tile(c), :] = jnp.concatenate(parts, axis=0).T

    s8 = _iota((8, T), 0)

    def wide_dot(i, p, rhs, fill):
        rows = _ds(p * 2 * GR, 2 * GR, 16)
        if not fill:
            return _dot(wt_s[i, rows, :], rhs(slice(None), slice(None)))
        rest = _dot(wt_s[i, rows, pl.ds(4 * T, T)], rhs(pl.ds(4 * T, T), slice(None)))
        fill.pop(0)()
        parts = []
        for t in range(NT):
            parts.append(_dot(wt_s[i, rows, pl.ds(0, 4 * T)], rhs(pl.ds(0, 4 * T), pl.ds(t * T, T))))
            if fill:
                fill.pop(0)()
        return jnp.concatenate(parts, axis=1) + rest

    def keep(i, val):
        for e, (q_s, k_s, v_s, pq_s, pk_s) in enumerate(bufs):
            part = val[e * GR:(e + 1) * GR]
            if i == 0:
                q_s[...] = part * QSCALE
                pq_s[...] = _phi(part)
            elif i == 1:
                kn = jnp.concatenate([part, jnp.zeros((T - GR, L), F32)], axis=0).T
                k_s[...] = kn.astype(BF16)
                pk_s[...] = _phi(kn).astype(BF16)
            else:
                v_s[...] = part

    def project(s, p, fill):
        if fill or SPLITP:
            for i in (1, 0, 2):
                keep(i, wide_dot(i, p, lambda r, c: xn_s[s, r, c], fill))
        else:
            rows = _ds(p * 2 * GR, 2 * GR, 16)
            qkvt = _dot(jnp.concatenate([wt_s[i, rows, :] for i in range(3)], axis=0), xn_s[s])
            for i in range(3):
                keep(i, qkvt[i * 2 * GR:(i + 1) * 2 * GR])

    def query_tiles(i, q_s):
        qp = q_s[:, pl.ds(i * T, T)]
        qr = pltpu.roll(qp, HT, 1)
        row = _iota((GR, T), 0)
        return [jnp.where((row >= DH * j) & (row < DH * (j + 1)), qp if j % 2 else qr, 0.0) for j in range(GH)]

    def as_weights(tiles):
        pad = jnp.zeros((KP - GR, T), F32)
        return jnp.concatenate([jnp.concatenate([q, pad], axis=0).astype(BF16) for q in tiles], axis=1)

    def attend(i, v_s, qk):
        consume, produce = v_s is not None, qk is not None
        lane = _iota((HT, T), 1)
        tri = _iota((HT, T), 0) > (lane & (HT - 1))
        masks = [jnp.where(tri & (lane >= HT), NEG, 0.0), jnp.where(tri & (lane < HT), NEG, 0.0)]
        rhs = as_weights(query_tiles(i, qk[0])) if produce else None
        m_old = [mx_s[i * GH + j] for j in range(GH)] if consume else None
        o = [None] * GH
        mx = [None] * GH

        def weighted_sum(kb, ps):
            keys = pl.ds(kb * T, T)
            for j in range(GH):
                if j < GH - 1:
                    vw = jnp.concatenate([v_s[pl.ds(16 * j, 16), keys],
                                          jnp.where(s8 == 7, 1.0, v_s[pl.ds(16 * j + 16, 8), keys])], axis=0)
                else:
                    vw = jnp.concatenate([jnp.where(s8 == 0, 1.0, v_s[pl.ds(48, 8), keys]),
                                          v_s[pl.ds(56, 16), keys]], axis=0)
                oj = _dot(vw, ps[j])
                o[j] = oj if o[j] is None else o[j] + oj

        def full_probs(kb):
            keys = pl.ds(kb * T, T)
            return [_exp2_shifted(st_s[i][j][keys, :], m_old[j]).astype(BF16) for j in range(GH)]

        def diag_probs():
            ps = []
            for j in range(GH):
                if j % 2 == 0:
                    mb = jnp.where(_iota((8, T), 1) < HT, m_old[j], m_old[j + 1])
                    pb = _exp2_shifted(sb_s[i][j // 2][...], mb)
                head = _exp2_shifted(st_s[i][j][pl.ds(i * T, HT), :], m_old[j])
                tail = jnp.where(lane >= HT if j % 2 else lane < HT, pb, 0.0)
                ps.append(jnp.concatenate([head, tail], axis=0).astype(BF16))
            return ps

        def logits(k0, n):
            st = _dot(qk[1][pl.ds(k0, n), :][:, :KP], rhs)
            for j in range(GH):
                sj = st[:, j * T:(j + 1) * T]
                if k0 + n > i * T:
                    tail = sj[n - HT:] + masks[j % 2]
                    sj = tail if n == HT else jnp.concatenate([sj[:n - HT], tail], axis=0)
                st_s[i][j][pl.ds(k0, n), :] = sj
                m = _rows_max(sj)
                mx[j] = m if mx[j] is None else jnp.maximum(mx[j], m)

        pd = diag_probs() if consume else None
        for kb in range(max(i, 1)):
            ps = full_probs(kb) if consume and kb < i else None
            if produce:
                logits(kb * T, T if kb < i - 1 else i * T + HT - kb * T)
            if ps is not None:
                weighted_sum(kb, ps)
        if not consume:
            return None, mx
        weighted_sum(i, pd)
        for j in range(GH):
            one = 23 if j < GH - 1 else 0
            o[j] = o[j] * (1.0 / o[j][one:one + 1])
            if j % 2 == 0:
                o[j] = pltpu.roll(o[j], HT, 1)
        return jnp.concatenate([
            o[0][0:16], jnp.where(s8 < 2, o[0][16:24], o[1][0:8]),
            o[1][8:16], jnp.where(s8 < 4, o[1][16:24], o[2][0:8]),
            o[2][8:16], jnp.where(s8 < 6, o[2][16:24], o[3][0:8]),
            o[3][8:24]], axis=0), mx

    def corner_logits(i, mx, qk):
        lane = _iota((HT, T), 1)
        mask = jnp.where(_iota((HT, T), 0) > (lane & (HT - 1)), NEG, 0.0)
        low = _iota((GR, T), 1) < HT
        q = query_tiles(i, qk[0])
        rhs = as_weights([jnp.where(low, q[j], q[j + 1]) for j in range(0, GH, 2)])
        st = _dot(qk[1][pl.ds(i * T + HT, HT), :][:, :KP], rhs)
        for j in range(0, GH, 2):
            sb = st[:, j // 2 * T:(j // 2 + 1) * T] + mask
            sb_s[i][j // 2][...] = sb
            mb = _rows_max(sb)
            for e in range(2):
                m = jnp.maximum(mx[j + e], jnp.where((_iota((8, T), 1) >= HT) == bool(e), mb, -jnp.inf))
                mx_s[i * GH + j + e] = jnp.broadcast_to(jnp.max(m, axis=0, keepdims=True), (8, T))

    def out_proj(s, p, fill=None):
        a = wide_dot(3, p, lambda r, c: ot_s[s].reshape(DP, L)[r, c], fill)
        for e in range(2):
            out_s[s, 2 * p + e] = (base_s[s, 2 * p + e] + a[e * GR:(e + 1) * GR]).astype(BF16)

    def memory(s, g, buf):
        _, _, v_s, pq_s, pk_s = buf
        nd = None
        if s > 0:
            row = _iota((GP, T), 0)
            col = _iota((GP, T), 1)
            row_head = jnp.where(row < GR, _head_of(row), row - GR)
            m_lhs = jnp.where((row_head == _head_of(col)) & (col < GR), m_s[g], 0.0)
            pq = jnp.concatenate([pq_s[...], jnp.zeros((T - GR, L), F32)], axis=0).astype(BF16)
            nd = _dot(m_lhs.astype(MT), pq)
        if s < NSEG - 1:
            v1 = jnp.concatenate([v_s[...], jnp.ones((GP - GR, L), F32)], axis=0)
            upd = _dot(v1.astype(MT), pk_s[...])
            m_s[g] = m_s[g] + upd if s > 0 else upd
        return nd

    def attend_tile(s, g, i, nd, v_s, qk):
        gate = gate_s[g]
        a_dot, mx = attend(i, v_s, qk)
        og = (1.0 - gate) * a_dot
        if nd is not None:
            inv_den = 1.0 / (nd[GR:GP, i * T:(i + 1) * T] + 1e-6)
            iv = [jnp.broadcast_to(inv_den[j:j + 1], (8, T)) for j in range(GH)]
            ivr = jnp.concatenate([
                iv[0], iv[0], jnp.where(s8 < 2, iv[0], iv[1]),
                iv[1], jnp.where(s8 < 4, iv[1], iv[2]),
                iv[2], jnp.where(s8 < 6, iv[2], iv[3]),
                iv[3], iv[3]], axis=0)
            og = gate * (nd[0:GR, i * T:(i + 1) * T] * ivr) + og
        og = jnp.concatenate([og, jnp.zeros((GP - GR, T), F32)], axis=0)
        ot_s[s][g, :, pl.ds(i * T, T)] = og.astype(BF16)
        return mx

    def attention(s, g, nd, v_s, qk):
        for pair in ((3, 2), (1, 0)):
            mxs = [attend_tile(s, g, i, nd, v_s, qk) for i in pair]
            for i, mx in zip(pair, mxs):
                corner_logits(i, mx, qk)

    def last_out_proj(t):
        s = NSEG - 1
        lanes = pl.ds(t * T, T)
        a = _dot(wt_s[3, pl.ds(0, D), :], ot_s[s].reshape(DP, L)[:, lanes]).reshape(NG, GR, T)
        out_s[s, :, :, lanes] = (base_s[s, :, :, lanes] + a).astype(BF16)
        tile_copy(s * NT + t, 7 + t).start()

    def pair_step(s, p, last=False):
        nxt = s * (NG // 2) + p + 1
        nd = [None, None]
        fill = gate_up(p) if s == NSEG - 2 else down(p) if s == NSEG - 1 and not last else None
        for ch in ORDER:
            if ch == "x":
                if s < 2:
                    layer_norm(2 * NT + s * NT + p)
            if ch == "w":
                if s == 0:
                    for e in range(3):
                        transpose_w(jnp.where(p < 2, e, 3),
                                    jnp.where(p < 2, p + 3, jnp.minimum(3 * (p - 2) + e, 4)))
            if ch == "m":
                nd[0] = memory(s, 2 * p, bufs[0])
            if ch == "n":
                nd[1] = memory(s, 2 * p + 1, bufs[1])
                v_keep[...] = bufs[1][2][...]
            if ch == "a":
                attention(s, 2 * p, nd[0], bufs[0][2], bufs[1])
            if ch == "p" and not last:
                project(nxt // (NG // 2), nxt % (NG // 2), fill)
            if ch == "o" and s > 0:
                out_proj(s - 1, p, fill)
            if ch == "b" and not last:
                attention(s, 2 * p + 1, nd[1], v_keep, bufs[0])
        return nd[1]

    def route():
        r = _rnd(jnp.concatenate([r_s[s] for s in range(NSEG)], axis=1))
        r = jnp.clip(jnp.where(jnp.abs(r) < F32_TINY, F32_TINY, r), -BF16_MAX, BF16_MAX)
        tok = _iota((8, S), 1)
        key = pltpu.bitcast(pltpu.bitcast(r, jnp.int32) | jnp.where(r > 0, S - 1 - tok, tok), F32)
        k0 = jnp.max(key, axis=1, keepdims=True)
        k1 = jnp.max(jnp.where(key == k0, -jnp.inf, key), axis=1, keepdims=True)
        top = jnp.broadcast_to(jnp.where(_iota((8, 1), 0) == 0, k0, k1), (8, T))
        bits = pltpu.bitcast(top, jnp.int32)
        pos = jnp.where(top > 0, S - 1 - (bits & (S - 1)), bits & (S - 1))
        return (pos[0, 0], pos[1, 0]), jax.nn.sigmoid(pltpu.bitcast(bits & -(1 << 16), F32))

    def gather(idx):
        xs = jnp.zeros((8, DP), F32)
        for c in range(2):
            tile = xn_s[idx[c] // L, :, _lane_tile((idx[c] % L) // T)]
            hot = ((_iota((8, T), 1) == idx[c] % T) & (_iota((8, T), 0) == c)).astype(F32)
            xs = xs + _dot_nt(hot, tile)
        xsel_s[...] = jnp.concatenate([xs[:, g * GP:g * GP + GR] for g in range(NG)], axis=1)
        yacc_s[...] = jnp.zeros((8, DP), F32)

    FA = F // T // (NG // 2)
    FB = F // T // (NG // 2 - 1)

    def gate_up(p):
        pre = {}

        def remainder(m):
            w = (wg_s, wu_s)[m]
            pre[m] = _dot(xsel_s[:, pl.ds(4 * T, D - 4 * T)], w[pl.ds(4 * T, D - 4 * T), _ds(p * FA * T, FA * T, T)])

        def main(t, m):
            w = (wg_s, wu_s)[m]
            acc = _dot(xsel_s[:, pl.ds(0, 4 * T)], w[pl.ds(0, 4 * T), _lane_tile(p * FA + t)])
            pre[m, t] = acc + pre[m][:, t * T:(t + 1) * T]
            if m == 1:
                h_s[:, _lane_tile(p * FA + t)] = pre[0, t] * jax.nn.sigmoid(pre[0, t]) * pre[1, t]

        jobs = [lambda m=m: remainder(m) for m in range(2)]
        return jobs + [lambda t=t, m=m: main(t, m) for t in range(FA) for m in range(2)]

    def down(p):
        def piece(c, d):
            n = min(T, D - d * T)
            cols = _ds((p * FB + 4 * c) * T, 4 * T, T)
            yacc_s[:, pl.ds(d * T, n)] += _dot_nt(h_s[:, cols], wd_s[pl.ds(d * T, n), cols])
        return [lambda c=c, d=d: piece(c, d) for c in range(FB // 4) for d in range(DP // T)]

    def routed_columns(idx, r_sel):
        y = yacc_s[...] * jnp.concatenate([r_sel] * (DP // T), axis=1)
        yt = jnp.concatenate([y, jnp.zeros((T - 8, DP), F32)], axis=0).T[:D]
        for c in range(2):
            upd = pltpu.roll(yt, (idx[c] + T - c) % T, 1)
            y_s[c] = jnp.where(_iota((D, T), 1) == idx[c] % T, upd, 0.0).reshape(NG, GR, T)

    def add_routed(idx):
        for c in range(2):
            s, lanes = idx[c] // L, _lane_tile((idx[c] % L) // T)

            @pl.when(s < NSEG - 1)
            def _():
                out_s[s, :, :, lanes] = (out_s[s, :, :, lanes].astype(F32) + y_s[c]).astype(BF16)

            @pl.when(s == NSEG - 1)
            def _():
                base_s[NSEG - 1, :, :, lanes] += y_s[c]

    with jax.named_scope("pro"):
        zero_s[0] = 0
        for t in range(NT):
            x_copy(t, 1).start()
        for t in range(NT):
            x_copy(t, 1).wait()
            if t < 3:
                w_copy((1, 0, 2)[t], 0).start()
            if t == 2:
                wr_copy.start()
                beta_copy.start()
            if t == NT - 1:
                x_copy(NT, NT).start()
            layer_norm(t, score=False, paced=False)
    with jax.named_scope("pro2"):
        def first_dot(i):
            return _dot(wt_s[i, pl.ds(0, 2 * GR), :], xn_s[0])
        w_copy(1, 0).wait()
        w_copy(0, 0).wait()
        for i in range(3):
            w_copy(i, 1).start()
        for c in range(2):
            transpose_w(1, c)
        kt = first_dot(1)
        for c in range(2):
            transpose_w(0, c)
        w_copy(2, 0).wait()
        wr_copy.wait()
        beta_copy.wait()
        x_copy(2 * NT, 1).start()
        for i in range(3):
            w_copy(i, 2).start()
        keep(1, kt)
        keep(0, first_dot(0))
        for c in range(2):
            transpose_w(2, c)
        make_gate()
        make_router()
    with jax.named_scope("pro3"):
        def first_logits(pair):
            mxs = [attend(i, None, bufs[0])[1] for i in pair]
            for i, mx in zip(pair, mxs):
                corner_logits(i, mx, bufs[0])
        x_copy(NT, NT).wait()
        keep(2, first_dot(2))
        r_s[0] = _dot(wr_s[...], xn_s[0])
        first_logits((3, 2))
        for t in range(NA):
            layer_norm(NT + t, score=False, paced=PACE1)
        for i in range(3):
            w_copy(i, 1).wait()
        for i in range(3):
            w_copy(i, 3).start()
        x_copy(2 * NT + 1, NT - 1).start()
        first_logits((1, 0))
        for i in range(3):
            transpose_w(i, 2)
        for t in range(NA, NT):
            layer_norm(NT + t, score=False, paced=PACE2)
        r_s[1] = _dot(wr_s[...], xn_s[1])
        x_copy(2 * NT, 1).wait()
        for i in range(3):
            w_copy(i, 2).wait()

    for s in range(NSEG):
        def body(p, c, s=s):
            if s == 0:
                @pl.when(p == 0)
                def _():
                    wo_copy().start()
                    x_copy(3 * NT, NT).start()

                @pl.when(p == 1)
                def _():
                    for i in range(3):
                        w_copy(i, 3).wait()
                    x_copy(2 * NT + 1, NT - 1).wait()
                    wo_copy().wait()
                    x_copy(3 * NT, NT).wait()
                    for i in range(3):
                        f_copy(i).start()
            if s >= 2:
                pl.when(p == 1)(lambda: o_copy(s - 2).start())
            pair_step(s, p)
            return c
        with jax.named_scope(f"seg{s}"):
            if s < NSEG - 1:
                lax.fori_loop(0, NG // 2, body, 0)
            else:
                lax.fori_loop(0, NG // 2 - 1, body, 0)
        if s == 1:
            with jax.named_scope("ffn"):
                for i in range(3):
                    f_copy(i).wait()
                idx, r_sel = route()
                gather(idx)

    with jax.named_scope("tail"):
        routed_columns(idx, r_sel)
        nd = pair_step(NSEG - 1, NG // 2 - 1, last=True)
        attend_tile(NSEG - 1, NG - 1, 0, nd, v_keep, None)
    with jax.named_scope("tail2"):
        o_copy(0).wait()
        o_copy(1).wait()
        add_routed(idx)
        o_copy(NSEG - 2).start()
        tiles = [i // T for i in idx]
        redo = [tiles[0] < 2 * NT, (tiles[1] < 2 * NT) & (tiles[1] != tiles[0])]
        for c in range(2):
            pl.when(redo[c])(lambda c=c: tile_copy(tiles[c], 13 + c).start())
    with jax.named_scope("tail3"):
        for t in range(NT):
            if t + 1 < NT:
                attend_tile(NSEG - 1, NG - 1, t + 1, nd, v_keep, None)
            last_out_proj(t)
    with jax.named_scope("fin"):
        for c in range(2):
            pl.when(redo[c])(lambda c=c: tile_copy(tiles[c], 13 + c).wait())
        o_copy(NSEG - 2).wait()
        for t in range(NT):
            tile_copy((NSEG - 1) * NT + t, 7 + t).wait()


@jax.jit
def pallas_parallel_sum__memory_aug_infini_attn__moe_arch_mod__prompt_kernel(
    A_x, A_wq, A_wk, A_wv, A_wo, A_beta, B_x, B_w_r, B_w_gate, B_w_up, B_w_down,
):
    del B_x
    xt = jnp.transpose(A_x[0]).reshape(NG, GR, S)
    wdt = jnp.transpose(B_w_down)
    hbm = pl.BlockSpec(memory_space=pltpu.HBM)
    carry = (pltpu.VMEM((GR, L), F32), pltpu.VMEM((L, T), BF16), pltpu.VMEM((GR, L), F32),
             pltpu.VMEM((GR, L), F32), pltpu.VMEM((L, T), BF16))
    out = pl.pallas_call(
        _kernel,
        out_shape=jax.ShapeDtypeStruct((NG, GR, S), BF16),
        in_specs=[hbm] * 10,
        out_specs=hbm,
        scratch_shapes=[
            pltpu.VMEM((NSEG, NG, GR, L), BF16),
            pltpu.VMEM((4, D, D), BF16),
            pltpu.VMEM((H,), BF16),
            pltpu.VMEM((D,), BF16),
            pltpu.VMEM((D, F), BF16),
            pltpu.VMEM((D, F), BF16),
            pltpu.VMEM((D, F), BF16),
            pltpu.VMEM((NSEG, DP, L), BF16),
            pltpu.VMEM((NSEG, NG, GR, L), F32),
            pltpu.VMEM((4, DP, DP), WT),
            pltpu.VMEM((8, DP), F32),
            pltpu.VMEM((NG, GR, T), F32),
            pltpu.VMEM((NG, GP, T), F32),
            [pltpu.VMEM((NG, GP, L), BF16)] * NSEG,
            pltpu.VMEM((NSEG, NG, GR, L), BF16),
            pltpu.VMEM((NSEG, 8, L), F32),
            pltpu.VMEM((2, NG, GR, T), F32),
            (carry, carry),
            pltpu.VMEM((GR, L), F32),
            [[pltpu.VMEM((i * T + HT, T), F32)] * GH for i in range(NT)],
            [[pltpu.VMEM((HT, T), F32)] * (GH // 2)] * NT,
            pltpu.VMEM((NT * GH, 8, T), F32),
            pltpu.VMEM((8, D), F32),
            pltpu.VMEM((8, F), F32),
            pltpu.VMEM((8, DP), F32),
            pltpu.VMEM((2, 8, T), F32),
            pltpu.SMEM((1,), jnp.int32),
            pltpu.SemaphoreType.DMA((NSEG * NT,)),
            pltpu.SemaphoreType.DMA((12,)),
            pltpu.SemaphoreType.DMA((15,)),
        ],
        compiler_params=pltpu.CompilerParams(vmem_limit_bytes=100 * 1024 * 1024),
        name="infini_mod",
    )(xt, A_wq, A_wk, A_wv, A_wo, A_beta, B_w_r, B_w_gate, B_w_up, wdt)
    return jnp.transpose(out.reshape(D, S))[None]
```

```python
import functools

import jax
import jax.numpy as jnp
import numpy as np
from jax import lax
import jax.experimental.pallas as pl
import jax.experimental.pallas.tpu as pltpu

D = 576
S = 2048
H = 32
DH = 18
NSEG = 4
L = 512
F = 4608
NG = 8
NP = NG // 2
GH = 4
GR = 72
GP = 80
DP = NG * GP
T = 128
HT = T // 2
NT = L // T

F32 = jnp.float32
BF16 = jnp.bfloat16
QSCALE = float(DH ** -0.5 * np.log2(np.e))
LN_EPS = float(np.asarray(1e-5, dtype=jnp.bfloat16).astype(np.float32))
MASKED = -1e30
F32_TINY = float(np.finfo(np.float32).tiny)
BF16_MAX = float(jnp.finfo(jnp.bfloat16).max)

SUM_SLAB = (2, 2, 2, 0)
SUM_ROW = (5, 6, 7, 0)
DEN_ROW = 1

JOBS_A = "L30 P30 L31 P31 L32 P32 P33 E3 L20 P20 L21 P21 P22 E2 L10 P10 P11 E1 L00 P00 E0 C3 M3 C2 M2 C1 M1 C0 M0"
JOBS_B = (
    "P33 L30 P30 L31 P31 L32 P32 E3 P22 L20 P20 L21 P21 E2 P11 L10 P10 E1 L00 P00 E0 C3 M3 C2 M2 C1 M1 C0 M0",
    "L00 P00 E0 L30 P30 L31 P31 L32 P32 P33 E3 L20 P20 L21 P21 P22 E2 L10 P10 C3 C2 P11 E1 C1 C0 M3 M2 M1 M0",
    "L30 P30 L31 P31 L32 P32 C3 C2 P33 E3 L20 P20 L21 P21 C1 C0 P22 E2 L10 P10 P11 E1 L00 P00 E0 M3 M2 M1 M0",
    "L00 P00 E0 L30 P30 L31 P31 L32 P32 P33 E3 L20 P20 L21 P21 P22 E2 L10 P10 C3 C2 P11 E1 C1 C0 M3 M2 M1 M0",
)
JOBS_FIRST = "L30 L31 L32 L20 L21 L10 L00 C3 M3 C2 M2 C1 M1 C0 M0"


def _rnd(x):
    return x.astype(BF16).astype(F32)


def _dot(a, b):
    return lax.dot_general(a, b, (((1,), (0,)), ((), ())), preferred_element_type=F32)


def _dot_nt(a, b):
    return lax.dot_general(a, b, (((1,), (1,)), ((), ())), preferred_element_type=F32)


def _phi(t):
    return jnp.where(t > 0, t + 1.0, jnp.exp(t))


def _iota(shape, axis):
    return lax.broadcasted_iota(jnp.int32, shape, axis)


def _head_of(i):
    return (i * 57) >> 10


def _ds(i, n, align):
    return pl.ds(i if isinstance(i, int) else pl.multiple_of(i, align), n)


def _lane_tile(t):
    return _ds(t * T, T, T)


def _rows_max(x):
    return jnp.max(x.reshape(x.shape[0] // 8, 8, T), axis=0)


def _exp2_shifted(x, m):
    return jnp.exp2(x.reshape(x.shape[0] // 8, 8, T) - m[None]).reshape(x.shape)


def _pad_rows(x, n):
    return jnp.concatenate([x, jnp.zeros((n - x.shape[0], x.shape[1]), x.dtype)], axis=0)


def _pad_groups(x, axis):
    zeros = jnp.zeros_like(lax.slice_in_dim(x, 0, GP - GR, axis=axis))
    parts = []
    for g in range(NG):
        parts += [lax.slice_in_dim(x, g * GR, (g + 1) * GR, axis=axis), zeros]
    return jnp.concatenate(parts, axis=axis)


def _merge_heads(w):
    row = _iota((8, T), 0)
    return jnp.concatenate([
        w[0][0], w[0][1], jnp.where(row < 2, w[0][2], w[1][0]),
        w[1][1], jnp.where(row < 4, w[1][2], w[2][0]),
        w[2][1], jnp.where(row < 6, w[2][2], w[3][0]),
        w[3][1], w[3][2]], axis=0)


def _kernel(x_hbm, wq_hbm, wk_hbm, wv_hbm, wo_hbm, beta_hbm, wr_hbm, wg_hbm, wu_hbm, wd_hbm,
            out_hbm,
            x_s, w_s, beta_s, wr_s, wg_s, wu_s, wd_s,
            xn_s, base_s, wt_s, router_s, mix_s, mem_s, ot_s, out_s,
            qkv_s, v_held, logit_s, corner_s, max_s,
            score_s, xsel_s, h_s, y_s, upd_s, stat_s, zero_s,
            x_sems, w_sems, sems):
    w_hbm = (wq_hbm, wk_hbm, wv_hbm)

    def x_copy(t0, n):
        return pltpu.make_async_copy(x_hbm.at[:, :, pl.ds(t0 * T, n * T)],
                                     x_s.at[t0 // NT, :, :, pl.ds(t0 % NT * T, n * T)], x_sems.at[t0])

    def w_copy(i, c):
        cols = pl.ds(0, 2 * T) if c == 0 else pl.ds((c + 1) * T, min(T, D - (c + 1) * T))
        return pltpu.make_async_copy(w_hbm[i].at[:, cols], w_s.at[i, :, cols], w_sems.at[4 * i + c])

    def ffn_copy(i):
        return pltpu.make_async_copy((wg_hbm, wu_hbm, wd_hbm)[i], (wg_s, wu_s, wd_s)[i], sems.at[i])

    def segment_store(s):
        return pltpu.make_async_copy(out_s.at[s], out_hbm.at[:, :, pl.ds(s * L, L)], sems.at[3 + s])

    def tile_store(n, sem):
        return pltpu.make_async_copy(out_s.at[n // NT, :, :, _lane_tile(n % NT)],
                                     out_hbm.at[:, :, _lane_tile(n)], sems.at[6 + sem])

    wo_copy = pltpu.make_async_copy(wo_hbm, w_s.at[3], sems.at[12])
    wr_copy = pltpu.make_async_copy(wr_hbm, wr_s, sems.at[13])
    beta_copy = pltpu.make_async_copy(beta_hbm, beta_s, sems.at[14])

    def make_mix():
        gate = jnp.broadcast_to(jax.nn.sigmoid(beta_s[...].astype(F32)).reshape(1, H), (8, H))
        row = _iota((8, H), 0)
        head = row - DEN_ROW
        for j in range(GH):
            head = jnp.where(row == SUM_ROW[j], j, head)
        weight = jnp.where(head == row - DEN_ROW, gate, 1.0 - gate)
        for g in range(NG):
            col = jnp.sum(jnp.where(head + g * GH == _iota((8, H), 1), weight, 0.0), axis=1, keepdims=True)
            mix_s[g] = jnp.broadcast_to(col, (8, T))

    def transpose_w(i, c):
        parts = []
        for g in range(NG):
            parts += [w_s[i, pl.ds(g * GR, GR), _lane_tile(c)], jnp.zeros((GP - GR, T), BF16)]
        w = jnp.concatenate(parts, axis=0)
        if not isinstance(c, int):
            w = jnp.where(_iota((DP, T), 1) < D - c * T, w, jnp.zeros_like(w))
        wt_s[i, _lane_tile(c), :] = w.T

    def inv_std(var):
        return 1.0 / _rnd(jnp.sqrt(_rnd(_rnd(var) + LN_EPS)))

    def layer_norm_now(t):
        lanes = _lane_tile(t)

        def x(g):
            return x_s[0, g, :, lanes].astype(F32).reshape(GR // 8, 8, T)

        def mean_of(f):
            acc = f(x(0))
            for g in range(1, NG):
                acc = acc + f(x(g))
            acc = acc[0:3] + acc[3:6] + acc[6:9]
            total = jnp.sum(acc[0] + acc[1] + acc[2], axis=0, keepdims=True)
            return jnp.broadcast_to(total / D, (8, T))

        stat_s[0] = mean = mean_of(lambda v: v)
        stat_s[1] = var = mean_of(lambda v: (v - mean[None]) * (v - mean[None]))
        mean, inv = _rnd(mean), inv_std(var)
        for g in range(NG):
            xg = x(g)
            xn = _rnd(_rnd(xg - mean[None]) * inv[None]).reshape(GR, T)
            base_s[0, g, :, lanes] = xg.reshape(GR, T) + xn
            xn_s[0, pl.ds(g * GP, GP), lanes] = _pad_rows(xn, GP).astype(BF16)

    def layer_norm_background(n, after=None):
        s, lanes = n // NT, _lane_tile(n % NT)
        x = x_s[s, :, :, lanes].astype(F32).reshape(D, T)
        mean = jnp.sum(x, axis=0, keepdims=True) / D
        var = jnp.sum((x - mean) * (x - mean), axis=0, keepdims=True) / D
        mean = jnp.broadcast_to(_rnd(mean), (8, T))
        inv = jnp.broadcast_to(inv_std(var), (8, T))
        never = _iota((8, T), 0) < zero_s[0]
        if after is not None:
            mean = jnp.where(never, after, mean)
        slabs = []
        for c in range(0, D, 8):
            slabs.append(_rnd(_rnd(x[c:c + 8] - mean) * inv))
            mean = jnp.where(never, slabs[-1], mean)
        xn = jnp.concatenate(slabs, axis=0)
        base_s[s, :, :, lanes] = (x + xn).reshape(NG, GR, T)
        xn_s[s, :, lanes] = _pad_groups(xn, 0).astype(BF16)
        score_s[s, :, lanes] = _dot(router_s[...], xn_s[s, :, lanes])
        return slabs[-1]

    def pair_rows(p):
        return _ds(p * 2 * GR, 2 * GR, 16)

    def weight_dot(i, p, rhs, fillers):
        if not fillers:
            return _dot(wt_s[i, pair_rows(p), :], rhs(slice(None), slice(None)))
        rest = _dot(wt_s[i, pair_rows(p), pl.ds(4 * T, T)], rhs(pl.ds(4 * T, T), slice(None)))
        fillers.pop(0)()
        parts = []
        for t in range(NT):
            parts.append(_dot(wt_s[i, pair_rows(p), pl.ds(0, 4 * T)], rhs(pl.ds(0, 4 * T), _lane_tile(t))))
            fillers.pop(0)()
        return jnp.concatenate(parts, axis=1) + rest

    def keep(i, val):
        for e, (q_s, k_s, v_s, pq_s, pk_s) in enumerate(qkv_s):
            part = val[e * GR:(e + 1) * GR]
            if i == 0:
                q_s[...] = part * QSCALE
                pq_s[...] = _phi(part)
            elif i == 1:
                k = _pad_rows(part, T).T
                k_s[...] = k.astype(BF16)
                pk_s[...] = _phi(k).astype(BF16)
            else:
                v_s[...] = part

    def project(s, p, fillers):
        if fillers:
            for i in (1, 0, 2):
                keep(i, weight_dot(i, p, lambda r, c: xn_s[s, r, c], fillers))
        else:
            qkv = _dot(jnp.concatenate([wt_s[i, pair_rows(p), :] for i in range(3)], axis=0), xn_s[s])
            for i in range(3):
                keep(i, qkv[i * 2 * GR:(i + 1) * 2 * GR])

    def out_project(s, p, fillers):
        a = weight_dot(3, p, lambda r, c: ot_s[s][r, c], fillers)
        for e in range(2):
            out_s[s, 2 * p + e] = (base_s[s, 2 * p + e] + a[e * GR:(e + 1) * GR]).astype(BF16)

    def memory(s, g, buf):
        _, _, v_s, pq_s, pk_s = buf
        read = None
        if s > 0:
            row, col = _iota((GP, T), 0), _iota((GP, T), 1)
            row_head = jnp.where(row < GR, _head_of(row), row - (GR + DEN_ROW))
            m = jnp.where((row_head == _head_of(col)) & (col < GR), mem_s[g], 0.0)
            read = _dot(m.astype(BF16), _pad_rows(pq_s[...], T).astype(BF16))
        if s < NSEG - 1:
            v1 = jnp.concatenate([v_s[...], jnp.ones((GP - GR, L), F32)], axis=0)
            update = _dot(v1.astype(BF16), pk_s[...])
            mem_s[g] = mem_s[g] + update if s > 0 else update
        return read

    def query_tiles(i, q_s):
        q = q_s[:, _lane_tile(i)]
        rotated = pltpu.roll(q, HT, 1)
        row = _iota((GR, T), 0)
        return [jnp.where((row >= DH * j) & (row < DH * (j + 1)), q if j % 2 else rotated, 0.0)
                for j in range(GH)]

    def key_logits(qk, k0, n, tiles):
        weights = jnp.concatenate([_pad_rows(q, GP).astype(BF16) for q in tiles], axis=1)
        return _dot(qk[1][pl.ds(k0, n), :][:, :GP], weights)

    def attention(s, g, jobs, mem_read, v_s, qk):
        lane = _iota((HT, T), 1)
        future = _iota((HT, T), 0) > (lane & (HT - 1))
        head_masks = [jnp.where(future & (lane >= HT), MASKED, 0.0), jnp.where(future & (lane < HT), MASKED, 0.0)]
        low = _iota((8, T), 1) < HT
        row = _iota((8, T), 0)
        acc, top = {}, {}

        @functools.cache
        def shift(i):
            return [max_s[i * GH + j] for j in range(GH)]

        @functools.cache
        def corner_probs(i):
            return [_exp2_shifted(corner_s[i][j // 2][...], jnp.where(low, shift(i)[j], shift(i)[j + 1]))
                    for j in range(0, GH, 2)]

        @functools.cache
        def probs(i, k):
            if k < i:
                return [_exp2_shifted(logit_s[i][j][pl.ds(k * T, T), :], shift(i)[j]).astype(BF16)
                        for j in range(GH)]
            ps = []
            for j in range(GH):
                head = _exp2_shifted(logit_s[i][j][pl.ds(i * T, HT), :], shift(i)[j])
                tail = jnp.where(lane >= HT if j % 2 else lane < HT, corner_probs(i)[j // 2], 0.0)
                ps.append(jnp.concatenate([head, tail], axis=0).astype(BF16))
            return ps

        @functools.cache
        def queries(i):
            return query_tiles(i, qk[0])

        def raise_top(i, j, m):
            top[i, j] = jnp.maximum(top[i, j], m) if (i, j) in top else m

        for job in jobs.split():
            kind, i, k = job[0], *(int(c) for c in job[1:].ljust(2, "0"))
            if kind == "P":
                for j in range(GH):
                    v = [v_s[pl.ds(16 * j + 8 * c, 8), _lane_tile(k)] for c in range(3)]
                    v[SUM_SLAB[j]] = jnp.where(row == SUM_ROW[j], 1.0, v[SUM_SLAB[j]])
                    o = _dot(jnp.concatenate(v, axis=0), probs(i, k)[j])
                    acc[i, j] = acc[i, j] + o if (i, j) in acc else o
            elif kind == "E":
                o = [acc[i, j] if j % 2 else pltpu.roll(acc[i, j], HT, 1) for j in range(GH)]
                o = [[oj[8 * c:8 * c + 8] for c in range(3)] for oj in o]
                den = mem_read[GR:GP, i * T:(i + 1) * T] + 1e-6 if s > 0 else jnp.ones((8, T), F32)
                for j in range(GH):
                    den = jnp.where(row == SUM_ROW[j], o[j][SUM_SLAB[j]], den)
                scale = mix_s[g] / den

                def per_head(rows):
                    return _merge_heads([[jnp.broadcast_to(scale[r:r + 1], (8, T))] * 3 for r in rows])

                mixed = _merge_heads(o) * per_head(SUM_ROW)
                if s > 0:
                    mixed = mixed + mem_read[0:GR, i * T:(i + 1) * T] * per_head(range(DEN_ROW, DEN_ROW + GH))
                ot_s[s][_ds(g * GP, GP, 16), _lane_tile(i)] = _pad_rows(mixed, GP).astype(BF16)
            elif kind == "L":
                diagonal = k >= i - 1
                n = i * T + HT - k * T if diagonal else T
                if v_s is not None:
                    probs(i, k)
                    if diagonal:
                        probs(i, i)
                st = key_logits(qk, k * T, n, queries(i))
                for j in range(GH):
                    sj = st[:, j * T:(j + 1) * T]
                    if diagonal:
                        end = sj[n - HT:] + head_masks[j % 2]
                        sj = end if n == HT else jnp.concatenate([sj[:n - HT], end], axis=0)
                    logit_s[i][j][pl.ds(k * T, n), :] = sj
                    raise_top(i, j, _rows_max(sj))
            elif kind == "C":
                if v_s is not None:
                    corner_probs(i)
                q = query_tiles(i, qk[0])
                first = _iota((GR, T), 1) < HT
                st = key_logits(qk, i * T + HT, HT, [jnp.where(first, q[j], q[j + 1]) for j in range(0, GH, 2)])
                for j in range(0, GH, 2):
                    sj = st[:, j // 2 * T:(j // 2 + 1) * T] + jnp.where(future, MASKED, 0.0)
                    corner_s[i][j // 2][...] = sj
                    m = _rows_max(sj)
                    raise_top(i, j, jnp.where(low, m, -jnp.inf))
                    raise_top(i, j + 1, jnp.where(low, -jnp.inf, m))
            elif kind == "M":
                if v_s is not None:
                    shift(i)
                for j in range(GH):
                    max_s[i * GH + j] = jnp.broadcast_to(jnp.max(top[i, j], axis=0, keepdims=True), (8, T))

    def route():
        r = _rnd(jnp.concatenate([score_s[s] for s in range(NSEG)], axis=1))
        r = jnp.clip(jnp.where(jnp.abs(r) < F32_TINY, F32_TINY, r), -BF16_MAX, BF16_MAX)
        tok = _iota((8, S), 1)
        key = pltpu.bitcast(pltpu.bitcast(r, jnp.int32) | jnp.where(r > 0, S - 1 - tok, tok), F32)
        k0 = jnp.max(key, axis=1, keepdims=True)
        k1 = jnp.max(jnp.where(key == k0, -jnp.inf, key), axis=1, keepdims=True)
        best = jnp.broadcast_to(jnp.where(_iota((8, 1), 0) == 0, k0, k1), (8, T))
        bits = pltpu.bitcast(best, jnp.int32)
        pos = jnp.where(best > 0, S - 1 - (bits & (S - 1)), bits & (S - 1))
        return (pos[0, 0], pos[1, 0]), jax.nn.sigmoid(pltpu.bitcast(bits & -(1 << 16), F32))

    def gather(idx):
        xs = jnp.zeros((8, DP), F32)
        for c in range(2):
            tile = xn_s[idx[c] // L, :, _lane_tile((idx[c] % L) // T)]
            hot = ((_iota((8, T), 1) == idx[c] % T) & (_iota((8, T), 0) == c)).astype(F32)
            xs = xs + _dot_nt(hot, tile)
        xsel_s[...] = jnp.concatenate([xs[:, g * GP:g * GP + GR] for g in range(NG)], axis=1)
        y_s[...] = jnp.zeros((8, DP), F32)

    def gate_up_jobs(p):
        n = F // T // NP
        pre = {}

        def last_rows(m):
            rows = pl.ds(4 * T, D - 4 * T)
            pre[m] = _dot(xsel_s[:, rows], (wg_s, wu_s)[m][rows, _ds(p * n * T, n * T, T)])

        def first_rows(t, m):
            rows, cols = pl.ds(0, 4 * T), _lane_tile(p * n + t)
            pre[m, t] = _dot(xsel_s[:, rows], (wg_s, wu_s)[m][rows, cols]) + pre[m][:, t * T:(t + 1) * T]
            if m == 1:
                h_s[:, cols] = pre[0, t] * jax.nn.sigmoid(pre[0, t]) * pre[1, t]

        return ([functools.partial(last_rows, m) for m in range(2)]
                + [functools.partial(first_rows, t, m) for t in range(n) for m in range(2)])

    def down_jobs(p):
        n = F // T // (NP - 1)

        def piece(c, d):
            rows, cols = pl.ds(d * T, min(T, D - d * T)), _ds((p * n + 4 * c) * T, 4 * T, T)
            y_s[:, rows] += _dot_nt(h_s[:, cols], wd_s[rows, cols])

        return [functools.partial(piece, c, d) for c in range(n // 4) for d in range(DP // T)]

    def place_updates(idx, r_sel):
        yt = _pad_rows(y_s[...] * jnp.concatenate([r_sel] * (DP // T), axis=1), T).T[:D]
        for c in range(2):
            upd = pltpu.roll(yt, (idx[c] + T - c) % T, 1)
            upd_s[c] = jnp.where(_iota((D, T), 1) == idx[c] % T, upd, 0.0).reshape(NG, GR, T)

    def add_updates(idx):
        for c in range(2):
            s, lanes = idx[c] // L, _lane_tile((idx[c] % L) // T)

            @pl.when(s < NSEG - 1)
            def _():
                out_s[s, :, :, lanes] = (out_s[s, :, :, lanes].astype(F32) + upd_s[c]).astype(BF16)

            @pl.when(s == NSEG - 1)
            def _():
                base_s[NSEG - 1, :, :, lanes] += upd_s[c]

    def step(s, p, last=False):
        fillers = []
        if s == NSEG - 2:
            fillers = gate_up_jobs(p)
        elif s == NSEG - 1 and not last:
            fillers = down_jobs(p)
        reads = [memory(s, 2 * p + e, qkv_s[e]) for e in range(2)]
        v_held[...] = qkv_s[1][2][...]
        attention(s, 2 * p, JOBS_A, reads[0], qkv_s[0][2], qkv_s[1])
        if not last:
            nxt = s * NP + p + 1
            project(nxt // NP, nxt % NP, fillers)
            if s == 0:
                layer_norm_background(NT + 2 * p + 1, layer_norm_background(NT + 2 * p))
                for e in range(3):
                    transpose_w(jnp.where(p < 2, e, 3),
                                jnp.where(p < 2, p + 3, jnp.minimum(3 * (p - 2) + e, 4)))
            elif s == 1:
                layer_norm_background(3 * NT + p)
            attention(s, 2 * p + 1, JOBS_B[s], reads[1], v_held, qkv_s[0])
        if s > 0:
            out_project(s - 1, p, fillers)
        assert not fillers
        return reads[1]

    def first_dot(i):
        return _dot(wt_s[i, pair_rows(0), :], xn_s[0])

    zero_s[0] = 0
    for t in range(NT):
        x_copy(t, 1).start()
    for t in range(NT):
        x_copy(t, 1).wait()
        if t < 3:
            w_copy((1, 0, 2)[t], 0).start()
        if t == 2:
            wr_copy.start()
            beta_copy.start()
        layer_norm_now(t)
    w_copy(1, 0).wait()
    for c in range(2):
        transpose_w(1, c)
    w_copy(0, 0).wait()
    for i in range(3):
        w_copy(i, 1).start()
    kt = first_dot(1)
    for c in range(2):
        transpose_w(0, c)
    w_copy(2, 0).wait()
    wr_copy.wait()
    beta_copy.wait()
    x_copy(NT, NT).start()
    for i in range(3):
        w_copy(i, 2).start()
    keep(1, kt)
    keep(0, first_dot(0))
    for c in range(2):
        transpose_w(2, c)
    make_mix()
    router_s[...] = _pad_groups(jnp.broadcast_to(wr_s[...].astype(F32).reshape(1, D), (8, D)), 1)
    for i in range(3):
        w_copy(i, 1).wait()
    for i in range(3):
        w_copy(i, 3).start()
    x_copy(2 * NT, NT).start()
    wo_copy.start()
    x_copy(3 * NT, NT).start()
    keep(2, first_dot(2))
    score_s[0] = _dot(router_s[...], xn_s[0])
    attention(0, 0, JOBS_FIRST, None, None, qkv_s[0])
    for i in range(3):
        transpose_w(i, 2)
    x_copy(NT, NT).wait()
    for i in range(3):
        w_copy(i, 2).wait()

    for s in range(NSEG):
        def body(p, carry, s=s):
            if s == 0:
                @pl.when(p == 1)
                def _():
                    for i in range(3):
                        w_copy(i, 3).wait()
                    x_copy(2 * NT, NT).wait()
                    wo_copy.wait()
                    x_copy(3 * NT, NT).wait()
                    for i in range(3):
                        ffn_copy(i).start()
            if s >= 2:
                pl.when(p == 1)(lambda: segment_store(s - 2).start())
            step(s, p)
            return carry

        lax.fori_loop(0, NP if s < NSEG - 1 else NP - 1, body, 0)
        if s == 1:
            for i in range(3):
                ffn_copy(i).wait()
            idx, r_sel = route()
            gather(idx)

    s = NSEG - 1
    place_updates(idx, r_sel)
    mem_read = step(s, NP - 1, last=True)
    attention(s, NG - 1, "P00 E0", mem_read, v_held, None)
    segment_store(0).wait()
    segment_store(1).wait()
    add_updates(idx)
    segment_store(2).start()
    tiles = [i // T for i in idx]
    again = [tiles[0] < 2 * NT, (tiles[1] < 2 * NT) & (tiles[1] != tiles[0])]
    for c in range(2):
        pl.when(again[c])(lambda c=c: tile_store(tiles[c], NT + c).start())
    for t in range(NT):
        if t + 1 < NT:
            jobs = " ".join(f"P{t + 1}{k}" for k in range(t + 2)) + f" E{t + 1}"
            attention(s, NG - 1, jobs, mem_read, v_held, None)
        lanes = _lane_tile(t)
        a = _dot(wt_s[3, pl.ds(0, D), :], ot_s[s][:, lanes]).reshape(NG, GR, T)
        out_s[s, :, :, lanes] = (base_s[s, :, :, lanes] + a).astype(BF16)
        tile_store(s * NT + t, t).start()
    for c in range(2):
        pl.when(again[c])(lambda c=c: tile_store(tiles[c], NT + c).wait())
    segment_store(2).wait()
    for t in range(NT):
        tile_store(s * NT + t, t).wait()


@jax.jit
def pallas_parallel_sum__memory_aug_infini_attn__moe_arch_mod__prompt_kernel(
    A_x, A_wq, A_wk, A_wv, A_wo, A_beta, B_x, B_w_r, B_w_gate, B_w_up, B_w_down,
):
    del B_x
    hbm = pl.BlockSpec(memory_space=pltpu.HBM)
    group = (pltpu.VMEM((GR, L), F32),
             pltpu.VMEM((L, T), BF16),
             pltpu.VMEM((GR, L), F32),
             pltpu.VMEM((GR, L), F32),
             pltpu.VMEM((L, T), BF16))
    out = pl.pallas_call(
        _kernel,
        out_shape=jax.ShapeDtypeStruct((NG, GR, S), BF16),
        in_specs=[hbm] * 10,
        out_specs=hbm,
        scratch_shapes=[
            pltpu.VMEM((NSEG, NG, GR, L), BF16),
            pltpu.VMEM((4, D, D), BF16),
            pltpu.VMEM((H,), BF16),
            pltpu.VMEM((D,), BF16),
            pltpu.VMEM((D, F), BF16),
            pltpu.VMEM((D, F), BF16),
            pltpu.VMEM((D, F), BF16),
            pltpu.VMEM((NSEG, DP, L), BF16),
            pltpu.VMEM((NSEG, NG, GR, L), F32),
            pltpu.VMEM((4, DP, DP), BF16),
            pltpu.VMEM((8, DP), F32),
            pltpu.VMEM((NG, 8, T), F32),
            pltpu.VMEM((NG, GP, T), F32),
            [pltpu.VMEM((DP, L), BF16)] * NSEG,
            pltpu.VMEM((NSEG, NG, GR, L), BF16),
            (group, group),
            pltpu.VMEM((GR, L), F32),
            [[pltpu.VMEM((i * T + HT, T), F32)] * GH for i in range(NT)],
            [[pltpu.VMEM((HT, T), F32)] * (GH // 2)] * NT,
            pltpu.VMEM((NT * GH, 8, T), F32),
            pltpu.VMEM((NSEG, 8, L), F32),
            pltpu.VMEM((8, D), F32),
            pltpu.VMEM((8, F), F32),
            pltpu.VMEM((8, DP), F32),
            pltpu.VMEM((2, NG, GR, T), F32),
            pltpu.VMEM((2, 8, T), F32),
            pltpu.SMEM((1,), jnp.int32),
            pltpu.SemaphoreType.DMA((NSEG * NT,)),
            pltpu.SemaphoreType.DMA((12,)),
            pltpu.SemaphoreType.DMA((15,)),
        ],
        compiler_params=pltpu.CompilerParams(vmem_limit_bytes=100 * 1024 * 1024),
        name="infini_mod",
    )(jnp.transpose(A_x[0]).reshape(NG, GR, S), A_wq, A_wk, A_wv, A_wo, A_beta, B_w_r,
      B_w_gate, B_w_up, jnp.transpose(B_w_down))
    return jnp.transpose(out.reshape(D, S))[None]
```

```python
import functools

import jax
import jax.numpy as jnp
import numpy as np
from jax import lax
import jax.experimental.pallas as pl
import jax.experimental.pallas.tpu as pltpu

D = 576
S = 2048
H = 32
DH = 18
NSEG = 4
L = 512
F = 4608
NG = 8
NP = NG // 2
GH = 4
GR = 72
GP = 80
DP = NG * GP
T = 128
HT = T // 2
NT = L // T

F32 = jnp.float32
BF16 = jnp.bfloat16
QSCALE = float(DH ** -0.5 * np.log2(np.e))
LN_EPS = float(np.asarray(1e-5, dtype=jnp.bfloat16).astype(np.float32))
MASKED = -1e30
F32_TINY = float(np.finfo(np.float32).tiny)
BF16_MAX = float(jnp.finfo(jnp.bfloat16).max)

SUM_SLAB = (2, 2, 2, 0)
SUM_ROW = (5, 6, 7, 0)
DEN_ROW = 1

JOBS_A = "L30 P30 L31 P31 L32 P32 P33 E3 L20 P20 L21 P21 P22 E2 L10 P10 P11 E1 L00 P00 E0 C3 M3 C2 M2 C1 M1 C0 M0"
JOBS_B = (
    "P33 L30 P30 L31 P31 L32 P32 E3 P22 L20 P20 L21 P21 E2 P11 L10 P10 E1 L00 P00 E0 C3 M3 C2 M2 C1 M1 C0 M0",
    "L00 P00 E0 L30 P30 L31 P31 L32 P32 P33 E3 L20 P20 L21 P21 P22 E2 L10 P10 C3 C2 P11 E1 C1 C0 M3 M2 M1 M0",
    "P11 L10 P10 E1 L00 P00 E0 P33 L30 P30 L31 P31 C1 C0 L32 P32 E3 C3 C2 P22 L20 P20 L21 P21 E2 M3 M2 M1 M0",
    "L00 P00 E0 L30 P30 L31 P31 L32 P32 P33 E3 L20 P20 L21 P21 P22 E2 L10 P10 C3 C2 P11 E1 C1 C0 M3 M2 M1 M0",
)
JOBS_FIRST = "L30 L31 L32 L20 L21 L10 L00 C3 M3 C2 M2 C1 M1 C0 M0"


def _rnd(x):
    return x.astype(BF16).astype(F32)


def _dot(a, b):
    return lax.dot_general(a, b, (((1,), (0,)), ((), ())), preferred_element_type=F32)


def _dot_nt(a, b):
    return lax.dot_general(a, b, (((1,), (1,)), ((), ())), preferred_element_type=F32)


def _phi(t):
    return jnp.where(t > 0, t + 1.0, jnp.exp(t))


def _iota(shape, axis):
    return lax.broadcasted_iota(jnp.int32, shape, axis)


def _head_of(i):
    return (i * 57) >> 10


def _ds(i, n, align):
    return pl.ds(i if isinstance(i, int) else pl.multiple_of(i, align), n)


def _lane_tile(t):
    return _ds(t * T, T, T)


def _rows_max(x):
    return jnp.max(x.reshape(x.shape[0] // 8, 8, T), axis=0)


def _exp2_shifted(x, m):
    return jnp.exp2(x.reshape(x.shape[0] // 8, 8, T) - m[None]).reshape(x.shape)


def _pad_rows(x, n):
    return jnp.concatenate([x, jnp.zeros((n - x.shape[0], x.shape[1]), x.dtype)], axis=0)


def _pad_groups(x, axis):
    zeros = jnp.zeros_like(lax.slice_in_dim(x, 0, GP - GR, axis=axis))
    parts = []
    for g in range(NG):
        parts += [lax.slice_in_dim(x, g * GR, (g + 1) * GR, axis=axis), zeros]
    return jnp.concatenate(parts, axis=axis)


def _merge_heads(w):
    row = _iota((8, T), 0)
    return jnp.concatenate([
        w[0][0], w[0][1], jnp.where(row < 2, w[0][2], w[1][0]),
        w[1][1], jnp.where(row < 4, w[1][2], w[2][0]),
        w[2][1], jnp.where(row < 6, w[2][2], w[3][0]),
        w[3][1], w[3][2]], axis=0)


def _kernel(x_hbm, wq_hbm, wk_hbm, wv_hbm, wo_hbm, beta_hbm, wr_hbm, wg_hbm, wu_hbm, wd_hbm,
            out_hbm,
            x_s, w_s, beta_s, wr_s, wg_s, wu_s, wd_s,
            xn_s, wt_s, router_s, mix_s, mem_s, ot_s, out_s,
            qkv_s, v_held, logit_s, corner_s, max_s,
            score_s, xsel_s, h_s, y_s, upd_s, stat_s, zero_s,
            x_sems, w_sems, sems):
    w_hbm = (wq_hbm, wk_hbm, wv_hbm)

    def x_copy(t0, n):
        return pltpu.make_async_copy(x_hbm.at[:, :, pl.ds(t0 * T, n * T)],
                                     x_s.at[t0 // NT, :, :, pl.ds(t0 % NT * T, n * T)], x_sems.at[t0])

    def w_copy(i, c):
        cols = pl.ds(0, 2 * T) if c == 0 else pl.ds((c + 1) * T, min(T, D - (c + 1) * T))
        return pltpu.make_async_copy(w_hbm[i].at[:, cols], w_s.at[i, :, cols], w_sems.at[4 * i + c])

    def ffn_copy(i):
        return pltpu.make_async_copy((wg_hbm, wu_hbm, wd_hbm)[i], (wg_s, wu_s, wd_s)[i], sems.at[i])

    def segment_store(s):
        return pltpu.make_async_copy(out_s.at[s], out_hbm.at[:, :, pl.ds(s * L, L)], sems.at[3 + s])

    def tile_store(n, sem):
        return pltpu.make_async_copy(out_s.at[n // NT, :, :, _lane_tile(n % NT)],
                                     out_hbm.at[:, :, _lane_tile(n)], sems.at[6 + sem])

    wo_copy = pltpu.make_async_copy(wo_hbm, w_s.at[3], sems.at[12])
    wr_copy = pltpu.make_async_copy(wr_hbm, wr_s, sems.at[13])
    beta_copy = pltpu.make_async_copy(beta_hbm, beta_s, sems.at[14])

    def make_mix():
        gate = jnp.broadcast_to(jax.nn.sigmoid(beta_s[...].astype(F32)).reshape(1, H), (8, H))
        row = _iota((8, H), 0)
        head = row - DEN_ROW
        for j in range(GH):
            head = jnp.where(row == SUM_ROW[j], j, head)
        weight = jnp.where(head == row - DEN_ROW, gate, 1.0 - gate)
        for g in range(NG):
            col = jnp.sum(jnp.where(head + g * GH == _iota((8, H), 1), weight, 0.0), axis=1, keepdims=True)
            mix_s[g] = jnp.broadcast_to(col, (8, T))

    def transpose_w(i, c):
        parts = []
        for g in range(NG):
            parts += [w_s[i, pl.ds(g * GR, GR), _lane_tile(c)], jnp.zeros((GP - GR, T), BF16)]
        w = jnp.concatenate(parts, axis=0)
        if not isinstance(c, int):
            w = jnp.where(_iota((DP, T), 1) < D - c * T, w, jnp.zeros_like(w))
        wt_s[i, _lane_tile(c), :] = w.T

    def inv_std(var):
        return 1.0 / _rnd(jnp.sqrt(_rnd(_rnd(var) + LN_EPS)))

    def layer_norm_now(t):
        lanes = _lane_tile(t)

        def x(g):
            return x_s[0, g, :, lanes].astype(F32).reshape(GR // 8, 8, T)

        def mean_of(f):
            acc = f(x(0))
            for g in range(1, NG):
                acc = acc + f(x(g))
            acc = acc[0:3] + acc[3:6] + acc[6:9]
            total = jnp.sum(acc[0] + acc[1] + acc[2], axis=0, keepdims=True)
            return jnp.broadcast_to(total / D, (8, T))

        stat_s[0] = mean = mean_of(lambda v: v)
        stat_s[1] = var = mean_of(lambda v: (v - mean[None]) * (v - mean[None]))
        mean, inv = _rnd(mean), inv_std(var)
        for g in range(NG):
            xn = (_rnd(x(g) - mean[None]) * inv[None]).reshape(GR, T)
            xn_s[0, pl.ds(g * GP, GP), lanes] = _pad_rows(xn, GP).astype(BF16)

    def layer_norm_background(n):
        s, lanes = n // NT, _lane_tile(n % NT)
        x = x_s[s, :, :, lanes].astype(F32).reshape(D, T)
        mean = jnp.sum(x, axis=0, keepdims=True) / D
        var = jnp.sum((x - mean) * (x - mean), axis=0, keepdims=True) / D
        mean = jnp.broadcast_to(_rnd(mean), (8, T))
        inv = jnp.broadcast_to(inv_std(var), (8, T))
        never = _iota((8, T), 0) < zero_s[0]
        slabs = []
        for c in range(0, D, 8):
            slabs.append(_rnd(x[c:c + 8] - mean) * inv)
            mean = jnp.where(never, slabs[-1], mean)
        xn_s[s, :, lanes] = _pad_groups(jnp.concatenate(slabs, axis=0), 0).astype(BF16)
        score_s[s, :, lanes] = _dot(router_s[...], xn_s[s, :, lanes])

    def pair_rows(p):
        return _ds(p * 2 * GR, 2 * GR, 16)

    def weight_dot(i, p, rhs, fillers):
        if not fillers:
            return _dot(wt_s[i, pair_rows(p), :], rhs(slice(None), slice(None)))
        rest = _dot(wt_s[i, pair_rows(p), pl.ds(4 * T, T)], rhs(pl.ds(4 * T, T), slice(None)))
        fillers.pop(0)()
        parts = []
        for t in range(NT):
            parts.append(_dot(wt_s[i, pair_rows(p), pl.ds(0, 4 * T)], rhs(pl.ds(0, 4 * T), _lane_tile(t))))
            fillers.pop(0)()
        return jnp.concatenate(parts, axis=1) + rest

    def keep(i, val):
        for e, (q_s, k_s, v_s, pq_s, pk_s) in enumerate(qkv_s):
            part = val[e * GR:(e + 1) * GR]
            if i == 0:
                q_s[...] = part * QSCALE
                pq_s[...] = _phi(part)
            elif i == 1:
                k = _pad_rows(part, T).T
                k_s[...] = k.astype(BF16)
                pk_s[...] = _phi(k).astype(BF16)
            else:
                v_s[...] = part

    def project(s, p, fillers):
        if fillers:
            for i in (1, 0, 2):
                keep(i, weight_dot(i, p, lambda r, c: xn_s[s, r, c], fillers))
        else:
            qkv = _dot(jnp.concatenate([wt_s[i, pair_rows(p), :] for i in range(3)], axis=0), xn_s[s])
            for i in range(3):
                keep(i, qkv[i * 2 * GR:(i + 1) * 2 * GR])

    def residual(s, g, lanes):
        return x_s[s, g, :, lanes].astype(F32) + xn_s[s, _ds(g * GP, GP, 16), lanes].astype(F32)[:GR]

    def out_project(s, p, fillers):
        a = weight_dot(3, p, lambda r, c: ot_s[s][r, c], fillers)
        for e in range(2):
            out_s[s, 2 * p + e] = (residual(s, 2 * p + e, slice(None)) + a[e * GR:(e + 1) * GR]).astype(BF16)

    def memory(s, g, buf):
        _, _, v_s, pq_s, pk_s = buf
        read = None
        if s > 0:
            row, col = _iota((GP, T), 0), _iota((GP, T), 1)
            row_head = jnp.where(row < GR, _head_of(row), row - (GR + DEN_ROW))
            m = jnp.where((row_head == _head_of(col)) & (col < GR), mem_s[g], 0.0)
            read = _dot(m.astype(BF16), _pad_rows(pq_s[...], T).astype(BF16))
        if s < NSEG - 1:
            v1 = jnp.concatenate([v_s[...], jnp.ones((GP - GR, L), F32)], axis=0)
            update = _dot(v1.astype(BF16), pk_s[...])
            mem_s[g] = mem_s[g] + update if s > 0 else update
        return read

    def query_tiles(i, q_s):
        q = q_s[:, _lane_tile(i)]
        rotated = pltpu.roll(q, HT, 1)
        row = _iota((GR, T), 0)
        return [jnp.where((row >= DH * j) & (row < DH * (j + 1)), q if j % 2 else rotated, 0.0)
                for j in range(GH)]

    def key_logits(qk, k0, n, tiles):
        weights = jnp.concatenate([_pad_rows(q, GP).astype(BF16) for q in tiles], axis=1)
        return _dot(qk[1][pl.ds(k0, n), :][:, :GP], weights)

    def attention(s, g, jobs, mem_read, v_s, qk):
        lane = _iota((HT, T), 1)
        future = _iota((HT, T), 0) > (lane & (HT - 1))
        head_masks = [jnp.where(future & (lane >= HT), MASKED, 0.0), jnp.where(future & (lane < HT), MASKED, 0.0)]
        low = _iota((8, T), 1) < HT
        row = _iota((8, T), 0)
        acc, top = {}, {}

        @functools.cache
        def shift(i):
            return [max_s[i * GH + j] for j in range(GH)]

        @functools.cache
        def corner_probs(i):
            return [_exp2_shifted(corner_s[i][j // 2][...], jnp.where(low, shift(i)[j], shift(i)[j + 1]))
                    for j in range(0, GH, 2)]

        @functools.cache
        def probs(i, k):
            if k < i:
                return [_exp2_shifted(logit_s[i][j][pl.ds(k * T, T), :], shift(i)[j]).astype(BF16)
                        for j in range(GH)]
            ps = []
            for j in range(GH):
                head = _exp2_shifted(logit_s[i][j][pl.ds(i * T, HT), :], shift(i)[j])
                tail = jnp.where(lane >= HT if j % 2 else lane < HT, corner_probs(i)[j // 2], 0.0)
                ps.append(jnp.concatenate([head, tail], axis=0).astype(BF16))
            return ps

        @functools.cache
        def queries(i):
            return query_tiles(i, qk[0])

        def raise_top(i, j, m):
            top[i, j] = jnp.maximum(top[i, j], m) if (i, j) in top else m

        for job in jobs.split():
            kind, i, k = job[0], *(int(c) for c in job[1:].ljust(2, "0"))
            if kind == "P":
                for j in range(GH):
                    v = [v_s[pl.ds(16 * j + 8 * c, 8), _lane_tile(k)] for c in range(3)]
                    v[SUM_SLAB[j]] = jnp.where(row == SUM_ROW[j], 1.0, v[SUM_SLAB[j]])
                    o = _dot(jnp.concatenate(v, axis=0), probs(i, k)[j])
                    acc[i, j] = acc[i, j] + o if (i, j) in acc else o
            elif kind == "E":
                o = [acc[i, j] if j % 2 else pltpu.roll(acc[i, j], HT, 1) for j in range(GH)]
                o = [[oj[8 * c:8 * c + 8] for c in range(3)] for oj in o]
                den = mem_read[GR:GP, i * T:(i + 1) * T] + 1e-6 if s > 0 else jnp.ones((8, T), F32)
                for j in range(GH):
                    den = jnp.where(row == SUM_ROW[j], o[j][SUM_SLAB[j]], den)
                scale = mix_s[g] / den

                def per_head(rows):
                    return _merge_heads([[jnp.broadcast_to(scale[r:r + 1], (8, T))] * 3 for r in rows])

                mixed = _merge_heads(o) * per_head(SUM_ROW)
                if s > 0:
                    mixed = mixed + mem_read[0:GR, i * T:(i + 1) * T] * per_head(range(DEN_ROW, DEN_ROW + GH))
                ot_s[s][_ds(g * GP, GP, 16), _lane_tile(i)] = _pad_rows(mixed, GP).astype(BF16)
            elif kind == "L":
                diagonal = k >= i - 1
                n = i * T + HT - k * T if diagonal else T
                if v_s is not None:
                    probs(i, k)
                    if diagonal:
                        probs(i, i)
                st = key_logits(qk, k * T, n, queries(i))
                for j in range(GH):
                    sj = st[:, j * T:(j + 1) * T]
                    if diagonal:
                        end = sj[n - HT:] + head_masks[j % 2]
                        sj = end if n == HT else jnp.concatenate([sj[:n - HT], end], axis=0)
                    logit_s[i][j][pl.ds(k * T, n), :] = sj
                    raise_top(i, j, _rows_max(sj))
            elif kind == "C":
                if v_s is not None:
                    corner_probs(i)
                q = query_tiles(i, qk[0])
                first = _iota((GR, T), 1) < HT
                st = key_logits(qk, i * T + HT, HT, [jnp.where(first, q[j], q[j + 1]) for j in range(0, GH, 2)])
                for j in range(0, GH, 2):
                    sj = st[:, j // 2 * T:(j // 2 + 1) * T] + jnp.where(future, MASKED, 0.0)
                    corner_s[i][j // 2][...] = sj
                    m = _rows_max(sj)
                    raise_top(i, j, jnp.where(low, m, -jnp.inf))
                    raise_top(i, j + 1, jnp.where(low, -jnp.inf, m))
            elif kind == "M":
                if v_s is not None:
                    shift(i)
                for j in range(GH):
                    max_s[i * GH + j] = jnp.broadcast_to(jnp.max(top[i, j], axis=0, keepdims=True), (8, T))

    def route():
        r = _rnd(jnp.concatenate([score_s[s] for s in range(NSEG)], axis=1))
        r = jnp.clip(jnp.where(jnp.abs(r) < F32_TINY, F32_TINY, r), -BF16_MAX, BF16_MAX)
        tok = _iota((8, S), 1)
        key = pltpu.bitcast(pltpu.bitcast(r, jnp.int32) | jnp.where(r > 0, S - 1 - tok, tok), F32)
        k0 = jnp.max(key, axis=1, keepdims=True)
        k1 = jnp.max(jnp.where(key == k0, -jnp.inf, key), axis=1, keepdims=True)
        best = jnp.broadcast_to(jnp.where(_iota((8, 1), 0) == 0, k0, k1), (8, T))
        bits = pltpu.bitcast(best, jnp.int32)
        pos = jnp.where(best > 0, S - 1 - (bits & (S - 1)), bits & (S - 1))
        return (pos[0, 0], pos[1, 0]), jax.nn.sigmoid(pltpu.bitcast(bits & -(1 << 16), F32))

    def gather(idx):
        xs = jnp.zeros((8, DP), F32)
        for c in range(2):
            tile = xn_s[idx[c] // L, :, _lane_tile((idx[c] % L) // T)]
            hot = ((_iota((8, T), 1) == idx[c] % T) & (_iota((8, T), 0) == c)).astype(F32)
            xs = xs + _dot_nt(hot, tile)
        xsel_s[...] = jnp.concatenate([xs[:, g * GP:g * GP + GR] for g in range(NG)], axis=1)
        y_s[...] = jnp.zeros((8, DP), F32)

    def gate_up_jobs(p):
        n = F // T // NP
        pre = {}

        def last_rows(m):
            rows = pl.ds(4 * T, D - 4 * T)
            pre[m] = _dot(xsel_s[:, rows], (wg_s, wu_s)[m][rows, _ds(p * n * T, n * T, T)])

        def first_rows(t, m):
            rows, cols = pl.ds(0, 4 * T), _lane_tile(p * n + t)
            pre[m, t] = _dot(xsel_s[:, rows], (wg_s, wu_s)[m][rows, cols]) + pre[m][:, t * T:(t + 1) * T]
            if m == 1:
                h_s[:, cols] = pre[0, t] * jax.nn.sigmoid(pre[0, t]) * pre[1, t]

        return ([functools.partial(last_rows, m) for m in range(2)]
                + [functools.partial(first_rows, t, m) for t in range(n) for m in range(2)])

    def down_jobs(p):
        n = F // T // (NP - 1)

        def piece(c, d):
            rows, cols = pl.ds(d * T, min(T, D - d * T)), _ds((p * n + 4 * c) * T, 4 * T, T)
            y_s[:, rows] += _dot_nt(h_s[:, cols], wd_s[rows, cols])

        return [functools.partial(piece, c, d) for c in range(n // 4) for d in range(DP // T)]

    def place_updates(idx, r_sel):
        yt = _pad_rows(y_s[...] * jnp.concatenate([r_sel] * (DP // T), axis=1), T).T[:D]
        for c in range(2):
            upd = pltpu.roll(yt, (idx[c] + T - c) % T, 1)
            upd_s[c] = jnp.where(_iota((D, T), 1) == idx[c] % T, upd, 0.0).reshape(NG, GR, T)

    def add_updates(idx):
        for c in range(2):
            s, lanes = idx[c] // L, _lane_tile((idx[c] % L) // T)

            @pl.when(s < NSEG - 1)
            def _():
                out_s[s, :, :, lanes] = (out_s[s, :, :, lanes].astype(F32) + upd_s[c]).astype(BF16)

    def step(s, p, last=False):
        fillers = []
        if s == NSEG - 2:
            fillers = gate_up_jobs(p)
        elif s == NSEG - 1 and not last:
            fillers = down_jobs(p)
        reads = [memory(s, 2 * p + e, qkv_s[e]) for e in range(2)]
        v_held[...] = qkv_s[1][2][...]
        attention(s, 2 * p, JOBS_A, reads[0], qkv_s[0][2], qkv_s[1])
        if not last:
            nxt = s * NP + p + 1
            project(nxt // NP, nxt % NP, fillers)
            if s == 0:
                layer_norm_background(NT + 2 * p)
                layer_norm_background(NT + 2 * p + 1)
                for e in range(3):
                    transpose_w(jnp.where(p < 2, e, 3),
                                jnp.where(p < 2, p + 3, jnp.minimum(3 * (p - 2) + e, 4)))
            elif s == 1:
                layer_norm_background(3 * NT + p)
            attention(s, 2 * p + 1, JOBS_B[s], reads[1], v_held, qkv_s[0])
        if s > 0:
            out_project(s - 1, p, fillers)
        assert not fillers
        return reads[1]

    def first_dot(i):
        return _dot(wt_s[i, pair_rows(0), :], xn_s[0])

    zero_s[0] = 0
    for t in range(NT):
        x_copy(t, 1).start()
    for t in range(NT):
        x_copy(t, 1).wait()
        if t < 3:
            w_copy((1, 0, 2)[t], 0).start()
        if t == 2:
            wr_copy.start()
            beta_copy.start()
        layer_norm_now(t)
    w_copy(1, 0).wait()
    for c in range(2):
        transpose_w(1, c)
    w_copy(0, 0).wait()
    for i in range(3):
        w_copy(i, 1).start()
    kt = first_dot(1)
    for c in range(2):
        transpose_w(0, c)
    w_copy(2, 0).wait()
    wr_copy.wait()
    beta_copy.wait()
    x_copy(NT, NT).start()
    for i in range(3):
        w_copy(i, 2).start()
    keep(1, kt)
    keep(0, first_dot(0))
    for c in range(2):
        transpose_w(2, c)
    make_mix()
    router_s[...] = _pad_groups(jnp.broadcast_to(wr_s[...].astype(F32).reshape(1, D), (8, D)), 1)
    for i in range(3):
        w_copy(i, 1).wait()
    for i in range(3):
        w_copy(i, 3).start()
    x_copy(2 * NT, NT).start()
    wo_copy.start()
    x_copy(3 * NT, NT).start()
    keep(2, first_dot(2))
    score_s[0] = _dot(router_s[...], xn_s[0])
    attention(0, 0, JOBS_FIRST, None, None, qkv_s[0])
    for i in range(3):
        transpose_w(i, 2)
    x_copy(NT, NT).wait()
    for i in range(3):
        w_copy(i, 2).wait()

    for s in range(NSEG):
        def body(p, carry, s=s):
            if s == 0:
                @pl.when(p == 1)
                def _():
                    for i in range(3):
                        w_copy(i, 3).wait()
                    x_copy(2 * NT, NT).wait()
                    wo_copy.wait()
                    x_copy(3 * NT, NT).wait()
                    for i in range(3):
                        ffn_copy(i).start()
            if s >= 2:
                pl.when(p == 1)(lambda: segment_store(s - 2).start())
            step(s, p)
            return carry

        lax.fori_loop(0, NP if s < NSEG - 1 else NP - 1, body, 0)
        if s == 1:
            for i in range(3):
                ffn_copy(i).wait()
            idx, r_sel = route()
            gather(idx)

    s = NSEG - 1
    place_updates(idx, r_sel)
    mem_read = step(s, NP - 1, last=True)
    attention(s, NG - 1, "P00 E0", mem_read, v_held, None)
    segment_store(0).wait()
    segment_store(1).wait()
    add_updates(idx)
    segment_store(2).start()
    tiles = [i // T for i in idx]
    again = [tiles[0] < 2 * NT, (tiles[1] < 2 * NT) & (tiles[1] != tiles[0])]
    for c in range(2):
        pl.when(again[c])(lambda c=c: tile_store(tiles[c], NT + c).start())
    for t in range(NT):
        if t + 1 < NT:
            jobs = " ".join(f"P{t + 1}{k}" for k in range(t + 2)) + f" E{t + 1}"
            attention(s, NG - 1, jobs, mem_read, v_held, None)
        lanes = _lane_tile(t)
        a = _dot(wt_s[3, pl.ds(0, D), :], ot_s[s][:, lanes]).reshape(NG, GR, T)
        for c in range(2):
            a = a + jnp.where(tiles[c] == s * NT + t, upd_s[c], 0.0)
        for g in range(NG):
            out_s[s, g, :, lanes] = (residual(s, g, lanes) + a[g]).astype(BF16)
        tile_store(s * NT + t, t).start()
    for c in range(2):
        pl.when(again[c])(lambda c=c: tile_store(tiles[c], NT + c).wait())
    segment_store(2).wait()
    for t in range(NT):
        tile_store(s * NT + t, t).wait()


@jax.jit
def pallas_parallel_sum__memory_aug_infini_attn__moe_arch_mod__prompt_kernel(
    A_x, A_wq, A_wk, A_wv, A_wo, A_beta, B_x, B_w_r, B_w_gate, B_w_up, B_w_down,
):
    del B_x
    hbm = pl.BlockSpec(memory_space=pltpu.HBM)
    group = (pltpu.VMEM((GR, L), F32),
             pltpu.VMEM((L, T), BF16),
             pltpu.VMEM((GR, L), F32),
             pltpu.VMEM((GR, L), F32),
             pltpu.VMEM((L, T), BF16))
    out = pl.pallas_call(
        _kernel,
        out_shape=jax.ShapeDtypeStruct((NG, GR, S), BF16),
        in_specs=[hbm] * 10,
        out_specs=hbm,
        scratch_shapes=[
            pltpu.VMEM((NSEG, NG, GR, L), BF16),
            pltpu.VMEM((4, D, D), BF16),
            pltpu.VMEM((H,), BF16),
            pltpu.VMEM((D,), BF16),
            pltpu.VMEM((D, F), BF16),
            pltpu.VMEM((D, F), BF16),
            pltpu.VMEM((D, F), BF16),
            pltpu.VMEM((NSEG, DP, L), BF16),
            pltpu.VMEM((4, DP, DP), BF16),
            pltpu.VMEM((8, DP), F32),
            pltpu.VMEM((NG, 8, T), F32),
            pltpu.VMEM((NG, GP, T), F32),
            [pltpu.VMEM((DP, L), BF16)] * NSEG,
            pltpu.VMEM((NSEG, NG, GR, L), BF16),
            (group, group),
            pltpu.VMEM((GR, L), F32),
            [[pltpu.VMEM((i * T + HT, T), F32)] * GH for i in range(NT)],
            [[pltpu.VMEM((HT, T), F32)] * (GH // 2)] * NT,
            pltpu.VMEM((NT * GH, 8, T), F32),
            pltpu.VMEM((NSEG, 8, L), F32),
            pltpu.VMEM((8, D), F32),
            pltpu.VMEM((8, F), F32),
            pltpu.VMEM((8, DP), F32),
            pltpu.VMEM((2, NG, GR, T), F32),
            pltpu.VMEM((2, 8, T), F32),
            pltpu.SMEM((1,), jnp.int32),
            pltpu.SemaphoreType.DMA((NSEG * NT,)),
            pltpu.SemaphoreType.DMA((12,)),
            pltpu.SemaphoreType.DMA((15,)),
        ],
        compiler_params=pltpu.CompilerParams(vmem_limit_bytes=100 * 1024 * 1024),
        name="infini_mod",
    )(jnp.transpose(A_x[0]).reshape(NG, GR, S), A_wq, A_wk, A_wv, A_wo, A_beta, B_w_r,
      B_w_gate, B_w_up, jnp.transpose(B_w_down))
    return jnp.transpose(out.reshape(D, S))[None]
```

```python
import functools

import jax
import jax.numpy as jnp
import numpy as np
from jax import lax
import jax.experimental.pallas as pl
import jax.experimental.pallas.tpu as pltpu

D = 576
S = 2048
H = 32
DH = 18
NSEG = 4
L = 512
F = 4608
NG = 8
NP = NG // 2
GH = 4
GR = 72
GP = 80
DP = NG * GP
T = 128
HT = T // 2
NT = L // T

F32 = jnp.float32
BF16 = jnp.bfloat16
QSCALE = float(DH ** -0.5 * np.log2(np.e))
LN_EPS = float(np.asarray(1e-5, dtype=jnp.bfloat16).astype(np.float32))
MASKED = -1e30
F32_TINY = float(np.finfo(np.float32).tiny)
BF16_MAX = float(jnp.finfo(jnp.bfloat16).max)

SUM_SLAB = (2, 2, 2, 0)
SUM_ROW = (5, 6, 7, 0)
DEN_ROW = 1

JOBS_A = "L30 P30 L31 P31 L32 P32 P33 E3 L20 P20 L21 P21 P22 E2 L10 P10 P11 E1 L00 P00 E0 C3 M3 C2 M2 C1 M1 C0 M0"
JOBS_B = (
    "P33 L30 P30 L31 P31 L32 P32 E3 P22 L20 P20 L21 P21 E2 P11 L10 P10 E1 L00 P00 E0 C3 M3 C2 M2 C1 M1 C0 M0",
    "L00 P00 E0 L30 P30 L31 P31 L32 P32 P33 E3 L20 P20 L21 P21 P22 E2 L10 P10 C3 C2 P11 E1 C1 C0 M3 M2 M1 M0",
    "P11 L10 P10 E1 L00 P00 E0 P33 L30 P30 L31 P31 C1 C0 L32 P32 E3 C3 C2 P22 L20 P20 L21 P21 E2 M3 M2 M1 M0",
    "L00 P00 E0 L30 P30 L31 P31 L32 P32 P33 E3 L20 P20 L21 P21 P22 E2 L10 P10 C3 C2 P11 E1 C1 C0 M3 M2 M1 M0",
)
JOBS_FIRST = "L30 L31 L32 L20 L21 L10 L00 C3 M3 C2 M2 C1 M1 C0 M0"


def _rnd(x):
    return x.astype(BF16).astype(F32)


def _dot(a, b):
    return lax.dot_general(a, b, (((1,), (0,)), ((), ())), preferred_element_type=F32)


def _dot_nt(a, b):
    return lax.dot_general(a, b, (((1,), (1,)), ((), ())), preferred_element_type=F32)


def _phi(t):
    return jnp.where(t > 0, t + 1.0, jnp.exp(t))


def _iota(shape, axis):
    return lax.broadcasted_iota(jnp.int32, shape, axis)


def _head_of(i):
    return (i * 57) >> 10


def _ds(i, n, align):
    return pl.ds(i if isinstance(i, int) else pl.multiple_of(i, align), n)


def _lane_tile(t):
    return _ds(t * T, T, T)


def _rows_max(x):
    return jnp.max(x.reshape(x.shape[0] // 8, 8, T), axis=0)


def _exp2_shifted(x, m):
    return jnp.exp2(x.reshape(x.shape[0] // 8, 8, T) - m[None]).reshape(x.shape)


def _pad_rows(x, n):
    return jnp.concatenate([x, jnp.zeros((n - x.shape[0], x.shape[1]), x.dtype)], axis=0)


def _pad_groups(x, axis):
    zeros = jnp.zeros_like(lax.slice_in_dim(x, 0, GP - GR, axis=axis))
    parts = []
    for g in range(NG):
        parts += [lax.slice_in_dim(x, g * GR, (g + 1) * GR, axis=axis), zeros]
    return jnp.concatenate(parts, axis=axis)


def _merge_heads(w):
    row = _iota((8, T), 0)
    return jnp.concatenate([
        w[0][0], w[0][1], jnp.where(row < 2, w[0][2], w[1][0]),
        w[1][1], jnp.where(row < 4, w[1][2], w[2][0]),
        w[2][1], jnp.where(row < 6, w[2][2], w[3][0]),
        w[3][1], w[3][2]], axis=0)


def _kernel(x_hbm, wq_hbm, wk_hbm, wv_hbm, wo_hbm, beta_hbm, wr_hbm, wg_hbm, wu_hbm, wd_hbm,
            out_hbm,
            x_s, w_s, beta_s, wr_s, wg_s, wu_s, wd_s,
            xn_s, wt_s, router_s, mix_s, mem_s, ot_s, out_s,
            qkv_s, v_held, logit_s, corner_s, max_s,
            score_s, xsel_s, h_s, y_s, upd_s, stat_s, zero_s,
            x_sems, w_sems, sems):
    w_hbm = (wq_hbm, wk_hbm, wv_hbm)

    def x_copy(t0, n):
        return pltpu.make_async_copy(x_hbm.at[:, :, pl.ds(t0 * T, n * T)],
                                     x_s.at[t0 // NT, :, :, pl.ds(t0 % NT * T, n * T)], x_sems.at[t0])

    def w_copy(i, c):
        cols = pl.ds(0, 2 * T) if c == 0 else pl.ds((c + 1) * T, min(T, D - (c + 1) * T))
        return pltpu.make_async_copy(w_hbm[i].at[:, cols], w_s.at[i, :, cols], w_sems.at[4 * i + c])

    def ffn_copy(i):
        return pltpu.make_async_copy((wg_hbm, wu_hbm, wd_hbm)[i], (wg_s, wu_s, wd_s)[i], sems.at[i])

    def segment_store(s):
        return pltpu.make_async_copy(out_s.at[s], out_hbm.at[:, :, pl.ds(s * L, L)], sems.at[3 + s])

    def tile_store(n, sem):
        return pltpu.make_async_copy(out_s.at[n // NT, :, :, _lane_tile(n % NT)],
                                     out_hbm.at[:, :, _lane_tile(n)], sems.at[6 + sem])

    wo_copy = pltpu.make_async_copy(wo_hbm, w_s.at[3], sems.at[12])
    wr_copy = pltpu.make_async_copy(wr_hbm, wr_s, sems.at[13])
    beta_copy = pltpu.make_async_copy(beta_hbm, beta_s, sems.at[14])

    def make_mix():
        gate = jnp.broadcast_to(jax.nn.sigmoid(beta_s[...].astype(F32)).reshape(1, H), (8, H))
        row = _iota((8, H), 0)
        head = row - DEN_ROW
        for j in range(GH):
            head = jnp.where(row == SUM_ROW[j], j, head)
        weight = jnp.where(head == row - DEN_ROW, gate, 1.0 - gate)
        for g in range(NG):
            col = jnp.sum(jnp.where(head + g * GH == _iota((8, H), 1), weight, 0.0), axis=1, keepdims=True)
            mix_s[g] = jnp.broadcast_to(col, (8, T))

    def transpose_w(i, c):
        parts = []
        for g in range(NG):
            parts += [w_s[i, pl.ds(g * GR, GR), _lane_tile(c)], jnp.zeros((GP - GR, T), BF16)]
        w = jnp.concatenate(parts, axis=0)
        if not isinstance(c, int):
            w = jnp.where(_iota((DP, T), 1) < D - c * T, w, jnp.zeros_like(w))
        wt_s[i, _lane_tile(c), :] = w.T

    def inv_std(var):
        return 1.0 / _rnd(jnp.sqrt(_rnd(_rnd(var) + LN_EPS)))

    def layer_norm_now(t):
        lanes = _lane_tile(t)

        def x(g):
            return x_s[0, g, :, lanes].astype(F32).reshape(GR // 8, 8, T)

        def mean_of(f):
            acc = f(x(0))
            for g in range(1, NG):
                acc = acc + f(x(g))
            acc = acc[0:3] + acc[3:6] + acc[6:9]
            total = jnp.sum(acc[0] + acc[1] + acc[2], axis=0, keepdims=True)
            return jnp.broadcast_to(total / D, (8, T))

        stat_s[0] = mean = mean_of(lambda v: v)
        stat_s[1] = var = mean_of(lambda v: (v - mean[None]) * (v - mean[None]))
        mean, inv = _rnd(mean), inv_std(var)
        for g in range(NG):
            xn = (_rnd(x(g) - mean[None]) * inv[None]).reshape(GR, T)
            xn_s[0, pl.ds(g * GP, GP), lanes] = _pad_rows(xn, GP).astype(BF16)

    def layer_norm_background(n):
        s, lanes = n // NT, _lane_tile(n % NT)
        x = x_s[s, :, :, lanes].astype(F32).reshape(D, T)
        mean = jnp.sum(x, axis=0, keepdims=True) / D
        var = jnp.sum((x - mean) * (x - mean), axis=0, keepdims=True) / D
        mean = jnp.broadcast_to(_rnd(mean), (8, T))
        inv = jnp.broadcast_to(inv_std(var), (8, T))
        never = _iota((8, T), 0) < zero_s[0]
        slabs = []
        for c in range(0, D, 8):
            slabs.append(_rnd(x[c:c + 8] - mean) * inv)
            mean = jnp.where(never, slabs[-1], mean)
        xn_s[s, :, lanes] = _pad_groups(jnp.concatenate(slabs, axis=0), 0).astype(BF16)
        score_s[s, :, lanes] = _dot(router_s[...], xn_s[s, :, lanes])

    def pair_rows(p):
        return _ds(p * 2 * GR, 2 * GR, 16)

    def weight_dot(i, p, rhs, fillers):
        fillers = fillers or [lambda: None] * (NT + 1)
        rest = _dot(wt_s[i, pair_rows(p), pl.ds(4 * T, T)], rhs(pl.ds(4 * T, T), slice(None)))
        fillers.pop(0)()
        parts = []
        for t in range(NT):
            parts.append(_dot(wt_s[i, pair_rows(p), pl.ds(0, 4 * T)], rhs(pl.ds(0, 4 * T), _lane_tile(t))))
            fillers.pop(0)()
        return jnp.concatenate(parts, axis=1) + rest

    def keep(i, val):
        for e, (q_s, k_s, v_s, pq_s, pk_s) in enumerate(qkv_s):
            part = val[e * GR:(e + 1) * GR]
            if i == 0:
                q_s[...] = part * QSCALE
                pq_s[...] = _phi(part)
            elif i == 1:
                k = _pad_rows(part, T).T
                k_s[...] = k.astype(BF16)
                pk_s[...] = _phi(k).astype(BF16)
            else:
                v_s[...] = part

    def project(s, p, fillers):
        if fillers:
            for i in (1, 0, 2):
                keep(i, weight_dot(i, p, lambda r, c: xn_s[s, r, c], fillers))
        else:
            qkv = _dot(jnp.concatenate([wt_s[i, pair_rows(p), :] for i in range(3)], axis=0), xn_s[s])
            for i in range(3):
                keep(i, qkv[i * 2 * GR:(i + 1) * 2 * GR])

    def residual(s, g, lanes):
        return x_s[s, g, :, lanes].astype(F32) + xn_s[s, _ds(g * GP, GP, 16), lanes].astype(F32)[:GR]

    def out_project(s, p, fillers):
        a = weight_dot(3, p, lambda r, c: ot_s[s][r, c], fillers)
        for e in range(2):
            out_s[s, 2 * p + e] = (residual(s, 2 * p + e, slice(None)) + a[e * GR:(e + 1) * GR]).astype(BF16)

    def memory(s, g, buf):
        _, _, v_s, pq_s, pk_s = buf
        read = None
        if s > 0:
            row, col = _iota((GP, T), 0), _iota((GP, T), 1)
            row_head = jnp.where(row < GR, _head_of(row), row - (GR + DEN_ROW))
            m = jnp.where((row_head == _head_of(col)) & (col < GR), mem_s[g], 0.0)
            read = _dot(m.astype(BF16), _pad_rows(pq_s[...], T).astype(BF16))
        if s < NSEG - 1:
            v1 = jnp.concatenate([v_s[...], jnp.ones((GP - GR, L), F32)], axis=0)
            update = _dot(v1.astype(BF16), pk_s[...])
            mem_s[g] = mem_s[g] + update if s > 0 else update
        return read

    def query_tiles(i, q_s):
        q = q_s[:, _lane_tile(i)]
        rotated = pltpu.roll(q, HT, 1)
        row = _iota((GR, T), 0)
        return [jnp.where((row >= DH * j) & (row < DH * (j + 1)), q if j % 2 else rotated, 0.0)
                for j in range(GH)]

    def key_logits(qk, k0, n, tiles):
        weights = jnp.concatenate([_pad_rows(q, GP).astype(BF16) for q in tiles], axis=1)
        return _dot(qk[1][pl.ds(k0, n), :][:, :GP], weights)

    def attention(s, g, jobs, mem_read, v_s, qk):
        lane = _iota((HT, T), 1)
        future = _iota((HT, T), 0) > (lane & (HT - 1))
        head_masks = [jnp.where(future & (lane >= HT), MASKED, 0.0), jnp.where(future & (lane < HT), MASKED, 0.0)]
        low = _iota((8, T), 1) < HT
        row = _iota((8, T), 0)
        acc, top = {}, {}

        @functools.cache
        def shift(i):
            return [max_s[i * GH + j] for j in range(GH)]

        @functools.cache
        def corner_probs(i):
            return [_exp2_shifted(corner_s[i][j // 2][...], jnp.where(low, shift(i)[j], shift(i)[j + 1]))
                    for j in range(0, GH, 2)]

        @functools.cache
        def probs(i, k):
            if k < i:
                return [_exp2_shifted(logit_s[i][j][pl.ds(k * T, T), :], shift(i)[j]).astype(BF16)
                        for j in range(GH)]
            ps = []
            for j in range(GH):
                head = _exp2_shifted(logit_s[i][j][pl.ds(i * T, HT), :], shift(i)[j])
                tail = jnp.where(lane >= HT if j % 2 else lane < HT, corner_probs(i)[j // 2], 0.0)
                ps.append(jnp.concatenate([head, tail], axis=0).astype(BF16))
            return ps

        @functools.cache
        def queries(i):
            return query_tiles(i, qk[0])

        def raise_top(i, j, m):
            top[i, j] = jnp.maximum(top[i, j], m) if (i, j) in top else m

        for job in jobs.split():
            kind, i, k = job[0], *(int(c) for c in job[1:].ljust(2, "0"))
            if kind == "P":
                for j in range(GH):
                    v = [v_s[pl.ds(16 * j + 8 * c, 8), _lane_tile(k)] for c in range(3)]
                    v[SUM_SLAB[j]] = jnp.where(row == SUM_ROW[j], 1.0, v[SUM_SLAB[j]])
                    o = _dot(jnp.concatenate(v, axis=0), probs(i, k)[j])
                    acc[i, j] = acc[i, j] + o if (i, j) in acc else o
            elif kind == "E":
                o = [acc[i, j] if j % 2 else pltpu.roll(acc[i, j], HT, 1) for j in range(GH)]
                o = [[oj[8 * c:8 * c + 8] for c in range(3)] for oj in o]
                den = mem_read[GR:GP, i * T:(i + 1) * T] + 1e-6 if s > 0 else jnp.ones((8, T), F32)
                for j in range(GH):
                    den = jnp.where(row == SUM_ROW[j], o[j][SUM_SLAB[j]], den)
                scale = mix_s[g] / den

                def per_head(rows):
                    return _merge_heads([[jnp.broadcast_to(scale[r:r + 1], (8, T))] * 3 for r in rows])

                mixed = _merge_heads(o) * per_head(SUM_ROW)
                if s > 0:
                    mixed = mixed + mem_read[0:GR, i * T:(i + 1) * T] * per_head(range(DEN_ROW, DEN_ROW + GH))
                ot_s[s][_ds(g * GP, GP, 16), _lane_tile(i)] = _pad_rows(mixed, GP).astype(BF16)
            elif kind == "L":
                diagonal = k >= i - 1
                n = i * T + HT - k * T if diagonal else T
                if v_s is not None:
                    probs(i, k)
                    if diagonal:
                        probs(i, i)
                st = key_logits(qk, k * T, n, queries(i))
                for j in range(GH):
                    sj = st[:, j * T:(j + 1) * T]
                    if diagonal:
                        end = sj[n - HT:] + head_masks[j % 2]
                        sj = end if n == HT else jnp.concatenate([sj[:n - HT], end], axis=0)
                    logit_s[i][j][pl.ds(k * T, n), :] = sj
                    raise_top(i, j, _rows_max(sj))
            elif kind == "C":
                if v_s is not None:
                    corner_probs(i)
                q = query_tiles(i, qk[0])
                first = _iota((GR, T), 1) < HT
                st = key_logits(qk, i * T + HT, HT, [jnp.where(first, q[j], q[j + 1]) for j in range(0, GH, 2)])
                for j in range(0, GH, 2):
                    sj = st[:, j // 2 * T:(j // 2 + 1) * T] + jnp.where(future, MASKED, 0.0)
                    corner_s[i][j // 2][...] = sj
                    m = _rows_max(sj)
                    raise_top(i, j, jnp.where(low, m, -jnp.inf))
                    raise_top(i, j + 1, jnp.where(low, -jnp.inf, m))
            elif kind == "M":
                if v_s is not None:
                    shift(i)
                for j in range(GH):
                    max_s[i * GH + j] = jnp.broadcast_to(jnp.max(top[i, j], axis=0, keepdims=True), (8, T))

    def route():
        r = _rnd(jnp.concatenate([score_s[s] for s in range(NSEG)], axis=1))
        r = jnp.clip(jnp.where(jnp.abs(r) < F32_TINY, F32_TINY, r), -BF16_MAX, BF16_MAX)
        tok = _iota((8, S), 1)
        key = pltpu.bitcast(pltpu.bitcast(r, jnp.int32) | jnp.where(r > 0, S - 1 - tok, tok), F32)
        k0 = jnp.max(key, axis=1, keepdims=True)
        k1 = jnp.max(jnp.where(key == k0, -jnp.inf, key), axis=1, keepdims=True)
        best = jnp.broadcast_to(jnp.where(_iota((8, 1), 0) == 0, k0, k1), (8, T))
        bits = pltpu.bitcast(best, jnp.int32)
        pos = jnp.where(best > 0, S - 1 - (bits & (S - 1)), bits & (S - 1))
        return (pos[0, 0], pos[1, 0]), jax.nn.sigmoid(pltpu.bitcast(bits & -(1 << 16), F32))

    def gather(idx):
        xs = jnp.zeros((8, DP), F32)
        for c in range(2):
            tile = xn_s[idx[c] // L, :, _lane_tile((idx[c] % L) // T)]
            hot = ((_iota((8, T), 1) == idx[c] % T) & (_iota((8, T), 0) == c)).astype(F32)
            xs = xs + _dot_nt(hot, tile)
        xsel_s[...] = jnp.concatenate([xs[:, g * GP:g * GP + GR] for g in range(NG)], axis=1)
        y_s[...] = jnp.zeros((8, DP), F32)

    def gate_up_jobs(p):
        n = F // T // NP
        pre = {}

        def last_rows(m):
            rows = pl.ds(4 * T, D - 4 * T)
            pre[m] = _dot(xsel_s[:, rows], (wg_s, wu_s)[m][rows, _ds(p * n * T, n * T, T)])

        def first_rows(t, m):
            rows, cols = pl.ds(0, 4 * T), _lane_tile(p * n + t)
            pre[m, t] = _dot(xsel_s[:, rows], (wg_s, wu_s)[m][rows, cols]) + pre[m][:, t * T:(t + 1) * T]
            if m == 1:
                h_s[:, cols] = pre[0, t] * jax.nn.sigmoid(pre[0, t]) * pre[1, t]

        return ([functools.partial(last_rows, m) for m in range(2)]
                + [functools.partial(first_rows, t, m) for t in range(n) for m in range(2)])

    def down_jobs(p):
        n = F // T // (NP - 1)

        def piece(c, d):
            rows, cols = pl.ds(d * T, min(T, D - d * T)), _ds((p * n + 4 * c) * T, 4 * T, T)
            y_s[:, rows] += _dot_nt(h_s[:, cols], wd_s[rows, cols])

        return [functools.partial(piece, c, d) for c in range(n // 4) for d in range(DP // T)]

    def place_updates(idx, r_sel):
        yt = _pad_rows(y_s[...] * jnp.concatenate([r_sel] * (DP // T), axis=1), T).T[:D]
        for c in range(2):
            upd = pltpu.roll(yt, (idx[c] + T - c) % T, 1)
            upd_s[c] = jnp.where(_iota((D, T), 1) == idx[c] % T, upd, 0.0).reshape(NG, GR, T)

    def add_updates(idx):
        for c in range(2):
            s, lanes = idx[c] // L, _lane_tile((idx[c] % L) // T)

            @pl.when(s < NSEG - 1)
            def _():
                out_s[s, :, :, lanes] = (out_s[s, :, :, lanes].astype(F32) + upd_s[c]).astype(BF16)

    def step(s, p, last=False):
        fillers = []
        if s == NSEG - 2:
            fillers = gate_up_jobs(p)
        elif s == NSEG - 1 and not last:
            fillers = down_jobs(p)
        reads = [memory(s, 2 * p + e, qkv_s[e]) for e in range(2)]
        v_held[...] = qkv_s[1][2][...]
        attention(s, 2 * p, JOBS_A, reads[0], qkv_s[0][2], qkv_s[1])
        if not last:
            nxt = s * NP + p + 1
            project(nxt // NP, nxt % NP, fillers)
            if s == 0:
                layer_norm_background(NT + 2 * p)
                layer_norm_background(NT + 2 * p + 1)
                for e in range(3):
                    transpose_w(jnp.where(p < 2, e, 3),
                                jnp.where(p < 2, p + 3, jnp.minimum(3 * (p - 2) + e, 4)))
            elif s == 1:
                layer_norm_background(3 * NT + p)
            attention(s, 2 * p + 1, JOBS_B[s], reads[1], v_held, qkv_s[0])
        if s > 0:
            out_project(s - 1, p, fillers)
        assert not fillers
        return reads[1]

    def first_dot(i, tokens=slice(None)):
        return _dot(wt_s[i, pair_rows(0), :], xn_s[0, :, tokens])

    zero_s[0] = 0
    for t in range(NT):
        x_copy(t, 1).start()
    for t in range(NT):
        x_copy(t, 1).wait()
        if t < 3:
            w_copy((1, 0, 2)[t], 0).start()
        if t == 2:
            wr_copy.start()
            beta_copy.start()
        layer_norm_now(t)
    w_copy(1, 0).wait()
    for i in range(3):
        w_copy(i, 1).start()
    for c in range(2):
        transpose_w(1, c)
    kt = first_dot(1, pl.ds(0, L // 2))
    w_copy(0, 0).wait()
    kt = jnp.concatenate([kt, first_dot(1, pl.ds(L // 2, L // 2))], axis=1)
    for c in range(2):
        transpose_w(0, c)
    w_copy(2, 0).wait()
    wr_copy.wait()
    beta_copy.wait()
    x_copy(NT, NT).start()
    for i in range(3):
        w_copy(i, 2).start()
    keep(1, kt)
    keep(0, first_dot(0))
    for c in range(2):
        transpose_w(2, c)
    make_mix()
    router_s[...] = _pad_groups(jnp.broadcast_to(wr_s[...].astype(F32).reshape(1, D), (8, D)), 1)
    keep(2, first_dot(2))
    for i in range(3):
        w_copy(i, 1).wait()
    for i in range(3):
        w_copy(i, 3).start()
    x_copy(2 * NT, NT).start()
    wo_copy.start()
    x_copy(3 * NT, NT).start()
    score_s[0] = _dot(router_s[...], xn_s[0])
    attention(0, 0, JOBS_FIRST, None, None, qkv_s[0])
    for i in range(3):
        transpose_w(i, 2)
    x_copy(NT, NT).wait()
    for i in range(3):
        w_copy(i, 2).wait()

    for s in range(NSEG):
        def body(p, carry, s=s):
            if s == 0:
                @pl.when(p == 1)
                def _():
                    for i in range(3):
                        w_copy(i, 3).wait()
                    x_copy(2 * NT, NT).wait()
                    wo_copy.wait()
                    x_copy(3 * NT, NT).wait()
                    for i in range(3):
                        ffn_copy(i).start()
            if s >= 2:
                pl.when(p == 1)(lambda: segment_store(s - 2).start())
            step(s, p)
            return carry

        lax.fori_loop(0, NP if s < NSEG - 1 else NP - 1, body, 0)
        if s == 1:
            for i in range(3):
                ffn_copy(i).wait()
            idx, r_sel = route()
            gather(idx)

    s = NSEG - 1
    segment_store(0).wait()
    segment_store(1).wait()
    place_updates(idx, r_sel)
    mem_read = step(s, NP - 1, last=True)
    attention(s, NG - 1, "P00 E0", mem_read, v_held, None)
    add_updates(idx)
    segment_store(2).start()
    tiles = [i // T for i in idx]
    again = [tiles[0] < 2 * NT, (tiles[1] < 2 * NT) & (tiles[1] != tiles[0])]
    for c in range(2):
        pl.when(again[c])(lambda c=c: tile_store(tiles[c], NT + c).start())
    for t in range(NT):
        if t + 1 < NT:
            jobs = " ".join(f"P{t + 1}{k}" for k in range(t + 2)) + f" E{t + 1}"
            attention(s, NG - 1, jobs, mem_read, v_held, None)
        lanes = _lane_tile(t)
        a = _dot(wt_s[3, pl.ds(0, D), pl.ds(0, 4 * T)], ot_s[s][pl.ds(0, 4 * T), lanes])
        a = a + jnp.concatenate([_dot(wt_s[3, pair_rows(q), pl.ds(4 * T, T)], ot_s[s][pl.ds(4 * T, T), lanes])
                                 for q in range(NP)], axis=0)
        a = a.reshape(NG, GR, T)
        for c in range(2):
            a = a + jnp.where(tiles[c] == s * NT + t, upd_s[c], 0.0)
        for g in range(NG):
            out_s[s, g, :, lanes] = (residual(s, g, lanes) + a[g]).astype(BF16)
        tile_store(s * NT + t, t).start()
    for c in range(2):
        pl.when(again[c])(lambda c=c: tile_store(tiles[c], NT + c).wait())
    segment_store(2).wait()
    for t in range(NT):
        tile_store(s * NT + t, t).wait()


@jax.jit
def pallas_parallel_sum__memory_aug_infini_attn__moe_arch_mod__prompt_kernel(
    A_x, A_wq, A_wk, A_wv, A_wo, A_beta, B_x, B_w_r, B_w_gate, B_w_up, B_w_down,
):
    del B_x
    hbm = pl.BlockSpec(memory_space=pltpu.HBM)
    group = (pltpu.VMEM((GR, L), F32),
             pltpu.VMEM((L, T), BF16),
             pltpu.VMEM((GR, L), F32),
             pltpu.VMEM((GR, L), F32),
             pltpu.VMEM((L, T), BF16))
    out = pl.pallas_call(
        _kernel,
        out_shape=jax.ShapeDtypeStruct((NG, GR, S), BF16),
        in_specs=[hbm] * 10,
        out_specs=hbm,
        scratch_shapes=[
            pltpu.VMEM((NSEG, NG, GR, L), BF16),
            pltpu.VMEM((4, D, D), BF16),
            pltpu.VMEM((H,), BF16),
            pltpu.VMEM((D,), BF16),
            pltpu.VMEM((D, F), BF16),
            pltpu.VMEM((D, F), BF16),
            pltpu.VMEM((D, F), BF16),
            pltpu.VMEM((NSEG, DP, L), BF16),
            pltpu.VMEM((4, DP, DP), BF16),
            pltpu.VMEM((8, DP), F32),
            pltpu.VMEM((NG, 8, T), F32),
            pltpu.VMEM((NG, GP, T), F32),
            [pltpu.VMEM((DP, L), BF16)] * NSEG,
            pltpu.VMEM((NSEG, NG, GR, L), BF16),
            (group, group),
            pltpu.VMEM((GR, L), F32),
            [[pltpu.VMEM((i * T + HT, T), F32)] * GH for i in range(NT)],
            [[pltpu.VMEM((HT, T), F32)] * (GH // 2)] * NT,
            pltpu.VMEM((NT * GH, 8, T), F32),
            pltpu.VMEM((NSEG, 8, L), F32),
            pltpu.VMEM((8, D), F32),
            pltpu.VMEM((8, F), F32),
            pltpu.VMEM((8, DP), F32),
            pltpu.VMEM((2, NG, GR, T), F32),
            pltpu.VMEM((2, 8, T), F32),
            pltpu.SMEM((1,), jnp.int32),
            pltpu.SemaphoreType.DMA((NSEG * NT,)),
            pltpu.SemaphoreType.DMA((12,)),
            pltpu.SemaphoreType.DMA((15,)),
        ],
        compiler_params=pltpu.CompilerParams(vmem_limit_bytes=100 * 1024 * 1024),
        name="infini_mod",
    )(jnp.transpose(A_x[0]).reshape(NG, GR, S), A_wq, A_wk, A_wv, A_wo, A_beta, B_w_r,
      B_w_gate, B_w_up, jnp.transpose(B_w_down))
    return jnp.transpose(out.reshape(D, S))[None]
```

```python
import functools

import jax
import jax.numpy as jnp
import numpy as np
from jax import lax
import jax.experimental.pallas as pl
import jax.experimental.pallas.tpu as pltpu

D = 576
S = 2048
H = 32
DH = 18
NSEG = 4
L = 512
F = 4608
NG = 8
NP = NG // 2
GH = 4
GR = 72
GP = 80
DP = NG * GP
T = 128
HT = T // 2
NT = L // T

F32 = jnp.float32
BF16 = jnp.bfloat16
QSCALE = float(DH ** -0.5 * np.log2(np.e))
LN_EPS = float(np.asarray(1e-5, dtype=jnp.bfloat16).astype(np.float32))
MASKED = -1e30
F32_TINY = float(np.finfo(np.float32).tiny)
BF16_MAX = float(jnp.finfo(jnp.bfloat16).max)

SUM_SLAB = (2, 2, 2, 0)
SUM_ROW = (5, 6, 7, 0)
DEN_ROW = 1

JOBS_A = "L30 P30 L31 P31 L32 P32 P33 E3 L20 P20 L21 P21 P22 E2 L10 P10 P11 E1 L00 P00 E0 C3 M3 C2 M2 C1 M1 C0 M0"
JOBS_B = (
    "P33 L30 P30 L31 P31 L32 P32 E3 P22 L20 P20 L21 P21 E2 P11 L10 P10 E1 L00 P00 E0 C3 M3 C2 M2 C1 M1 C0 M0",
    "L00 P00 E0 L30 P30 L31 P31 L32 P32 P33 E3 L20 P20 L21 P21 P22 E2 L10 P10 C3 C2 P11 E1 C1 C0 M3 M2 M1 M0",
    "P11 L10 P10 E1 L00 P00 E0 P33 L30 P30 L31 P31 C1 C0 L32 P32 E3 C3 C2 P22 L20 P20 L21 P21 E2 M3 M2 M1 M0",
    "L00 P00 E0 L30 P30 L31 P31 L32 P32 P33 E3 L20 P20 L21 P21 P22 E2 L10 P10 C3 C2 P11 E1 C1 C0 M3 M2 M1 M0",
)
JOBS_FIRST = "L30 L31 L32 L20 L21 L10 L00 C3 M3 C2 M2 C1 M1 C0 M0"


def _rnd(x):
    return x.astype(BF16).astype(F32)


def _dot(a, b):
    return lax.dot_general(a, b, (((1,), (0,)), ((), ())), preferred_element_type=F32)


def _dot_nt(a, b):
    return lax.dot_general(a, b, (((1,), (1,)), ((), ())), preferred_element_type=F32)


def _phi(t):
    return jnp.where(t > 0, t + 1.0, jnp.exp(t))


def _iota(shape, axis):
    return lax.broadcasted_iota(jnp.int32, shape, axis)


def _head_of(i):
    return (i * 57) >> 10


def _ds(i, n, align):
    return pl.ds(i if isinstance(i, int) else pl.multiple_of(i, align), n)


def _lane_tile(t):
    return _ds(t * T, T, T)


def _rows_max(x):
    return jnp.max(x.reshape(x.shape[0] // 8, 8, T), axis=0)


def _exp2_shifted(x, m):
    return jnp.exp2(x.reshape(x.shape[0] // 8, 8, T) - m[None]).reshape(x.shape)


def _pad_rows(x, n):
    return jnp.concatenate([x, jnp.zeros((n - x.shape[0], x.shape[1]), x.dtype)], axis=0)


def _pad_groups(x, axis):
    zeros = jnp.zeros_like(lax.slice_in_dim(x, 0, GP - GR, axis=axis))
    parts = []
    for g in range(NG):
        parts += [lax.slice_in_dim(x, g * GR, (g + 1) * GR, axis=axis), zeros]
    return jnp.concatenate(parts, axis=axis)


def _merge_heads(w):
    row = _iota((8, T), 0)
    return jnp.concatenate([
        w[0][0], w[0][1], jnp.where(row < 2, w[0][2], w[1][0]),
        w[1][1], jnp.where(row < 4, w[1][2], w[2][0]),
        w[2][1], jnp.where(row < 6, w[2][2], w[3][0]),
        w[3][1], w[3][2]], axis=0)


def _kernel(x_hbm, wq_hbm, wk_hbm, wv_hbm, wo_hbm, beta_hbm, wr_hbm, wg_hbm, wu_hbm, wd_hbm,
            out_hbm,
            x_s, w_s, w_end_s, beta_s, wr_s, wg_s, wu_s, wd_s,
            xn_s, wt_s, router_s, mix_s, mem_s, ot_s, out_s,
            qkv_s, v_held, logit_s, corner_s, max_s,
            score_s, xsel_s, h_s, y_s, upd_s, stat_s, zero_s,
            x_sems, w_sems, sems):
    w_hbm = (wq_hbm, wk_hbm, wv_hbm, wo_hbm)

    def x_copy(t0, n):
        return pltpu.make_async_copy(x_hbm.at[:, :, pl.ds(t0 * T, n * T)],
                                     x_s.at[t0 // NT, :, :, pl.ds(t0 % NT * T, n * T)], x_sems.at[t0])

    def w_copy(i, c):
        if c == 3:
            return pltpu.make_async_copy(w_hbm[i].at[:, pl.ds(4 * T, HT)], w_end_s.at[i], w_sems.at[4 * i + c])
        cols = pl.ds(0, (4 if i == 3 else 2) * T) if c == 0 else _lane_tile(c + 1)
        return pltpu.make_async_copy(w_hbm[i].at[:, cols], w_s.at[i, :, cols], w_sems.at[4 * i + c])

    def ffn_copy(i):
        return pltpu.make_async_copy((wg_hbm, wu_hbm, wd_hbm)[i], (wg_s, wu_s, wd_s)[i], sems.at[i])

    def segment_store(s):
        return pltpu.make_async_copy(out_s.at[s], out_hbm.at[:, :, pl.ds(s * L, L)], sems.at[3 + s])

    def tile_store(n, sem):
        return pltpu.make_async_copy(out_s.at[n // NT, :, :, _lane_tile(n % NT)],
                                     out_hbm.at[:, :, _lane_tile(n)], sems.at[6 + sem])

    wr_copy = pltpu.make_async_copy(wr_hbm, wr_s, sems.at[12])
    beta_copy = pltpu.make_async_copy(beta_hbm, beta_s, sems.at[13])

    def make_mix():
        gate = jnp.broadcast_to(jax.nn.sigmoid(beta_s[...].astype(F32)).reshape(1, H), (8, H))
        row = _iota((8, H), 0)
        head = row - DEN_ROW
        for j in range(GH):
            head = jnp.where(row == SUM_ROW[j], j, head)
        weight = jnp.where(head == row - DEN_ROW, gate, 1.0 - gate)
        for g in range(NG):
            col = jnp.sum(jnp.where(head + g * GH == _iota((8, H), 1), weight, 0.0), axis=1, keepdims=True)
            mix_s[g] = jnp.broadcast_to(col, (8, T))

    def transpose_w(i, c):
        parts = []
        for g in range(NG):
            parts += [w_s[i, pl.ds(g * GR, GR), _lane_tile(c)], jnp.zeros((GP - GR, T), BF16)]
        wt_s[i, _lane_tile(c), :] = jnp.concatenate(parts, axis=0).T

    def inv_std(var):
        return 1.0 / _rnd(jnp.sqrt(_rnd(_rnd(var) + LN_EPS)))

    def layer_norm_now(t):
        lanes = _lane_tile(t)

        def x(g):
            return x_s[0, g, :, lanes].astype(F32).reshape(GR // 8, 8, T)

        def mean_of(f):
            acc = f(x(0))
            for g in range(1, NG):
                acc = acc + f(x(g))
            acc = acc[0:3] + acc[3:6] + acc[6:9]
            total = jnp.sum(acc[0] + acc[1] + acc[2], axis=0, keepdims=True)
            return jnp.broadcast_to(total / D, (8, T))

        stat_s[0] = mean = mean_of(lambda v: v)
        stat_s[1] = var = mean_of(lambda v: (v - mean[None]) * (v - mean[None]))
        mean, inv = _rnd(mean), inv_std(var)
        for g in range(NG):
            xn = (_rnd(x(g) - mean[None]) * inv[None]).reshape(GR, T)
            xn_s[0, pl.ds(g * GP, GP), lanes] = _pad_rows(xn, GP).astype(BF16)

    def layer_norm_background(n):
        s, lanes = n // NT, _lane_tile(n % NT)
        x = x_s[s, :, :, lanes].astype(F32).reshape(D, T)
        mean = jnp.sum(x, axis=0, keepdims=True) / D
        var = jnp.sum((x - mean) * (x - mean), axis=0, keepdims=True) / D
        mean = jnp.broadcast_to(_rnd(mean), (8, T))
        inv = jnp.broadcast_to(inv_std(var), (8, T))
        never = _iota((8, T), 0) < zero_s[0]
        slabs = []
        for c in range(0, D, 8):
            slabs.append(_rnd(x[c:c + 8] - mean) * inv)
            mean = jnp.where(never, slabs[-1], mean)
        xn_s[s, :, lanes] = _pad_groups(jnp.concatenate(slabs, axis=0), 0).astype(BF16)
        score_s[s, :, lanes] = _dot(router_s[...], xn_s[s, :, lanes])

    def pair_rows(p):
        return _ds(p * 2 * GR, 2 * GR, 16)

    def weight_dot(i, p, rhs, fillers):
        fillers = fillers or [lambda: None] * (NT + 1)
        rest = _dot(wt_s[i, pair_rows(p), pl.ds(4 * T, T)], rhs(pl.ds(4 * T, T), slice(None)))
        fillers.pop(0)()
        parts = []
        for t in range(NT):
            parts.append(_dot(wt_s[i, pair_rows(p), pl.ds(0, 4 * T)], rhs(pl.ds(0, 4 * T), _lane_tile(t))))
            fillers.pop(0)()
        return jnp.concatenate(parts, axis=1) + rest

    def keep(i, val):
        for e, (q_s, k_s, v_s, pq_s, pk_s) in enumerate(qkv_s):
            part = val[e * GR:(e + 1) * GR]
            if i == 0:
                q_s[...] = part * QSCALE
                pq_s[...] = _phi(part)
            elif i == 1:
                k = _pad_rows(part, T).T
                k_s[...] = k.astype(BF16)
                pk_s[...] = _phi(k).astype(BF16)
            else:
                v_s[...] = part

    def project(s, p, fillers):
        if fillers:
            for i in (1, 0, 2):
                keep(i, weight_dot(i, p, lambda r, c: xn_s[s, r, c], fillers))
        else:
            qkv = _dot(jnp.concatenate([wt_s[i, pair_rows(p), :] for i in range(3)], axis=0), xn_s[s])
            for i in range(3):
                keep(i, qkv[i * 2 * GR:(i + 1) * 2 * GR])

    def residual(s, g, lanes):
        return x_s[s, g, :, lanes].astype(F32) + xn_s[s, _ds(g * GP, GP, 16), lanes].astype(F32)[:GR]

    def out_project(s, p, fillers):
        a = weight_dot(3, p, lambda r, c: ot_s[s][r, c], fillers)
        for e in range(2):
            out_s[s, 2 * p + e] = (residual(s, 2 * p + e, slice(None)) + a[e * GR:(e + 1) * GR]).astype(BF16)

    def memory(s, g, buf):
        _, _, v_s, pq_s, pk_s = buf
        read = None
        if s > 0:
            row, col = _iota((GP, T), 0), _iota((GP, T), 1)
            row_head = jnp.where(row < GR, _head_of(row), row - (GR + DEN_ROW))
            m = jnp.where((row_head == _head_of(col)) & (col < GR), mem_s[g], 0.0)
            read = _dot(m.astype(BF16), _pad_rows(pq_s[...], T).astype(BF16))
        if s < NSEG - 1:
            v1 = jnp.concatenate([v_s[...], jnp.ones((GP - GR, L), F32)], axis=0)
            update = _dot(v1.astype(BF16), pk_s[...])
            mem_s[g] = mem_s[g] + update if s > 0 else update
        return read

    def query_tiles(i, q_s):
        q = q_s[:, _lane_tile(i)]
        rotated = pltpu.roll(q, HT, 1)
        row = _iota((GR, T), 0)
        return [jnp.where((row >= DH * j) & (row < DH * (j + 1)), q if j % 2 else rotated, 0.0)
                for j in range(GH)]

    def key_logits(qk, k0, n, tiles):
        weights = jnp.concatenate([_pad_rows(q, GP).astype(BF16) for q in tiles], axis=1)
        return _dot(qk[1][pl.ds(k0, n), :][:, :GP], weights)

    def attention(s, g, jobs, mem_read, v_s, qk):
        lane = _iota((HT, T), 1)
        future = _iota((HT, T), 0) > (lane & (HT - 1))
        head_masks = [jnp.where(future & (lane >= HT), MASKED, 0.0), jnp.where(future & (lane < HT), MASKED, 0.0)]
        low = _iota((8, T), 1) < HT
        row = _iota((8, T), 0)
        acc, top = {}, {}

        @functools.cache
        def shift(i):
            return [max_s[i * GH + j] for j in range(GH)]

        @functools.cache
        def corner_probs(i):
            return [_exp2_shifted(corner_s[i][j // 2][...], jnp.where(low, shift(i)[j], shift(i)[j + 1]))
                    for j in range(0, GH, 2)]

        @functools.cache
        def probs(i, k):
            if k < i:
                return [_exp2_shifted(logit_s[i][j][pl.ds(k * T, T), :], shift(i)[j]).astype(BF16)
                        for j in range(GH)]
            ps = []
            for j in range(GH):
                head = _exp2_shifted(logit_s[i][j][pl.ds(i * T, HT), :], shift(i)[j])
                tail = jnp.where(lane >= HT if j % 2 else lane < HT, corner_probs(i)[j // 2], 0.0)
                ps.append(jnp.concatenate([head, tail], axis=0).astype(BF16))
            return ps

        @functools.cache
        def queries(i):
            return query_tiles(i, qk[0])

        def raise_top(i, j, m):
            top[i, j] = jnp.maximum(top[i, j], m) if (i, j) in top else m

        for job in jobs.split():
            kind, i, k = job[0], *(int(c) for c in job[1:].ljust(2, "0"))
            if kind == "P":
                for j in range(GH):
                    v = [v_s[pl.ds(16 * j + 8 * c, 8), _lane_tile(k)] for c in range(3)]
                    v[SUM_SLAB[j]] = jnp.where(row == SUM_ROW[j], 1.0, v[SUM_SLAB[j]])
                    o = _dot(jnp.concatenate(v, axis=0), probs(i, k)[j])
                    acc[i, j] = acc[i, j] + o if (i, j) in acc else o
            elif kind == "E":
                o = [acc[i, j] if j % 2 else pltpu.roll(acc[i, j], HT, 1) for j in range(GH)]
                o = [[oj[8 * c:8 * c + 8] for c in range(3)] for oj in o]
                den = mem_read[GR:GP, i * T:(i + 1) * T] + 1e-6 if s > 0 else jnp.ones((8, T), F32)
                for j in range(GH):
                    den = jnp.where(row == SUM_ROW[j], o[j][SUM_SLAB[j]], den)
                scale = mix_s[g] / den

                def per_head(rows):
                    return _merge_heads([[jnp.broadcast_to(scale[r:r + 1], (8, T))] * 3 for r in rows])

                mixed = _merge_heads(o) * per_head(SUM_ROW)
                if s > 0:
                    mixed = mixed + mem_read[0:GR, i * T:(i + 1) * T] * per_head(range(DEN_ROW, DEN_ROW + GH))
                ot_s[s][_ds(g * GP, GP, 16), _lane_tile(i)] = _pad_rows(mixed, GP).astype(BF16)
            elif kind == "L":
                diagonal = k >= i - 1
                n = i * T + HT - k * T if diagonal else T
                if v_s is not None:
                    probs(i, k)
                    if diagonal:
                        probs(i, i)
                st = key_logits(qk, k * T, n, queries(i))
                for j in range(GH):
                    sj = st[:, j * T:(j + 1) * T]
                    if diagonal:
                        end = sj[n - HT:] + head_masks[j % 2]
                        sj = end if n == HT else jnp.concatenate([sj[:n - HT], end], axis=0)
                    logit_s[i][j][pl.ds(k * T, n), :] = sj
                    raise_top(i, j, _rows_max(sj))
            elif kind == "C":
                if v_s is not None:
                    corner_probs(i)
                q = query_tiles(i, qk[0])
                first = _iota((GR, T), 1) < HT
                st = key_logits(qk, i * T + HT, HT, [jnp.where(first, q[j], q[j + 1]) for j in range(0, GH, 2)])
                for j in range(0, GH, 2):
                    sj = st[:, j // 2 * T:(j // 2 + 1) * T] + jnp.where(future, MASKED, 0.0)
                    corner_s[i][j // 2][...] = sj
                    m = _rows_max(sj)
                    raise_top(i, j, jnp.where(low, m, -jnp.inf))
                    raise_top(i, j + 1, jnp.where(low, -jnp.inf, m))
            elif kind == "M":
                if v_s is not None:
                    shift(i)
                for j in range(GH):
                    max_s[i * GH + j] = jnp.broadcast_to(jnp.max(top[i, j], axis=0, keepdims=True), (8, T))

    def route():
        r = _rnd(jnp.concatenate([score_s[s] for s in range(NSEG)], axis=1))
        r = jnp.clip(jnp.where(jnp.abs(r) < F32_TINY, F32_TINY, r), -BF16_MAX, BF16_MAX)
        tok = _iota((8, S), 1)
        key = pltpu.bitcast(pltpu.bitcast(r, jnp.int32) | jnp.where(r > 0, S - 1 - tok, tok), F32)
        k0 = jnp.max(key, axis=1, keepdims=True)
        k1 = jnp.max(jnp.where(key == k0, -jnp.inf, key), axis=1, keepdims=True)
        best = jnp.broadcast_to(jnp.where(_iota((8, 1), 0) == 0, k0, k1), (8, T))
        bits = pltpu.bitcast(best, jnp.int32)
        pos = jnp.where(best > 0, S - 1 - (bits & (S - 1)), bits & (S - 1))
        return (pos[0, 0], pos[1, 0]), jax.nn.sigmoid(pltpu.bitcast(bits & -(1 << 16), F32))

    def gather(idx):
        xs = jnp.zeros((8, DP), F32)
        for c in range(2):
            tile = xn_s[idx[c] // L, :, _lane_tile((idx[c] % L) // T)]
            hot = ((_iota((8, T), 1) == idx[c] % T) & (_iota((8, T), 0) == c)).astype(F32)
            xs = xs + _dot_nt(hot, tile)
        xsel_s[...] = jnp.concatenate([xs[:, g * GP:g * GP + GR] for g in range(NG)], axis=1)
        y_s[...] = jnp.zeros((8, DP), F32)

    def gate_up_jobs(p):
        n = F // T // NP
        pre = {}

        def last_rows(m):
            rows = pl.ds(4 * T, D - 4 * T)
            pre[m] = _dot(xsel_s[:, rows], (wg_s, wu_s)[m][rows, _ds(p * n * T, n * T, T)])

        def first_rows(t, m):
            rows, cols = pl.ds(0, 4 * T), _lane_tile(p * n + t)
            pre[m, t] = _dot(xsel_s[:, rows], (wg_s, wu_s)[m][rows, cols]) + pre[m][:, t * T:(t + 1) * T]
            if m == 1:
                h_s[:, cols] = pre[0, t] * jax.nn.sigmoid(pre[0, t]) * pre[1, t]

        return ([functools.partial(last_rows, m) for m in range(2)]
                + [functools.partial(first_rows, t, m) for t in range(n) for m in range(2)])

    def down_jobs(p):
        n = F // T // (NP - 1)

        def piece(c, d):
            rows, cols = pl.ds(d * T, min(T, D - d * T)), _ds((p * n + 4 * c) * T, 4 * T, T)
            y_s[:, rows] += _dot_nt(h_s[:, cols], wd_s[rows, cols])

        return [functools.partial(piece, c, d) for c in range(n // 4) for d in range(DP // T)]

    def place_updates(idx, r_sel):
        yt = _pad_rows(y_s[...] * jnp.concatenate([r_sel] * (DP // T), axis=1), T).T[:D]
        for c in range(2):
            upd = pltpu.roll(yt, (idx[c] + T - c) % T, 1)
            upd_s[c] = jnp.where(_iota((D, T), 1) == idx[c] % T, upd, 0.0).reshape(NG, GR, T)

    def add_updates(idx):
        for c in range(2):
            s, lanes = idx[c] // L, _lane_tile((idx[c] % L) // T)

            @pl.when(s < NSEG - 1)
            def _():
                out_s[s, :, :, lanes] = (out_s[s, :, :, lanes].astype(F32) + upd_s[c]).astype(BF16)

    def step(s, p, last=False):
        fillers = []
        if s == NSEG - 2:
            fillers = gate_up_jobs(p)
        elif s == NSEG - 1 and not last:
            fillers = down_jobs(p)
        reads = [memory(s, 2 * p + e, qkv_s[e]) for e in range(2)]
        v_held[...] = qkv_s[1][2][...]
        attention(s, 2 * p, JOBS_A, reads[0], qkv_s[0][2], qkv_s[1])
        if not last:
            nxt = s * NP + p + 1
            project(nxt // NP, nxt % NP, fillers)
            if s == 0:
                layer_norm_background(NT + 2 * p)
                layer_norm_background(NT + 2 * p + 1)
                for e in range(3):
                    transpose_w(jnp.where(p < 2, e, 3),
                                jnp.where(p < 2, p + 3, jnp.minimum(3 * (p - 2) + e, 4)))
            elif s == 1:
                layer_norm_background(3 * NT + p)
            attention(s, 2 * p + 1, JOBS_B[s], reads[1], v_held, qkv_s[0])
        if s > 0:
            out_project(s - 1, p, fillers)
        assert not fillers
        return reads[1]

    def first_dot(i, tokens=slice(None)):
        return _dot(wt_s[i, pair_rows(0), :], xn_s[0, :, tokens])

    zero_s[0] = 0
    for t in range(NT):
        x_copy(t, 1).start()
    for t in range(NT):
        x_copy(t, 1).wait()
        if t < 3:
            w_copy((1, 0, 2)[t], 0).start()
        if t == 2:
            wr_copy.start()
            beta_copy.start()
        layer_norm_now(t)
    w_copy(1, 0).wait()
    for i in range(3):
        w_copy(i, 1).start()
    for c in range(2):
        transpose_w(1, c)
    kt = first_dot(1, pl.ds(0, L // 2))
    w_copy(0, 0).wait()
    kt = jnp.concatenate([kt, first_dot(1, pl.ds(L // 2, L // 2))], axis=1)
    for c in range(2):
        transpose_w(0, c)
    w_copy(2, 0).wait()
    wr_copy.wait()
    beta_copy.wait()
    x_copy(NT, NT).start()
    for i in range(3):
        w_copy(i, 2).start()
    keep(1, kt)
    keep(0, first_dot(0))
    for c in range(2):
        transpose_w(2, c)
    make_mix()
    router_s[...] = _pad_groups(jnp.broadcast_to(wr_s[...].astype(F32).reshape(1, D), (8, D)), 1)
    keep(2, first_dot(2))
    for i in range(3):
        w_copy(i, 1).wait()
    for i in range(4):
        w_copy(i, 3).start()
    x_copy(2 * NT, NT).start()
    w_copy(3, 0).start()
    x_copy(3 * NT, NT).start()
    score_s[0] = _dot(router_s[...], xn_s[0])
    attention(0, 0, JOBS_FIRST, None, None, qkv_s[0])
    for i in range(3):
        transpose_w(i, 2)
    x_copy(NT, NT).wait()
    for i in range(3):
        w_copy(i, 2).wait()

    for s in range(NSEG):
        def body(p, carry, s=s):
            if s == 0:
                @pl.when(p == 1)
                def _():
                    for i in range(4):
                        w_copy(i, 3).wait()
                        w_s[i, :, _lane_tile(4)] = jnp.concatenate([w_end_s[i], jnp.zeros((D, HT), BF16)], axis=1)
                    x_copy(2 * NT, NT).wait()
                    w_copy(3, 0).wait()
                    x_copy(3 * NT, NT).wait()
                    for i in range(3):
                        ffn_copy(i).start()
            if s >= 2:
                pl.when(p == 1)(lambda: segment_store(s - 2).start())
            step(s, p)
            return carry

        lax.fori_loop(0, NP if s < NSEG - 1 else NP - 1, body, 0)
        if s == 1:
            for i in range(3):
                ffn_copy(i).wait()
            idx, r_sel = route()
            gather(idx)

    s = NSEG - 1
    segment_store(0).wait()
    segment_store(1).wait()
    place_updates(idx, r_sel)
    mem_read = step(s, NP - 1, last=True)
    attention(s, NG - 1, "P00 E0", mem_read, v_held, None)
    add_updates(idx)
    segment_store(2).start()
    tiles = [i // T for i in idx]
    again = [tiles[0] < 2 * NT, (tiles[1] < 2 * NT) & (tiles[1] != tiles[0])]
    for c in range(2):
        pl.when(again[c])(lambda c=c: tile_store(tiles[c], NT + c).start())
    for t in range(NT):
        if t + 1 < NT:
            jobs = " ".join(f"P{t + 1}{k}" for k in range(t + 2)) + f" E{t + 1}"
            attention(s, NG - 1, jobs, mem_read, v_held, None)
        lanes = _lane_tile(t)
        a = _dot(wt_s[3, pl.ds(0, D), pl.ds(0, 4 * T)], ot_s[s][pl.ds(0, 4 * T), lanes])
        a = a + jnp.concatenate([_dot(wt_s[3, pair_rows(q), pl.ds(4 * T, T)], ot_s[s][pl.ds(4 * T, T), lanes])
                                 for q in range(NP)], axis=0)
        a = a.reshape(NG, GR, T)
        for c in range(2):
            a = a + jnp.where(tiles[c] == s * NT + t, upd_s[c], 0.0)
        for g in range(NG):
            out_s[s, g, :, lanes] = (residual(s, g, lanes) + a[g]).astype(BF16)
        tile_store(s * NT + t, t).start()
    for c in range(2):
        pl.when(again[c])(lambda c=c: tile_store(tiles[c], NT + c).wait())
    segment_store(2).wait()
    for t in range(NT):
        tile_store(s * NT + t, t).wait()


@jax.jit
def pallas_parallel_sum__memory_aug_infini_attn__moe_arch_mod__prompt_kernel(
    A_x, A_wq, A_wk, A_wv, A_wo, A_beta, B_x, B_w_r, B_w_gate, B_w_up, B_w_down,
):
    del B_x
    hbm = pl.BlockSpec(memory_space=pltpu.HBM)
    group = (pltpu.VMEM((GR, L), F32),
             pltpu.VMEM((L, T), BF16),
             pltpu.VMEM((GR, L), F32),
             pltpu.VMEM((GR, L), F32),
             pltpu.VMEM((L, T), BF16))
    out = pl.pallas_call(
        _kernel,
        out_shape=jax.ShapeDtypeStruct((NG, GR, S), BF16),
        in_specs=[hbm] * 10,
        out_specs=hbm,
        scratch_shapes=[
            pltpu.VMEM((NSEG, NG, GR, L), BF16),
            pltpu.VMEM((4, D, DP), BF16),
            pltpu.VMEM((4, D, HT), BF16),
            pltpu.VMEM((H,), BF16),
            pltpu.VMEM((D,), BF16),
            pltpu.VMEM((D, F), BF16),
            pltpu.VMEM((D, F), BF16),
            pltpu.VMEM((D, F), BF16),
            pltpu.VMEM((NSEG, DP, L), BF16),
            pltpu.VMEM((4, DP, DP), BF16),
            pltpu.VMEM((8, DP), F32),
            pltpu.VMEM((NG, 8, T), F32),
            pltpu.VMEM((NG, GP, T), F32),
            [pltpu.VMEM((DP, L), BF16)] * NSEG,
            pltpu.VMEM((NSEG, NG, GR, L), BF16),
            (group, group),
            pltpu.VMEM((GR, L), F32),
            [[pltpu.VMEM((i * T + HT, T), F32)] * GH for i in range(NT)],
            [[pltpu.VMEM((HT, T), F32)] * (GH // 2)] * NT,
            pltpu.VMEM((NT * GH, 8, T), F32),
            pltpu.VMEM((NSEG, 8, L), F32),
            pltpu.VMEM((8, D), F32),
            pltpu.VMEM((8, F), F32),
            pltpu.VMEM((8, DP), F32),
            pltpu.VMEM((2, NG, GR, T), F32),
            pltpu.VMEM((2, 8, T), F32),
            pltpu.SMEM((1,), jnp.int32),
            pltpu.SemaphoreType.DMA((NSEG * NT,)),
            pltpu.SemaphoreType.DMA((16,)),
            pltpu.SemaphoreType.DMA((14,)),
        ],
        compiler_params=pltpu.CompilerParams(vmem_limit_bytes=100 * 1024 * 1024),
        name="infini_mod",
    )(jnp.transpose(A_x[0]).reshape(NG, GR, S), A_wq, A_wk, A_wv, A_wo, A_beta, B_w_r,
      B_w_gate, B_w_up, jnp.transpose(B_w_down))
    return jnp.transpose(out.reshape(D, S))[None]
```
